```python
import jax
import jax.numpy as jnp

def _softmax(x, axis=-1):
    return jax.nn.softmax(x, axis=axis)
def _gelu(x):
    return jax.nn.gelu(x, approximate=True)
def _silu(x):
    return jax.nn.silu(x)
def _sigmoid(x):
    return jax.nn.sigmoid(x)
def _layernorm(x, axis=-1, eps=1e-5):
    m = jnp.mean(x, axis=axis, keepdims=True)
    v = jnp.var(x, axis=axis, keepdims=True)
    return (x - m) / jnp.sqrt(v + eps)
def _scatter_add(tgt, idx, src, axis=0):
    return tgt.at[idx].add(src)
def _segment_sum(src, seg, n):
    return jax.ops.segment_sum(src, seg, n)
class _Rng:
    def __init__(self, key):
        self._k = key
    def _next(self):
        self._k, sub = jax.random.split(self._k)
        return sub
    def normal(self, shape):
        return jax.random.normal(self._next(), shape, dtype=jnp.bfloat16)
    def randint(self, lo, hi, shape):
        return jax.random.randint(self._next(), shape, lo, hi, dtype=jnp.int32)
    def uniform(self, shape, lo=0.0, hi=1.0):
        return jax.random.uniform(self._next(), shape, jnp.bfloat16, lo, hi)
    def permutation(self, n):
        return jax.random.permutation(self._next(), n)


kernel_name = 'recurrent_scan__ssm_conv_s4__moe_arch_mod__prompt'

def setup_inputs():
    _rng = _Rng(jax.random.key(int.from_bytes(__import__("os").urandom(4), "little")))
    _w = (lambda a: (lambda t: t.astype(jnp.bfloat16) if jnp.issubdtype(t.dtype, jnp.floating) else t)(jnp.asarray(a)))
    def _A_setup():
        B, L, D, N = 1, 2048, 576, 128
        A_re = -jnp.exp((lambda *s: _rng.normal(s) * 0.05)(D, N))
        A_im = jnp.pi * (lambda *s: _rng.normal(s) * 0.05)(D, N)
        B_re = (lambda *s: _rng.normal(s) * 0.05)(D, N)
        B_im = (lambda *s: _rng.normal(s) * 0.05)(D, N)
        C_re = (lambda *s: _rng.normal(s) * 0.05)(D, N)
        C_im = (lambda *s: _rng.normal(s) * 0.05)(D, N)
        log_dt = (lambda *s: _rng.normal(s) * 0.05)(D) * 0.5 - 4.0
        Dskip = (lambda *s: _rng.normal(s) * 0.05)(D)
        return {
            "u": _w((lambda *s: _rng.normal(s) * 0.05)(B, L, D)),
            "A_re": _w(A_re),
            "A_im": _w(A_im),
            "B_re": _w(B_re),
            "B_im": _w(B_im),
            "C_re": _w(C_re),
            "C_im": _w(C_im),
            "log_dt": _w(log_dt),
            "Dskip": _w(Dskip),
        }
    _A_in = _A_setup()

    def _B_setup():
        B, S, D, F, C = 1, 2048, 576, 4608, 8
        return {
            "x": _w((lambda *s: _rng.normal(s) * 0.05)(B, S, D)),
            "w_r": _w((lambda *s: _rng.normal(s) * 0.05)(D)),
            "w_gate": _w((lambda *s: _rng.normal(s) * 0.05)(D, F)),
            "w_up": _w((lambda *s: _rng.normal(s) * 0.05)(D, F)),
            "w_down": _w((lambda *s: _rng.normal(s) * 0.05)(F, D)),
        }
    _B_in = _B_setup()

    return {
        "A_u": _A_in["u"],
        "A_A_re": _A_in["A_re"],
        "A_A_im": _A_in["A_im"],
        "A_B_re": _A_in["B_re"],
        "A_B_im": _A_in["B_im"],
        "A_C_re": _A_in["C_re"],
        "A_C_im": _A_in["C_im"],
        "A_log_dt": _A_in["log_dt"],
        "A_Dskip": _A_in["Dskip"],
        "B_x": _B_in["x"],
        "B_w_r": _B_in["w_r"],
        "B_w_gate": _B_in["w_gate"],
        "B_w_up": _B_in["w_up"],
        "B_w_down": _B_in["w_down"],
    }

def reference(A_u, A_A_re, A_A_im, A_B_re, A_B_im, A_C_re, A_C_im, A_log_dt, A_Dskip, B_x, B_w_r, B_w_gate, B_w_up, B_w_down):
    def _A_ref(u, A_re, A_im, B_re, B_im, C_re, C_im, log_dt, Dskip):
        Bsz, L, D = u.shape
        dt = jnp.exp(log_dt)[:, None]
        A = A_re + 1j * A_im
        Bc = B_re + 1j * B_im
        Cc = C_re + 1j * C_im
        logdA = dt * A
        dB = dt * Bc
        l = (lambda x, dt: x.astype(dt))(jnp.arange(L), A_re.dtype)
        P = jnp.exp(logdA[:, :, None] * l[None, None, :])
        K = jnp.einsum("dn,dnl,dn->dl", Cc, P, dB).real
        L2 = 2 * L
        Kp = jnp.pad(K, ((0, 0), (0, L)))
        up = (lambda x, *d: x.transpose(*d))(u, 0, 2, 1)
        up = jnp.pad(up, ((0, 0), (0, 0), (0, L)))
        Kf = (lambda x, axes=(-2,-1): jnp.fft.rfft2(x.astype(jnp.float32), axes=axes))(Kp[:, None, :], axes=(-2, -1))
        Uf = (lambda x, axes=(-2,-1): jnp.fft.rfft2(x.astype(jnp.float32), axes=axes))(up[:, :, None, :], axes=(-2, -1))
        Yf = Uf * Kf[None, :, :, :]
        y = (lambda x, s, axes=(-2,-1): jnp.fft.irfft2(x, s=s, axes=axes).astype(jnp.bfloat16))(Yf, (1, L2), axes=(-2, -1))[:, :, 0, :L]
        y = (lambda x, *d: x.transpose(*d))(y, 0, 2, 1) + u * Dskip[None, None, :]
        return y

    def _B_ref(x, w_r, w_gate, w_up, w_down):
        B, S, D = x.shape
        C = 8
        r = x @ w_r
        idx = jnp.argsort(-r, axis=-1)[:, :C]
        idx_e = jnp.repeat(idx.reshape(B, C, 1), D, axis=2)
        x_sel = jnp.take_along_axis(x, idx_e, axis=1)
        g = _silu(x_sel @ w_gate)
        u = x_sel @ w_up
        y = (g * u) @ w_down
        r_sel = _sigmoid(jnp.take_along_axis(r, idx, axis=1))
        y = y * r_sel.reshape(B, C, 1)
        b_off = (jnp.arange(B) * S).reshape(B, 1)
        flat_idx = (idx + b_off).reshape(B * C)
        zero = (x * 0.0).reshape(B * S, D)
        upd = _scatter_add(zero, flat_idx, y.reshape(B * C, D), axis=0)
        return x + upd.reshape(B, S, D)

    x = A_u
    xn = _layernorm(x, axis=-1)
    s = _A_ref(xn, A_A_re, A_A_im, A_B_re, A_B_im, A_C_re, A_C_im, A_log_dt, A_Dskip)
    g = _silu(_B_ref(xn, B_w_r, B_w_gate, B_w_up, B_w_down))
    return x + s * g
```

```python
import functools

import jax
import jax.numpy as jnp
import numpy as np
import jax.experimental.pallas as pl
import jax.experimental.pallas.tpu as pltpu

F32 = jnp.float32
BF16 = jnp.bfloat16
P = 128


def _bf16_bits(a):
    u = np.ascontiguousarray(a, dtype=np.float32).view(np.uint32)
    return ((u + 0x7FFF + ((u >> 16) & 1)) >> 16).astype(np.uint32)


def _round_bf16(a):
    return (_bf16_bits(a) << 16).view(np.float32)


def _pack_rows(a):
    b = _bf16_bits(a)
    return (b[0::2] | (b[1::2] << 16)).astype(np.uint32)


_BASE = (
    tuple(1 + a for a in range(8)),
    tuple(129 + a for a in range(8)),
    tuple(256 + 128 * (a // 4) + 2 * (a % 4 + 1) for a in range(8)),
    tuple(512 + 128 * (a // 2) + 4 * (a % 2 + 1) for a in range(8)),
    tuple(1032 + 128 * a for a in range(8)),
)
_MERGED = ((2, 3, 2), (4, 3, 2), (4, 4, 3))
_SRC = ((0,), (0, 1), (1, 2), (1, 2), (5,), (6,), (3,), (3,), (7,), (7,)) + ((4,),) * 6


def _tables():
    k = np.arange(P)
    phi = 2 * np.pi * (k + 0.25) / P

    def coords(m):
        z = np.exp(1j * np.outer(m, phi))
        return np.concatenate([z.real + z.imag / np.sqrt(3), 2 * z.imag / np.sqrt(3)], axis=1)

    fu = 2.0 * coords(np.arange(P))
    zi = np.exp(-1j * np.outer(phi, np.arange(P)))
    fi = np.concatenate([zi.real, (np.exp(2j * np.pi / 3) * zi).real], axis=0) / P
    lane = np.arange(P)
    lags = [np.array(b)[lane // 16] + 8 * (lane % 16) for b in _BASE]
    for thr, lo, hi in _MERGED:
        lags.append(np.where(lane // 16 < thr, lags[lo], lags[hi]))
    gs = []
    for j, src in enumerate(_SRC):
        m = np.arange(-P + 1, P)
        m = m[P * j + m >= 1]
        rl = _round_bf16(P * j + m)
        cm = coords(m)
        hit = np.zeros(len(m), int)
        for t in src:
            sel = (lags[t][:, None] == rl[None, :])
            hit += sel.sum(0)
            gs.append(sel.astype(np.float64) @ cm)
        assert (hit == 1).all(), (j, hit)
    return _pack_rows(fu), _pack_rows(fi), _pack_rows(np.concatenate(gs, axis=0))


def _cmul(a, b):
    return (a[0] * b[0] - a[1] * b[1], a[0] * b[1] + a[1] * b[0])


def _csq(a):
    t = a[0] * a[1]
    return ((a[0] - a[1]) * (a[0] + a[1]), t + t)


def _dot(a, b):
    return jax.lax.dot_general(a, b, (((1,), (0,)), ((), ())), preferred_element_type=F32)


def _dot_nt(a, b):
    return jax.lax.dot_general(a, b, (((1,), (1,)), ((), ())), preferred_element_type=F32)


def _rbf(x):
    return x.astype(BF16).astype(F32)


def _kernel(x_hbm, are_ref, aim_ref, bre_ref, bim_ref, cre_ref, cim_ref, ldt_ref, dsk_ref,
            wr_ref, wg_hbm, wu_hbm, wd_hbm, fu_hbm, fi_hbm, g_hbm, o_hbm,
            x_v, wg_v, wu_v, wd_v, fu_v, fi_v, g_v, o_v, h_v, s_v, kc_v, dt_v, d0_v,
            key_v, oh_v, act_v, uh_v, kh_v, yh_v, sems, osem,
            *, GA, GD, NF, GE, debug):
    D, L = x_v.shape
    FF = wg_v.shape[1]
    NB = L // P
    FC = FF // NF
    NE = D // GE

    cx = pltpu.make_async_copy(x_hbm, x_v, sems.at[0])
    cfu = pltpu.make_async_copy(fu_hbm, fu_v, sems.at[1])
    cfi = pltpu.make_async_copy(fi_hbm, fi_v, sems.at[2])
    cg = pltpu.make_async_copy(g_hbm, g_v, sems.at[3])

    def cwg(i):
        return pltpu.make_async_copy(wg_hbm.at[:, pl.ds(i * FC, FC)], wg_v.at[:, pl.ds(i * FC, FC)], sems.at[4 + i])

    def cwu(i):
        return pltpu.make_async_copy(wu_hbm.at[:, pl.ds(i * FC, FC)], wu_v.at[:, pl.ds(i * FC, FC)], sems.at[4 + NF + i])

    def cwd(i):
        r = pl.ds(pl.multiple_of(i * GE, GE), GE)
        return pltpu.make_async_copy(wd_hbm.at[r], wd_v.at[r], sems.at[4 + 2 * NF + i])

    def cout(i):
        r = pl.ds(pl.multiple_of(i * GE, GE), GE)
        return pltpu.make_async_copy(o_v.at[r], o_hbm.at[r], osem.at[i])

    cx.start()
    cfu.start()
    cfi.start()
    cg.start()
    for i in range(NF):
        cwg(i).start()
        cwu(i).start()
    for i in range(NE):
        cwd(i).start()

    dt_row = _rbf(jnp.exp(ldt_ref[...].astype(F32)[None, :]))
    dsk_row = dsk_ref[...].astype(F32)[None, :]
    for row, dst in ((dt_row, dt_v), (dsk_row, d0_v)):
        for c0 in range(0, D, P):
            n = min(P, D - c0)
            eye = (jax.lax.broadcasted_iota(jnp.int32, (n, n), 0)
                   == jax.lax.broadcasted_iota(jnp.int32, (n, n), 1))
            dst[c0:c0 + n, :] = _dot(jnp.where(eye, row[:, c0:c0 + n], 0.0), jnp.ones((n, P), F32))

    lane8 = jax.lax.broadcasted_iota(jnp.int32, (8, P), 1)
    sub8 = jax.lax.broadcasted_iota(jnp.int32, (8, P), 0)

    def kgen(i, _):
        r0 = pl.multiple_of(i * GA, GA)
        rows = pl.ds(r0, GA)
        dt = dt_v[rows, :]
        a_re = dt * are_ref[rows, :].astype(F32)
        a_im = dt * aim_ref[rows, :].astype(F32)
        db = (dt * bre_ref[rows, :].astype(F32), dt * bim_ref[rows, :].astype(F32))
        w = _cmul((cre_ref[rows, :].astype(F32), cim_ref[rows, :].astype(F32)), db)
        d0_v[rows, :] = d0_v[rows, :] + jnp.sum(w[0], axis=1, keepdims=True)
        mag = jnp.exp(a_re)
        z1 = (mag * jnp.cos(a_im), mag * jnp.sin(a_im))
        bit = [(lane8 & (16 << b)) == 0 for b in range(3)]
        diag = (lane8 & 15) * 8 + sub8
        for g in range(GA // 8):
            sl = slice(8 * g, 8 * g + 8)
            z = {1: (z1[0][sl], z1[1][sl])}
            for e in range(10):
                z[2 << e] = _csq(z[1 << e])
            bs = {0: (jnp.ones((8, P), F32), jnp.zeros((8, P), F32))}
            for j in range(1, 16):
                hb = 1 << (j.bit_length() - 1)
                if j == hb:
                    bs[j] = (z[8 * j][0], -z[8 * j][1])
                else:
                    bs[j] = _cmul(bs[hb], bs[j - hb])
            av = {0: (w[0][sl], w[1][sl])}

            def aval(e):
                if e not in av:
                    hb = 1 << (e.bit_length() - 1)
                    av[e] = _cmul(aval(e - hb), z[hb])
                return av[e]

            b_re = jnp.concatenate([bs[j][0] for j in range(16)], axis=0)
            b_im = jnp.concatenate([bs[j][1] for j in range(16)], axis=0)
            l_re = jnp.concatenate([aval(e)[0] for t in _BASE for e in t], axis=0)
            l_im = jnp.concatenate([aval(e)[1] for t in _BASE for e in t], axis=0)
            out = _dot_nt(l_re, b_re) + _dot_nt(l_im, b_im)
            tiles = []
            for t in range(5):
                v = [out[(8 * t + a) * 8:(8 * t + a + 1) * 8] for a in range(8)]
                v = [jnp.take_along_axis(u, diag, axis=1, mode='promise_in_bounds') for u in v]
                for b in range(3):
                    v = [jnp.where(bit[b], v[2 * q], v[2 * q + 1]) for q in range(len(v) // 2)]
                tiles.append(v[0])
            for thr, lo, hi in _MERGED:
                tiles.append(jnp.where(lane8 < 16 * thr, tiles[lo], tiles[hi]))
            for t, tile in enumerate(tiles):
                kc_v[t, pl.ds(pl.multiple_of(r0 + 8 * g, 8), 8), :] = tile
        return 0

    with jax.named_scope("kgen"):
        jax.lax.fori_loop(0, D // GA, kgen, 0)

    cx.wait()
    wr = jnp.broadcast_to(2.0 * wr_ref[...].astype(F32)[None, :], (8, D))
    LB = 2 * P

    def lnorm(c, _):
        cols = pl.ds(pl.multiple_of(c * LB, LB), LB)
        xf = x_v[:, cols].astype(F32)
        m = jnp.sum(xf, axis=0, keepdims=True) / D
        mb = _rbf(m)
        d = xf - mb
        var = jnp.sum(d * d, axis=0, keepdims=True) / D - (m - mb) * (m - mb)
        sd = _rbf(jnp.sqrt(_rbf(_rbf(jnp.maximum(var, 0.0)) + _rbf(jnp.full_like(var, 1e-5)))))
        h = (_rbf(d) * (0.5 / sd)).astype(BF16)
        h_v[:, cols] = h
        r = _rbf(_dot(wr, h))
        bits = pltpu.bitcast(jnp.where(r == 0.0, 0.0, r), jnp.int32)
        ordered = jnp.where(bits < 0, ~bits, bits ^ jnp.int32(-2**31))
        idx = c * LB + jax.lax.broadcasted_iota(jnp.int32, (8, LB), 1)
        key = (jax.lax.shift_right_logical(ordered, 16) << 11) + (0x20000000 + L - 1 - idx)
        key_v[:, cols] = pltpu.bitcast(key, F32)
        return 0

    with jax.named_scope("lnorm"):
        jax.lax.fori_loop(0, L // LB, lnorm, 0)

    with jax.named_scope("topk"):
        ks = []
        for hf in range(NB // 8):
            kk = key_v[:, hf * 8 * P:(hf * 8 + 1) * P]
            for q in range(1, 8):
                kk = jnp.where(sub8 == q, key_v[:, (hf * 8 + q) * P:(hf * 8 + q + 1) * P], kk)
            ks.append(kk)
        top = jnp.zeros((8, P), F32)
        for q in range(8):
            mx = jnp.max(functools.reduce(jnp.maximum, ks), axis=0, keepdims=True)
            mx = jnp.max(mx, axis=1, keepdims=True)
            top = jnp.where(sub8 == q, mx, top)
            ks = [jnp.where(kk == mx, 0.0, kk) for kk in ks]
        for c in range(NB):
            oh_v[:, c * P:(c + 1) * P] = jnp.where(key_v[:, c * P:(c + 1) * P] == top, 1.0, 0.0)
        o16 = jax.lax.shift_right_logical(pltpu.bitcast(top, jnp.int32) - 0x20000000, 11) << 16
        r_top = pltpu.bitcast(jnp.where(o16 < 0, o16 ^ jnp.int32(-2**31), (~o16) & jnp.int32(-65536)), F32)
        gate = jax.nn.sigmoid(r_top)
        x_sel = 2.0 * _dot_nt(oh_v[...], h_v[...])

    cfu.wait()
    cfi.wait()
    cg.wait()

    def conv(i, _):
        r0 = pl.multiple_of(i * GD, GD)
        rows = pl.ds(r0, GD)
        lhs = jnp.concatenate([h_v[rows, c * P:(c + 1) * P] for c in range(NB)], axis=0)
        uh = _dot(lhs, pltpu.bitcast(fu_v[...], BF16))
        for c in range(NB):
            a = uh[c * GD:(c + 1) * GD, :P]
            b = uh[c * GD:(c + 1) * GD, P:]
            uh_v[0, c] = a
            uh_v[1, c] = b
            uh_v[2, c] = a - b
        gi = 0
        for j, src in enumerate(_SRC):
            kh = None
            for t in src:
                part = _dot(kc_v[t, rows, :], pltpu.bitcast(g_v[gi * 64:(gi + 1) * 64, :], BF16))
                kh = part if kh is None else kh + part
                gi += 1
            a = kh[:, :P]
            b = kh[:, P:]
            if j == 0:
                a = a + d0_v[rows, :]
            kh_v[0, j] = a
            kh_v[1, j] = b
            kh_v[2, j] = a - b
        for g in range(GD // 8):
            sl = slice(8 * g, 8 * g + 8)
            for c in range(NB):
                m0 = kh_v[0, 0, sl, :] * uh_v[0, c, sl, :]
                for j in range(1, c + 1):
                    m0 = m0 + kh_v[0, j, sl, :] * uh_v[0, c - j, sl, :]
                for q in (1, 2):
                    acc = m0
                    for j in range(c + 1):
                        acc = acc - kh_v[q, j, sl, :] * uh_v[q, c - j, sl, :]
                    yh_v[c * GD + 8 * g:c * GD + 8 * g + 8, (q - 1) * P:q * P] = acc
        y = _dot(yh_v[...], pltpu.bitcast(fi_v[...], BF16))
        for c in range(NB):
            s_v[rows, c * P:(c + 1) * P] = y[c * GD:(c + 1) * GD]
        return 0

    with jax.named_scope("conv"):
        jax.lax.fori_loop(0, D // GD, conv, 0)

    with jax.named_scope("gateup"):
        for i in range(NF):
            cwg(i).wait()
            cwu(i).wait()
            a = 0.5 * _dot(x_sel, wg_v[:, i * FC:(i + 1) * FC])
            u = _dot(x_sel, wu_v[:, i * FC:(i + 1) * FC])
            act_v[:, i * FC:(i + 1) * FC] = (a + a * jnp.tanh(a)) * u

    def final(i, _):
        rows = pl.ds(pl.multiple_of(i * GE, GE), GE)
        cwd(i).wait()
        y = _dot_nt(act_v[...], wd_v[rows, :]) * (0.5 * gate[:, :GE])
        eye = (jax.lax.broadcasted_iota(jnp.int32, (GE, GE), 0)
               == jax.lax.broadcasted_iota(jnp.int32, (GE, GE), 1)).astype(F32)
        yt = _dot_nt(eye, y)
        h = h_v[rows, :].astype(F32) + _dot(yt, oh_v[...])
        q = s_v[rows, :] * h
        out = (x_v[rows, :].astype(F32) + q) + q * jnp.tanh(h)
        if debug:
            out = s_v[rows, :]
        o_v[rows, :] = out.astype(o_v.dtype)
        cout(i).start()
        return 0

    with jax.named_scope("final"):
        jax.lax.fori_loop(0, NE, final, 0)
        for i in range(NE):
            cout(i).wait()


def run(A_u, A_A_re, A_A_im, A_B_re, A_B_im, A_C_re, A_C_im, A_log_dt, A_Dskip, B_x, B_w_r,
        B_w_gate, B_w_up, B_w_down, GA=16, GD=32, NF=4, GE=64, debug=False, interpret=False):
    _, L, D = A_u.shape
    FF = B_w_gate.shape[1]
    fu, fi, g = _tables()
    odt = F32 if debug else A_u.dtype
    hbm = pl.BlockSpec(memory_space=pl.ANY)
    vm = pl.BlockSpec(memory_space=pltpu.VMEM)
    NB = L // P
    out = pl.pallas_call(
        functools.partial(_kernel, GA=GA, GD=GD, NF=NF, GE=GE, debug=debug),
        out_shape=jax.ShapeDtypeStruct((D, L), odt),
        in_specs=[hbm] + [vm] * 9 + [hbm] * 6,
        out_specs=hbm,
        scratch_shapes=[
            pltpu.VMEM((D, L), BF16), pltpu.VMEM((D, FF), BF16), pltpu.VMEM((D, FF), BF16),
            pltpu.VMEM((D, FF), BF16),
            pltpu.VMEM(fu.shape, jnp.uint32), pltpu.VMEM(fi.shape, jnp.uint32),
            pltpu.VMEM(g.shape, jnp.uint32),
            pltpu.VMEM((D, L), odt), pltpu.VMEM((D, L), BF16), pltpu.VMEM((D, L), F32),
            pltpu.VMEM((8, D, P), F32), pltpu.VMEM((D, P), F32), pltpu.VMEM((D, P), F32),
            pltpu.VMEM((8, L), F32), pltpu.VMEM((8, L), F32), pltpu.VMEM((8, FF), F32),
            pltpu.VMEM((3, NB, GD, P), F32), pltpu.VMEM((3, NB, GD, P), F32),
            pltpu.VMEM((NB * GD, 2 * P), F32),
            pltpu.SemaphoreType.DMA((4 + 2 * NF + D // GE,)),
            pltpu.SemaphoreType.DMA((D // GE,)),
        ],
        compiler_params=pltpu.CompilerParams(vmem_limit_bytes=100 * 2**20),
        interpret=interpret,
        name="ssm_moe",
    )(A_u[0].T, A_A_re, A_A_im, A_B_re, A_B_im, A_C_re, A_C_im, A_log_dt, A_Dskip, B_w_r,
      B_w_gate, B_w_up, B_w_down.T, fu, fi, g)
    return out.T[None]


@jax.jit
def pallas_recurrent_scan__ssm_conv_s4__moe_arch_mod__prompt_kernel(
    A_u: jax.Array,
    A_A_re: jax.Array,
    A_A_im: jax.Array,
    A_B_re: jax.Array,
    A_B_im: jax.Array,
    A_C_re: jax.Array,
    A_C_im: jax.Array,
    A_log_dt: jax.Array,
    A_Dskip: jax.Array,
    B_x: jax.Array,
    B_w_r: jax.Array,
    B_w_gate: jax.Array,
    B_w_up: jax.Array,
    B_w_down: jax.Array,
):
    return run(A_u, A_A_re, A_A_im, A_B_re, A_B_im, A_C_re, A_C_im, A_log_dt, A_Dskip, B_x,
               B_w_r, B_w_gate, B_w_up, B_w_down)
```

```python
import functools

import jax
import jax.numpy as jnp
import numpy as np
import jax.experimental.pallas as pl
import jax.experimental.pallas.tpu as pltpu

F32 = jnp.float32
BF16 = jnp.bfloat16
P = 128


def _bf16_bits(a):
    u = np.ascontiguousarray(a, dtype=np.float32).view(np.uint32)
    return ((u + 0x7FFF + ((u >> 16) & 1)) >> 16).astype(np.uint32)


def _round_bf16(a):
    return (_bf16_bits(a) << 16).view(np.float32)


def _pack_rows(a):
    b = _bf16_bits(a)
    return (b[0::2] | (b[1::2] << 16)).astype(np.uint32)


def _tile_lags():
    lane = np.arange(P)
    quarter, hb, j = lane // 32, (lane // 16) % 2, lane % 16

    def half(offsets, second):
        q = (quarter + 2 * second) % 4
        return np.array(offsets)[q] + 128 * (hb ^ second) + 8 * j

    l1, u1 = half((1, 2, 3, 4), 0), half((5, 6, 7, 8), 1)
    l2, u2 = half((258, 260, 516, 772), 0), half((262, 264, 520, 776), 1)
    l3, u3 = half((1032, 1288) * 2, 0), half((1544, 1800) * 2, 1)
    lags = [np.where(hb == 0, l1, u1), np.where(hb == 0, u1, l1),
            np.where(lane < 64, l2, u2), np.where(lane < 64, u2, l2), np.where(lane < 64, l3, u3)]
    return lags


_SRC = ((0,), (0, 1), (1, 2), (1, 2), (2, 3), (2, 3), (3,), (3,), (5,), (5,)) + ((4,),) * 6


def _tables():
    k = np.arange(P)
    phi = 2 * np.pi * (k + 0.25) / P

    def coords(m):
        z = np.exp(1j * np.outer(m, phi))
        return np.concatenate([z.real + z.imag / np.sqrt(3), 2 * z.imag / np.sqrt(3)], axis=1)

    fu = 2.0 * coords(np.arange(P))
    zi = np.exp(-1j * np.outer(phi, np.arange(P)))
    fi = np.concatenate([zi.real, (np.exp(2j * np.pi / 3) * zi).real], axis=0) / P
    lags = _tile_lags()
    lags.append(np.where(np.arange(P) < 32, lags[4], lags[3]))
    gs = []
    for j, src in enumerate(_SRC):
        m = np.arange(-P + 1, P)
        m = m[P * j + m >= 1]
        rl = _round_bf16(P * j + m)
        cm = coords(m)
        hit = np.zeros(len(m), int)
        for t in src:
            sel = (lags[t][:, None] == rl[None, :])
            hit += sel.sum(0)
            gs.append(sel.astype(np.float64) @ cm)
        assert (hit == 1).all(), (j, hit)
    return _pack_rows(fu), _pack_rows(fi), _pack_rows(np.concatenate(gs, axis=0))


def _cmul(a, b):
    return (a[0] * b[0] - a[1] * b[1], a[0] * b[1] + a[1] * b[0])


def _csq(a):
    t = a[0] * a[1]
    return ((a[0] - a[1]) * (a[0] + a[1]), t + t)


def _dot(a, b):
    return jax.lax.dot_general(a, b, (((1,), (0,)), ((), ())), preferred_element_type=F32)


def _dot_nt(a, b):
    return jax.lax.dot_general(a, b, (((1,), (1,)), ((), ())), preferred_element_type=F32)


def _rbf(x):
    return x.astype(BF16).astype(F32)


def _interleave(*gens):
    state = [[0.0, k, g, total] for k, (g, total) in enumerate(gens)]
    while state:
        cur = min(state, key=lambda e: (e[0], e[1]))
        w = next(cur[2], None)
        if w is None:
            state.remove(cur)
        else:
            cur[0] += w / cur[3]


def _zip(*gens):
    _interleave(*((g, 1.0) for g in gens))


_ZP = (1, 2, 8, 16, 32, 64, 128, 256)
_WP = (0, 4, 8, 1032, 1544)


def _kernel(x_hbm, are_hbm, aim_hbm, bre_hbm, bim_hbm, cre_hbm, cim_hbm, ldt_hbm, dsk_hbm,
            wr_hbm, wg_hbm, wu_hbm, wd_hbm, fu_hbm, fi_hbm, g_hbm, o_hbm,
            ldt_ref, dsk_ref, wr_ref, x_v, prm_v, wg_v, wu_v, wd_v, fu_v, fi_v, g_v, o_v, d_v, h_v, s_v, kc_v, dt_v, d0_v,
            key_v, oh_v, act_v, uy_v, kh_v, p_v, sems, psem, osem, vsem,
            *, GA, GD, NF, GE, KS, CS, UB, debug):
    D, L = x_v.shape
    FF = wg_v.shape[1]
    NB = L // P
    FC = FF // NF
    NA, ND, NE = D // GA, D // GD, D // GE

    def rows_of(i, n, off=0, size=None):
        start = i * n + off
        if not isinstance(start, int):
            start = pl.multiple_of(start, size or n)
        return pl.ds(start, size or n)

    prm_hbm = (are_hbm, aim_hbm, bre_hbm, bim_hbm, cre_hbm, cim_hbm)

    def cprm(part, k):
        r = pl.ds(0, 2 * GA) if part == 0 else pl.ds(2 * GA, D - 2 * GA)
        return pltpu.make_async_copy(prm_hbm[k].at[r], prm_v.at[k, r], psem.at[6 * part + k])

    cx = pltpu.make_async_copy(x_hbm, x_v, sems.at[0])
    cfu = pltpu.make_async_copy(fu_hbm, fu_v, sems.at[1])
    cfi = pltpu.make_async_copy(fi_hbm, fi_v, sems.at[2])
    cg = pltpu.make_async_copy(g_hbm, g_v, sems.at[3])

    def cwg(i):
        return pltpu.make_async_copy(wg_hbm.at[:, rows_of(i, FC)], wg_v.at[:, rows_of(i, FC)], sems.at[4 + i])

    def cwu(i):
        return pltpu.make_async_copy(wu_hbm.at[:, rows_of(i, FC)], wu_v.at[:, rows_of(i, FC)], sems.at[4 + NF + i])

    def cwd(i):
        return pltpu.make_async_copy(wd_hbm.at[rows_of(i, GE)], wd_v.at[rows_of(i, GE)], sems.at[4 + 2 * NF + i])

    def cout(i):
        return pltpu.make_async_copy(o_v.at[rows_of(i, GE)], o_hbm.at[rows_of(i, GE)], osem.at[i])

    cvec = [pltpu.make_async_copy(src, dst, vsem.at[k]) for k, (src, dst) in enumerate(
        ((ldt_hbm, ldt_ref), (dsk_hbm, dsk_ref), (wr_hbm, wr_ref)))]
    for c in cvec:
        c.start()
    for k in range(6):
        cprm(0, k).start()

    @pl.loop(0, NF)
    def _(i):
        cwg(i).start(priority=1)
        cwu(i).start(priority=1)

    @pl.loop(0, NE)
    def _(i):
        cwd(i).start(priority=1)

    cg.start()
    for k in range(6):
        cprm(1, k).start()
    for c in cvec:
        c.wait()

    dt_row = _rbf(jnp.exp(ldt_ref[...].astype(F32)[None, :]))
    dsk_row = dsk_ref[...].astype(F32)[None, :]
    for c0 in range(0, D, GA):
        eye = (jax.lax.broadcasted_iota(jnp.int32, (GA, P), 0) + c0 % P
               == jax.lax.broadcasted_iota(jnp.int32, (GA, P), 1))
        lo = c0 - c0 % P
        n = min(P, D - lo)
        for k, row in enumerate((dt_row, dsk_row)):
            dt_v[k, c0:c0 + GA, :] = _dot(jnp.where(eye[:, :n], row[:, lo:lo + n], 0.0), jnp.ones((n, P), BF16))

    lane8 = jax.lax.broadcasted_iota(jnp.int32, (8, P), 1)
    sub8 = jax.lax.broadcasted_iota(jnp.int32, (8, P), 0)

    def k_setup(src, dst):
        for g in range(GA // 16):
            rows = rows_of(src, GA, 16 * g, 16)
            sl = slice(16 * g, 16 * g + 16)
            dt = dt_v[0, rows, :]
            a_re, a_im, b_re, b_im, c_re, c_im = (prm_v[k, rows, :].astype(F32) for k in range(6))
            w = {0: _cmul((c_re, c_im), (dt * b_re, dt * b_im))}
            d0_v[dst + 1, sl, :] = dt_v[1, rows, :] + jnp.sum(w[0][0], axis=1, keepdims=True)
            mag = jnp.exp(dt * a_re)
            z = {1: (mag * jnp.cos(dt * a_im), mag * jnp.sin(dt * a_im))}
            yield 11
            for e in range(10):
                z[2 << e] = _csq(z[1 << e])
            yield 3
            w[4], w[8] = _cmul(w[0], z[4]), _cmul(w[0], z[8])
            w[1032] = _cmul(w[8], z[1024])
            w[1544] = _cmul(w[1032], z[512])
            for n, v in enumerate([z[e] for e in _ZP] + [w[e] for e in _WP]):
                for q in range(2):
                    p_v[dst, q, n, sl, :] = v[q]
            yield 2

    def k_lags(i):
        low = sub8 < 4
        bit4, bit5, bit6 = ((lane8 & b) == 0 for b in (16, 32, 64))
        bit6x = ((lane8 >> 4) ^ sub8) & 4 == 0
        diag = (lane8 & 15) * 8 + (((lane8 >> 2) & 4) ^ sub8)
        for g in range(GA // 8):
            sl = slice(8 * g, 8 * g + 8)
            out = []
            for h in range(2):
                vals = [tuple(jnp.take_along_axis(p_v[i, q, n, sl, :], (sub8 & 3) + 4 * h, axis=0,
                                                  mode="promise_in_bounds") for q in range(2))
                        for n in range(len(_ZP) + len(_WP))]
                z = dict(zip(_ZP, vals))
                w = dict(zip(_WP, vals[len(_ZP):]))

                def pair(a, b):
                    if h:
                        a, b = b, a
                    return tuple(jnp.where(low, x, y) for x, y in zip(a, b))

                bs = [pair((1.0, 0.0), z[128])]
                for j in range(1, 16):
                    hb = 1 << (j.bit_length() - 1)
                    bs.append(_cmul(bs[j - hb], z[8 * hb]))
                r = pair(w[0], w[4])
                a1, a2, a4 = _cmul(r, z[1]), _cmul(r, z[2]), pair(w[4], w[8])
                av = [a1, a2, _cmul(a2, z[1]), a4, _cmul(a2, z[256]), _cmul(a4, z[256])]
                av.append(_cmul(av[-1], z[256]))
                av.append(_cmul(av[-1], z[256]))
                av.append(pair(w[1032], w[1544]))
                av.append(_cmul(av[-1], z[256]))
                out.append([_dot_nt(jnp.concatenate([v[q] for v in av], axis=0),
                                    jnp.concatenate([v[q] for v in bs], axis=0).astype(BF16))
                            for q in range(2)])
            halves = []
            for lo, hi in ((0, 4), (4, 8), (8, 10)):
                xs = []
                for h in range(2):
                    v = [jnp.take_along_axis(out[h][0][8 * n:8 * n + 8] - out[h][1][8 * n:8 * n + 8], diag,
                                             axis=1, mode="promise_in_bounds") for n in range(lo, hi)]
                    v = [jnp.where(bit5, v[n], v[n + 1]) for n in range(0, len(v), 2)]
                    xs.append(jnp.where(bit6x, v[h], v[1 - h]) if len(v) == 2 else v[0])
                halves.append((jnp.where(low, xs[0], xs[1]), pltpu.roll(jnp.where(low, xs[1], xs[0]), 4, 0)))
            (l1, u1), (l2, u2), (l3, u3) = halves
            tiles = [jnp.where(bit4, l1, u1), jnp.where(bit4, u1, l1), jnp.where(bit6, l2, u2),
                     jnp.where(bit6, u2, l2), jnp.where(bit6, l3, u3)]
            tiles.append(jnp.where(lane8 < 32, tiles[4], tiles[3]))
            for t, tile in enumerate(tiles):
                kc_v[i + 1, t, sl, :] = tile
            yield 8

    def k_window(i, j):
        gi = sum(len(s) for s in _SRC[:j])
        kh = None
        for n, t in enumerate(_SRC[j]):
            part = _dot(kc_v[i, t], pltpu.bitcast(g_v[(gi + n) * 64:(gi + n + 1) * 64, :], BF16))
            kh = part if kh is None else kh + part
        for g in range(GA // 8):
            sl = slice(8 * g, 8 * g + 8)
            a, b = kh[sl, :P], kh[sl, P:]
            if j == 0:
                a = a + d0_v[i, sl, :]
            for q, v in enumerate((a, b, a - b)):
                kh_v[i * (GA // GD) + 8 * g // GD, q, j, 8 * g % GD:8 * g % GD + 8, :] = v
            yield 1

    def k_spectra(i):
        for pair in ((1, 2), (3, 4), (5,), (0, 6), (7, 8), (9, 10), (11, 12), (13, 14), (15,)):
            _zip(*(k_window(i, j) for j in pair))
            yield sum(len(_SRC[j]) for j in pair)

    def k_step(i, _):
        @pl.when(i == 1)
        def _():
            for k in range(6):
                cprm(1, k).wait()

        if KS == 0:
            _interleave((k_spectra(i), 21.0), (k_setup(jnp.minimum(i + 1, NA - 1), i + 1), GA))
            _zip(k_lags(i))
        else:
            _zip(k_lags(i))
            _interleave((k_spectra(i), 21.0 * KS), (k_setup(jnp.minimum(i + 1, NA - 1), i + 1), GA))
        return 0

    with jax.named_scope("kgen"):
        kc_v[0] = jnp.zeros(kc_v.shape[1:], F32)
        d0_v[0] = jnp.zeros(d0_v.shape[1:], F32)
        for k in range(6):
            cprm(0, k).wait()
        _zip(k_setup(0, 0))
        cg.wait()
        cx.start()
        cfu.start()
        cfi.start()
        jax.lax.fori_loop(0, NA, k_step, 0)

    RB = 64

    def col_sum(v):
        return functools.reduce(jnp.add, [v[8 * g:8 * g + 8] for g in range(v.shape[0] // 8)])

    with jax.named_scope("lnorm"):
        cx.wait()
        tot = jax.lax.fori_loop(
            0, D // RB, lambda i, acc: acc + col_sum(x_v[rows_of(i, RB), :].astype(F32)),
            jnp.zeros((8, L), F32))
        m = jnp.sum(tot, axis=0, keepdims=True) / D
        mb = _rbf(m)

        def centre(i, acc):
            d = x_v[rows_of(i, RB), :].astype(F32) - mb
            d_v[rows_of(i, RB), :] = d.astype(BF16)
            return acc + col_sum(d * d)

        tot = jax.lax.fori_loop(0, D // RB, centre, jnp.zeros((8, L), F32))
        var = jnp.maximum(jnp.sum(tot, axis=0, keepdims=True) / D - (m - mb) * (m - mb), 0.0)
        key_v[...] = jnp.broadcast_to(
            0.5 / _rbf(jnp.sqrt(_rbf(_rbf(var) + _rbf(jnp.full_like(var, 1e-5))))), (8, L))
        wr = jnp.broadcast_to(2.0 * wr_ref[...].astype(F32)[None, :], (8, D))
        LB = 4 * P

        def scale(c, _):
            cols = rows_of(c, LB)
            h = (d_v[:, cols].astype(F32) * key_v[0:1, cols]).astype(BF16)
            h_v[:, cols] = h
            oh_v[:, cols] = _dot(wr, h)
            return 0

        jax.lax.fori_loop(0, L // LB, scale, 0)

    def c_signal(src, dst, c0, n):
        lhs = jnp.concatenate([h_v[rows_of(src, GD), c * P:(c + 1) * P] for c in range(c0, c0 + n)], axis=0)
        uh = _dot(lhs, pltpu.bitcast(fu_v[...], BF16))
        for c in range(n):
            for g in range(GD // 8):
                r = slice(c * GD + 8 * g, c * GD + 8 * g + 8)
                a, b = uh[r, :P], uh[r, P:]
                for q, v in enumerate((a, b, a - b)):
                    uy_v[dst, q, c0 + c, 8 * g:8 * g + 8, :] = v
                yield 1

    def c_inverse(i, c0, n):
        lhs = jnp.concatenate([jnp.concatenate([uy_v[i, 3 + q, c] for q in range(2)], axis=1)
                               for c in range(c0, c0 + n)], axis=0)
        y = _dot(lhs, pltpu.bitcast(fi_v[...], BF16))
        for c in range(n):
            for g in range(GD // 8):
                s_v[i, 8 * g:8 * g + 8, (c0 + c) * P:(c0 + c + 1) * P] = y[c * GD + 8 * g:c * GD + 8 * g + 8]
                yield 1

    def c_transforms(i):
        for c0 in range(0, NB, UB):
            _zip(c_signal(jnp.minimum(i + 1, ND - 1), i + 1, c0, UB), c_inverse(i, c0, UB))
            yield UB

    def c_product(i):
        for g in range(GD // 8):
            sl = slice(8 * g, 8 * g + 8)
            for cs in (range(8, 16), range(8)):
                m0 = {}
                for q in range(3):
                    acc = dict(m0)
                    for j in reversed(range(max(cs) + 1)):
                        k = kh_v[i + GA // GD, q, j, sl, :]
                        live = [c for c in cs if c >= j]
                        for c in live:
                            t = k * uy_v[i, q, c - j, sl, :]
                            acc[c] = t if c not in acc else (acc[c] - t if q else acc[c] + t)
                        yield len(live)
                    if q == 0:
                        m0 = acc
                    else:
                        for c in cs:
                            uy_v[i + 1, 2 + q, c, sl, :] = acc[c]

    def c_step(i, _):
        _interleave((c_product(i), GD // 8 * 3 * 136), (c_transforms(i), NB * CS))
        return 0

    with jax.named_scope("topk"):
        cfu.wait()
        cfi.wait()
        r = _rbf(oh_v[...])
        bits = pltpu.bitcast(jnp.where(r == 0.0, 0.0, r), jnp.int32)
        ordered = jnp.where(bits < 0, ~bits, bits ^ jnp.int32(-2**31))
        idx = jax.lax.broadcasted_iota(jnp.int32, (8, L), 1)
        key = pltpu.bitcast((jax.lax.shift_right_logical(ordered, 16) << 11) + (0x20000000 + L - 1 - idx), F32)
        ks = []
        for hf in range(NB // 8):
            kk = key[:, hf * 8 * P:(hf * 8 + 1) * P]
            for q in range(1, 8):
                kk = jnp.where(sub8 == q, key[:, (hf * 8 + q) * P:(hf * 8 + q + 1) * P], kk)
            ks.append(kk)
        top = jnp.zeros((8, P), F32)
        for q in range(8):
            mx = jnp.max(functools.reduce(jnp.maximum, ks), axis=0, keepdims=True)
            mx = jnp.max(mx, axis=1, keepdims=True)
            top = jnp.where(sub8 == q, mx, top)
            ks = [jnp.where(kk == mx, 0.0, kk) for kk in ks]
        _zip(k_spectra(NA))
        _zip(c_signal(0, 0, 0, NB // 2), c_signal(0, 0, NB // 2, NB // 2))
        uy_v[0, 3:5] = jnp.zeros((2,) + uy_v.shape[2:], F32)
        for c in range(NB):
            oh_v[:, c * P:(c + 1) * P] = jnp.where(key[:, c * P:(c + 1) * P] == top, 1.0, 0.0)
        o16 = jax.lax.shift_right_logical(pltpu.bitcast(top, jnp.int32) - 0x20000000, 11) << 16
        r_top = pltpu.bitcast(jnp.where(o16 < 0, o16 ^ jnp.int32(-2**31), (~o16) & jnp.int32(-65536)), F32)
        gate = jax.nn.sigmoid(r_top)
        kc_v[0, 0] = p_v[NA, 0, 0]

    with jax.named_scope("gather"):
        x_sel = 2.0 * jax.lax.fori_loop(
            0, L // LB, lambda c, acc: acc + _dot_nt(oh_v[:, rows_of(c, LB)], h_v[:, rows_of(c, LB)]),
            jnp.zeros((8, D), F32))

    with jax.named_scope("conv"):
        jax.lax.fori_loop(0, ND, c_step, 0)
        _zip(c_inverse(ND, 0, NB // 2), c_inverse(ND, NB // 2, NB // 2))

    def gate_up(i, _):
        cwg(i).wait()
        cwu(i).wait()
        a = 0.5 * _dot(x_sel, wg_v[:, rows_of(i, FC)])
        u = _dot(x_sel, wu_v[:, rows_of(i, FC)])
        act_v[:, rows_of(i, FC)] = (a + a * jnp.tanh(a)) * u
        return 0

    with jax.named_scope("gateup"):
        jax.lax.fori_loop(0, NF, gate_up, 0)

    def down(src):
        return _dot_nt(act_v[...], wd_v[rows_of(src, GE), :]) * (0.5 * gate[:, :GE])

    def final(i, y):
        @pl.when(i + 1 < NE)
        def _():
            cwd(i + 1).wait()

        rows = rows_of(i, GE)
        upd = jax.lax.dot_general(y, oh_v[...], (((0,), (0,)), ((), ())), preferred_element_type=F32)
        h = h_v[rows, :].astype(F32) + upd
        s = jnp.concatenate([s_v[i * (GE // GD) + 1 + n] for n in range(GE // GD)], axis=0)
        q = s * h
        out = (x_v[rows, :].astype(F32) + q) + q * jnp.tanh(h)
        if debug:
            out = s
        o_v[rows, :] = out.astype(o_v.dtype)
        y = down(jnp.minimum(i + 1, NE - 1))
        cout(i).start()
        return y

    with jax.named_scope("final"):
        cwd(0).wait()
        jax.lax.fori_loop(0, NE, final, down(0))
        for i in range(NE):
            cout(i).wait()


def run(A_u, A_A_re, A_A_im, A_B_re, A_B_im, A_C_re, A_C_im, A_log_dt, A_Dskip, B_x, B_w_r,
        B_w_gate, B_w_up, B_w_down, GA=64, GD=32, NF=4, GE=64, KS=1.1, CS=1.12, UB=1,
        debug=False, interpret=False, flags=None):
    _, L, D = A_u.shape
    FF = B_w_gate.shape[1]
    fu, fi, g = _tables()
    odt = F32 if debug else A_u.dtype
    hbm = pl.BlockSpec(memory_space=pl.ANY)
    vm = pl.BlockSpec(memory_space=pltpu.VMEM)
    NB = L // P
    out = pl.pallas_call(
        functools.partial(_kernel, GA=GA, GD=GD, NF=NF, GE=GE, KS=KS, CS=CS, UB=UB, debug=debug),
        out_shape=jax.ShapeDtypeStruct((D, L), odt),
        in_specs=[hbm] * 16,
        out_specs=hbm,
        scratch_shapes=[
            *[pltpu.VMEM((D,), BF16)] * 3,
            pltpu.VMEM((D, L), BF16), pltpu.VMEM((6, D, P), BF16),
            pltpu.VMEM((D, FF), BF16), pltpu.VMEM((D, FF), BF16), pltpu.VMEM((D, FF), BF16),
            pltpu.VMEM(fu.shape, jnp.uint32), pltpu.VMEM(fi.shape, jnp.uint32),
            pltpu.VMEM(g.shape, jnp.uint32),
            pltpu.VMEM((D, L), odt), pltpu.VMEM((D, L), BF16), pltpu.VMEM((D, L), BF16),
            pltpu.VMEM((D // GD + 1, GD, L), F32),
            pltpu.VMEM((D // GA + 1, 6, GA, P), F32), pltpu.VMEM((2, D, P), F32),
            pltpu.VMEM((D // GA + 2, GA, P), F32),
            pltpu.VMEM((8, L), F32), pltpu.VMEM((8, L), F32), pltpu.VMEM((8, FF), F32),
            pltpu.VMEM((D // GD + 1, 5, NB, GD, P), F32),
            pltpu.VMEM(((D + GA) // GD, 3, NB, GD, P), F32),
            pltpu.VMEM((D // GA + 1, 2, len(_ZP) + len(_WP), GA, P), F32),
            pltpu.SemaphoreType.DMA((4 + 2 * NF + D // GE,)),
            pltpu.SemaphoreType.DMA((12,)),
            pltpu.SemaphoreType.DMA((D // GE,)),
            pltpu.SemaphoreType.DMA((3,)),
        ],
        compiler_params=pltpu.CompilerParams(vmem_limit_bytes=112 * 2**20, flags=flags),
        interpret=interpret,
        name="ssm_moe",
    )(A_u[0].T, A_A_re, A_A_im, A_B_re, A_B_im, A_C_re, A_C_im, A_log_dt, A_Dskip, B_w_r,
      B_w_gate, B_w_up, B_w_down.T, fu, fi, g)
    return out.T[None]


@jax.jit
def pallas_recurrent_scan__ssm_conv_s4__moe_arch_mod__prompt_kernel(
    A_u: jax.Array,
    A_A_re: jax.Array,
    A_A_im: jax.Array,
    A_B_re: jax.Array,
    A_B_im: jax.Array,
    A_C_re: jax.Array,
    A_C_im: jax.Array,
    A_log_dt: jax.Array,
    A_Dskip: jax.Array,
    B_x: jax.Array,
    B_w_r: jax.Array,
    B_w_gate: jax.Array,
    B_w_up: jax.Array,
    B_w_down: jax.Array,
):
    return run(A_u, A_A_re, A_A_im, A_B_re, A_B_im, A_C_re, A_C_im, A_log_dt, A_Dskip, B_x,
               B_w_r, B_w_gate, B_w_up, B_w_down)
```

```python
import functools

import jax
import jax.numpy as jnp
import numpy as np
import jax.experimental.pallas as pl
import jax.experimental.pallas.tpu as pltpu

F32 = jnp.float32
BF16 = jnp.bfloat16
P = 128


def _bf16_bits(a):
    u = np.ascontiguousarray(a, dtype=np.float32).view(np.uint32)
    return ((u + 0x7FFF + ((u >> 16) & 1)) >> 16).astype(np.uint32)


def _round_bf16(a):
    return (_bf16_bits(a) << 16).view(np.float32)


def _pack_rows(a):
    b = _bf16_bits(a)
    return (b[0::2] | (b[1::2] << 16)).astype(np.uint32)


def _tile_lags():
    lane = np.arange(P)
    quarter, hb, j = lane // 32, (lane // 16) % 2, lane % 16

    def half(offsets, second):
        q = (quarter + 2 * second) % 4
        return np.array(offsets)[q] + 128 * (hb ^ second) + 8 * j

    l1, u1 = half((1, 2, 3, 4), 0), half((5, 6, 7, 8), 1)
    l2, u2 = half((258, 260, 516, 772), 0), half((262, 264, 520, 776), 1)
    l3, u3 = half((1032, 1288) * 2, 0), half((1544, 1800) * 2, 1)
    lags = [np.where(hb == 0, l1, u1), np.where(hb == 0, u1, l1),
            np.where(lane < 64, l2, u2), np.where(lane < 64, u2, l2), np.where(lane < 64, l3, u3)]
    lags.append(np.where((lane // 16 == 2) | (lane // 16 == 5), np.roll(lags[3], 16), lags[2]))
    lags.append(np.where(lane < 96, lags[3], lags[2]))
    lags.append(np.where(lane < 32, lags[4], lags[3]))
    return lags


_SRC = ((0,), (0, 1), (1, 2), (2,), (5,), (6,), (3,), (3,), (7,), (7,)) + ((4,),) * 6


@functools.cache
def _tables():
    k = np.arange(P)
    phi = 2 * np.pi * (k + 0.25) / P

    def coords(m):
        z = np.exp(1j * np.outer(m, phi))
        return np.concatenate([z.real + z.imag / np.sqrt(3), 2 * z.imag / np.sqrt(3)], axis=1)

    fu = 2.0 * coords(np.arange(P))
    zi = np.exp(-1j * np.outer(phi, np.arange(P)))
    fi = np.concatenate([zi.real, (np.exp(2j * np.pi / 3) * zi).real], axis=0) / P
    lags = _tile_lags()
    groups, layout = [], []
    for j, src in enumerate(_SRC):
        m = np.arange(-P + 1 + (j == 3), P)
        m = m[P * j + m >= 1]
        rl = _round_bf16(P * j + m)
        hit = np.zeros(len(m), int)
        layout.append([])
        for t in src:
            sel = (lags[t][:, None] == rl[None, :])
            hit += sel.sum(0)
            g = _pack_rows(sel.astype(np.float64) @ coords(m))
            ids = []
            for r in range(0, P // 2, 8):
                known = [n for n, e in enumerate(groups) if np.array_equal(e, g[r:r + 8])]
                if not sel[2 * r:2 * r + 16].any():
                    ids.append(None)
                elif known:
                    ids.append(known[0])
                else:
                    ids.append(len(groups))
                    groups.append(g[r:r + 8])
            layout[-1].append(ids)
        assert (hit == 1).all()
    edge = np.broadcast_to(coords(np.array([-P + 1])).astype(np.float32), (8, 2 * P)).view(np.uint32)
    lane256 = int(np.nonzero(lags[1] == 2 * P)[0][0])
    return _pack_rows(fu), _pack_rows(fi), np.stack(groups + [edge]), layout, lane256


def _cmul(a, b):
    return (a[0] * b[0] - a[1] * b[1], a[0] * b[1] + a[1] * b[0])


def _csq(a):
    t = a[0] * a[1]
    return ((a[0] - a[1]) * (a[0] + a[1]), t + t)


def _dot(a, b):
    return jax.lax.dot_general(a, b, (((1,), (0,)), ((), ())), preferred_element_type=F32)


def _dot_nt(a, b):
    return jax.lax.dot_general(a, b, (((1,), (1,)), ((), ())), preferred_element_type=F32)


def _rbf(x):
    return x.astype(BF16).astype(F32)


def _interleave(*gens):
    state = [[0.0, k, g, total] for k, (g, total) in enumerate(gens)]
    while state:
        cur = min(state, key=lambda e: (e[0], e[1]))
        w = next(cur[2], None)
        if w is None:
            state.remove(cur)
        else:
            cur[0] += w / cur[3]


def _zip(*gens):
    _interleave(*((g, 1.0) for g in gens))


_ZP = (1, 8, 32, 256)


def _kernel(x_hbm, are_hbm, aim_hbm, bre_hbm, bim_hbm, cre_hbm, cim_hbm, ldt_hbm, dsk_hbm,
            wr_hbm, wg_hbm, wu_hbm, wd_hbm, fu_hbm, fi_hbm, g_hbm, o_hbm,
            ldt_v, dsk_v, wr_v, x_v, prm_v, wg_v, wu_v, wd_v, fu_v, fi_v, g_v, o_v, d_v, h_v, s_v,
            kc_v, dt_v, row_v, oh_v, act_v, hat_v, p_v, sems, psem, osem,
            *, GS, GA, GD, NG, NF, GE, CS, UB, debug):
    D, L = x_v.shape
    FF = wg_v.shape[1]
    NB = L // P
    FC = FF // NF
    ND, NE = D // GD, D // GE
    layout, lane256 = _tables()[3:]

    def span(i, n):
        start = i * n
        if not isinstance(start, int):
            start = pl.multiple_of(start, n)
        return pl.ds(start, n)

    prm_hbm = (are_hbm, aim_hbm, bre_hbm, bim_hbm, cre_hbm, cim_hbm)

    def cprm(part, k):
        r = pl.ds(0, 3 * GS) if part == 0 else pl.ds(3 * GS, D - 3 * GS)
        return pltpu.make_async_copy(prm_hbm[k].at[r], prm_v.at[k, r], psem.at[6 * part + k])

    cx, cfu, cfi, cg, *cvec = (
        pltpu.make_async_copy(src, dst, sems.at[k]) for k, (src, dst) in enumerate((
            (x_hbm, x_v), (fu_hbm, fu_v), (fi_hbm, fi_v), (g_hbm, g_v),
            (ldt_hbm, ldt_v), (dsk_hbm, dsk_v), (wr_hbm, wr_v))))

    def cwg(i):
        return pltpu.make_async_copy(wg_hbm.at[:, span(i, FC)], wg_v.at[:, span(i, FC)], sems.at[7 + i])

    def cwu(i):
        return pltpu.make_async_copy(wu_hbm.at[:, span(i, FC)], wu_v.at[:, span(i, FC)], sems.at[7 + NF + i])

    def cwd(i):
        return pltpu.make_async_copy(wd_hbm.at[span(i, GE)], wd_v.at[span(i, GE)], sems.at[7 + 2 * NF + i])

    def cout(i):
        return pltpu.make_async_copy(o_v.at[span(i, GE)], o_hbm.at[span(i, GE)], osem.at[i])

    for c in cvec:
        c.start()
    for k in range(6):
        cprm(0, k).start()

    @pl.loop(0, NF)
    def _(i):
        cwg(i).start(priority=1)
        cwu(i).start(priority=1)

    @pl.loop(0, NE)
    def _(i):
        cwd(i).start(priority=1)

    for k in range(6):
        cprm(1, k).start()
    for c in cvec:
        c.wait()

    dt_row = _rbf(jnp.exp(ldt_v[...].astype(F32)[None, :]))
    dsk_row = dsk_v[...].astype(F32)[None, :] * (1.0 / P)
    for c0 in range(0, D, P):
        n = min(P, D - c0)
        eye = (jax.lax.broadcasted_iota(jnp.int32, (n, n), 0) == jax.lax.broadcasted_iota(jnp.int32, (n, n), 1))
        for k, row in enumerate((dt_row, dsk_row)):
            dt_v[k, c0:c0 + n, :] = _dot(jnp.where(eye, row[:, c0:c0 + n], 0.0), jnp.ones((n, P), BF16))

    lane8 = jax.lax.broadcasted_iota(jnp.int32, (8, P), 1)
    sub8 = jax.lax.broadcasted_iota(jnp.int32, (8, P), 0)

    def k_setup(i, _):
        @pl.when(i == 3)
        def _():
            for k in range(6):
                cprm(1, k).wait()

        low = sub8 < 4
        for g in range(GS // 16):
            sl = slice(16 * g, 16 * g + 16)
            dt, dsk = (dt_v.at[k, span(i, GS)][sl, :] for k in range(2))
            a_re, a_im, b_re, b_im, c_re, c_im = (prm_v.at[k, span(i, GS)][sl, :].astype(F32) for k in range(6))
            dst = p_v.at[:, span(i, GS)]
            w = {0: _cmul((c_re, c_im), (dt * b_re, dt * b_im))}
            dst[24, sl, :] = w[0][0] + dsk
            mag = jnp.exp(dt * a_re)
            z = {1: (mag * jnp.cos(dt * a_im), mag * jnp.sin(dt * a_im))}
            for e in range(10):
                z[2 << e] = _csq(z[1 << e])
            for n, e in enumerate(_ZP):
                for q in range(2):
                    dst[2 * n + q, sl, :] = z[e][q]
            w[4], w[8] = _cmul(w[0], z[4]), _cmul(w[0], z[8])
            w[1032] = _cmul(w[8], z[1024])
            w[1544] = _cmul(w[1032], z[512])
            one = (jnp.ones((16, P), F32), jnp.zeros((16, P), F32))
            for n, (a, b) in enumerate(((one, z[128]), (w[0], w[4]), (w[4], w[8]), (w[1032], w[1544]))):
                for q in range(2):
                    for t in range(2):
                        x, y = a[q][8 * t:8 * t + 8], pltpu.roll(b[q][8 * t:8 * t + 8], 4, 0)
                        r = slice(16 * g + 8 * t, 16 * g + 8 * t + 8)
                        dst[8 + 4 * n + q, r, :] = jnp.where(low, x, y)
                        dst[10 + 4 * n + q, r, :] = jnp.where(low, y, x)
        return 0

    def k_lags(i, _):
        low = sub8 < 4
        bit4, bit5, bit6 = ((lane8 & b) == 0 for b in (16, 32, 64))
        bit6x = ((lane8 >> 4) ^ sub8) & 4 == 0
        diag = (lane8 & 15) * 8 + (((lane8 >> 2) & 4) ^ sub8)
        src, dst = p_v.at[:, span(i, GA)], kc_v.at[:, span(i, GA)]
        for g in range(GA // 8):
            sl = slice(8 * g, 8 * g + 8)
            out = []
            for h in range(2):
                off = (4 if h else 0) if g + 1 < GA // 8 else (0 if h else -4)
                z = {e: tuple(jnp.take_along_axis(src[2 * n + q, 8 * g + off:8 * g + off + 8, :],
                                                  (sub8 & 3) + (4 * h - off), axis=0,
                                                  mode="promise_in_bounds") for q in range(2))
                     for n, e in enumerate(_ZP)}
                b0, r, a4, far = (tuple(src[8 + 4 * n + 2 * h + q, sl, :] for q in range(2)) for n in range(4))
                bs = [b0]
                for j in range(1, 16):
                    bs.append(_cmul(bs[j - 1], z[8]) if j < 4 else _cmul(bs[j - 4], z[32]))
                av = [_cmul(r, z[1])]
                av += [_cmul(av[0], z[1])]
                av += [_cmul(av[1], z[1]), a4, _cmul(av[1], z[256]), _cmul(a4, z[256])]
                av.append(_cmul(av[-1], z[256]))
                av.append(_cmul(av[-1], z[256]))
                av += [far, _cmul(far, z[256])]
                out.append([_dot_nt(jnp.concatenate([v[q] for v in av], axis=0),
                                    jnp.concatenate([v[q] for v in reversed(bs)], axis=0).astype(BF16))
                            for q in range(2)])
            v = [[None] * 10, [None] * 10]
            for n in range(10):
                for h in range(2):
                    v[h][n] = jnp.take_along_axis(out[h][0][8 * n:8 * n + 8] - out[h][1][8 * n:8 * n + 8],
                                                  diag ^ 120, axis=1, mode="promise_in_bounds")
            halves = []
            for lo, hi in ((0, 4), (4, 8), (8, 10)):
                xs = []
                for h in range(2):
                    u = [jnp.where(bit5, v[h][n], v[h][n + 1]) for n in range(lo, hi, 2)]
                    xs.append(jnp.where(bit6x, u[h], u[1 - h]) if len(u) == 2 else u[0])
                halves.append((jnp.where(low, xs[0], xs[1]), pltpu.roll(jnp.where(low, xs[1], xs[0]), 4, 0)))
            (l1, u1), (l2, u2), (l3, u3) = halves
            tiles = [jnp.where(bit4, l1, u1), jnp.where(bit4, u1, l1), jnp.where(bit6, l2, u2),
                     jnp.where(bit6, u2, l2), jnp.where(bit6, l3, u3)]
            tiles.append(jnp.where(((lane8 >> 4) == 2) | ((lane8 >> 4) == 5), pltpu.roll(tiles[3], 16, 1), tiles[2]))
            tiles.append(jnp.where(lane8 < 96, tiles[3], tiles[2]))
            tiles.append(jnp.where(lane8 < 32, tiles[4], tiles[3]))
            for u in (src[24, sl, :], jnp.where(lane8 == lane256, tiles[1], 0.0)):
                tiles.append(jnp.broadcast_to(jnp.sum(u, axis=1, keepdims=True), (8, P)))
            for t, tile in enumerate(tiles):
                dst[t, sl, :] = tile
        return 0

    with jax.named_scope("setup"):
        for k in range(6):
            cprm(0, k).wait()
        for c in (cx, cg, cfu, cfi):
            c.start()
        jax.lax.fori_loop(0, D // GS, k_setup, 0)
    with jax.named_scope("lags"):
        jax.lax.fori_loop(0, D // GA, k_lags, 0)

    LB = 2 * P

    def col_sum(parts):
        acc = [functools.reduce(jnp.add, parts[k::4]) for k in range(4)]
        return (acc[0] + acc[1]) + (acc[2] + acc[3])

    def ln_sum(c, _):
        src = x_v.at[:, span(c, LB)]
        row_v[0, :, span(c, LB)] = col_sum([src[r:r + 8, :].astype(F32) for r in range(0, D, 8)])
        return 0

    def ln_centre(c, _):
        src, dst = x_v.at[:, span(c, LB)], d_v.at[:, span(c, LB)]
        mb = row_v[0, :, span(c, LB)]
        acc = [0.0] * 4
        for r in range(0, D, 8):
            d = src[r:r + 8, :].astype(F32) - mb
            dst[r:r + 8, :] = d.astype(BF16)
            acc[r // 8 % 4] += d * d
        row_v[1, :, span(c, LB)] = col_sum(acc)
        return 0

    def ln_scale(c, _):
        src, dst = d_v.at[:, span(c, LB)], h_v.at[:, span(c, LB)]
        inv = row_v[0, :, span(c, LB)]
        for r in range(0, D, 8):
            dst[r:r + 8, :] = (src[r:r + 8, :].astype(F32) * inv).astype(BF16)
        return 0

    def compact(v):
        return jnp.concatenate([functools.reduce(
            lambda a, q: jnp.where(sub8 == q, v[:, (c + q) * P:(c + q + 1) * P], a),
            range(1, 8), v[:, c * P:(c + 1) * P]) for c in range(0, NB, 8)], axis=0)

    def spread(v):
        return jnp.concatenate([jnp.broadcast_to(v[c:c + 1], (8, P)) for c in range(NB)], axis=1)

    def total(k):
        return compact(jnp.broadcast_to(jnp.sum(row_v[k], axis=0, keepdims=True), (8, L)))

    with jax.named_scope("lnorm"):
        cx.wait()
        jax.lax.fori_loop(0, L // LB, ln_sum, 0)
        m = total(0) / D
        mb = _rbf(m)
        row_v[0] = spread(mb)
        jax.lax.fori_loop(0, L // LB, ln_centre, 0)
        var = jnp.maximum(total(1) / D - (m - mb) * (m - mb), 0.0)
        row_v[0] = spread(0.5 / _rbf(jnp.sqrt(_rbf(_rbf(var) + _rbf(jnp.full_like(var, 1e-5))))))
        jax.lax.fori_loop(0, L // LB, ln_scale, 0)

    def put(dst, kind, c, g, a, b):
        for q, v in enumerate((a, b, a - b)):
            hat_v[dst, 3 * kind + q, c, 8 * g:8 * g + 8, :] = v

    def c_signal(src, dst, c0, n):
        lhs = jnp.concatenate([h_v[span(src, GD), c * P:(c + 1) * P] for c in range(c0, c0 + n)], axis=0)
        uh = _dot(lhs, pltpu.bitcast(fu_v[...], BF16))
        for c in range(n):
            for g in range(GD // 8):
                r = slice(c * GD + 8 * g, c * GD + 8 * g + 8)
                put(dst, 0, c0 + c, g, uh[r, :P], uh[r, P:])
                yield 1

    def c_window(src, dst, j):
        tiles = kc_v.at[:, span(src, GD)]
        kh = None
        for t, ids in zip(_SRC[j], layout[j]):
            rhs = jnp.concatenate([jnp.zeros((8, 2 * P), jnp.uint32) if n is None else g_v[n] for n in ids], axis=0)
            part = _dot(tiles[t], pltpu.bitcast(rhs, BF16))
            kh = part if kh is None else kh + part
        for g in range(GD // 8):
            sl = slice(8 * g, 8 * g + 8)
            a, b = kh[sl, :P], kh[sl, P:]
            if j == 0:
                a = a + tiles[8, sl, :]
            if j == 3:
                edge = pltpu.bitcast(g_v[g_v.shape[0] - 1], F32)
                a, b = a + tiles[9, sl, :] * edge[:, :P], b + tiles[9, sl, :] * edge[:, P:]
            put(dst, 1, j, g, a, b)
            yield 1

    def c_inverse(i, c0, n):
        lhs = jnp.concatenate([jnp.concatenate([hat_v[i, 6 + q, c] for q in range(2)], axis=1)
                               for c in range(c0, c0 + n)], axis=0)
        y = _dot(lhs, pltpu.bitcast(fi_v[...], BF16))
        for c in range(n):
            for g in range(GD // 8):
                s_v[i, 8 * g:8 * g + 8, (c0 + c) * P:(c0 + c + 1) * P] = y[c * GD + 8 * g:c * GD + 8 * g + 8]
                yield 1

    window_pairs = ((14, 15), (12, 13), (10, 11), (8, 9), (6, 7), (4, 5), (0, 3), (1, 2))

    def c_transforms(i):
        nxt = jnp.minimum(i + 1, ND - 1)
        for c0 in range(0, NB, UB):
            _zip(c_signal(nxt, i + 1, c0, UB), c_inverse(i, c0, UB))
            yield UB
            for pair in window_pairs[c0 // 2:(c0 + UB) // 2]:
                _zip(*(c_window(nxt, i + 1, j) for j in pair))
                yield len(_SRC[pair[0]])

    def c_product(i):
        for g in range(GD // 8):
            sl = slice(8 * g, 8 * g + 8)
            for cs in (range(8, 16), range(8)):
                m0 = {}
                for q in range(3):
                    acc = dict(m0)
                    for j in reversed(range(max(cs) + 1)):
                        k = hat_v[i, 3 + q, j, sl, :]
                        live = [c for c in cs if c >= j]
                        for c in live:
                            t = k * hat_v[i, q, c - j, sl, :]
                            acc[c] = t if c not in acc else (acc[c] - t if q else acc[c] + t)
                        yield len(live)
                    if q == 0:
                        m0 = acc
                    else:
                        for c in cs:
                            hat_v[i + 1, 5 + q, c, sl, :] = acc[c]

    def c_step(i, pace, *extra):
        _interleave((c_product(i), GD // 8 * 3 * 136), (c_transforms(i), 25 * pace), *extra)

    with jax.named_scope("topk"):
        for c in (cg, cfu, cfi):
            c.wait()
        wr = jnp.broadcast_to(2.0 * wr_v[...].astype(F32)[None, :], (8, D))
        r = _rbf(compact(_dot(wr, h_v[...])))
        bits = pltpu.bitcast(jnp.where(r == 0.0, 0.0, r), jnp.int32)
        ordered = jnp.where(bits < 0, ~bits, bits ^ jnp.int32(-2**31))
        idx = (jax.lax.broadcasted_iota(jnp.int32, (NB, P), 0) * P
               + jax.lax.broadcasted_iota(jnp.int32, (NB, P), 1))
        key = pltpu.bitcast((jax.lax.shift_right_logical(ordered, 16) << 11) + (0x20000000 + L - 1 - idx), F32)
        rest, top = key, jnp.zeros((8, P), F32)
        for q in range(8):
            mx = jnp.max(jnp.max(rest, axis=0, keepdims=True), axis=1, keepdims=True)
            top = jnp.where(sub8 == q, mx, top)
            rest = jnp.where(rest == mx, 0.0, rest)
        _zip(c_signal(0, 0, 0, NB // 2), c_signal(0, 0, NB // 2, NB // 2))
        for pair in window_pairs:
            _zip(*(c_window(0, 0, j) for j in pair))
        hat_v[0, 6:8] = jnp.zeros((2,) + hat_v.shape[2:], F32)
        oh_v[...] = jnp.where(spread(key) == jnp.concatenate([top] * NB, axis=1), 1.0, 0.0)
        o16 = jax.lax.shift_right_logical(pltpu.bitcast(top, jnp.int32) - 0x20000000, 11) << 16
        r_top = pltpu.bitcast(jnp.where(o16 < 0, o16 ^ jnp.int32(-2**31), (~o16) & jnp.int32(-65536)), F32)
        gate = 0.5 * jax.nn.sigmoid(r_top)

    def gather_step(i, acc):
        n = L // NG
        oh, h = oh_v.at[:, span(i, n)], h_v.at[:, span(i, n)]
        parts = []

        def gather():
            for r in range(0, D, P):
                yield 0.5
                parts.append(functools.reduce(jnp.add, [
                    _dot_nt(oh[:, c:c + P], h[r:min(r + P, D), c:c + P]) for c in range(0, n, P)]))
                yield 0.5

        c_step(i, CS[0], (gather(), 5 * CS[0]))
        return acc + jnp.concatenate(parts, axis=1)

    with jax.named_scope("conv0"):
        x_sel = 2.0 * jax.lax.fori_loop(0, NG, gather_step, jnp.zeros((8, D), F32))
        row_v[0, :, :D] = x_sel

    def gate_up_step(i, _):
        cwg(i).wait()
        cwu(i).wait()
        ws, dst = (wg_v.at[:, span(i, FC)], wu_v.at[:, span(i, FC)]), act_v.at[:, :, span(i, FC)]

        def gate_up():
            for c in range(0, FC, 2 * P):
                acc = [0.0, 0.0]
                for r in range(0, D, P):
                    yield 0.5
                    rs = slice(r, min(r + P, D))
                    acc = [a + _dot(row_v[0, :, rs], w[rs, c:c + 2 * P]) for a, w in zip(acc, ws)]
                    yield 0.5
                for k in range(2):
                    dst[k, :, c:c + 2 * P] = acc[k]

        c_step(i + NG, CS[1], (gate_up(), FC // (2 * P) * 5 * CS[1]))
        return 0

    with jax.named_scope("conv1"):
        jax.lax.fori_loop(0, NF, gate_up_step, 0)
        a = 0.5 * act_v[0]
        act_v[0] = (a + a * jnp.tanh(a)) * act_v[1]

    eye = (jax.lax.broadcasted_iota(jnp.int32, (GE, GE), 0)
           == jax.lax.broadcasted_iota(jnp.int32, (GE, GE), 1)).astype(F32)

    def finish(e, lead):
        w = wd_v.at[span(e, GE)]
        acc = 0.0
        for c in range(0, FF, 4 * P):
            yield 0.5
            acc = acc + functools.reduce(jnp.add, [
                _dot_nt(act_v[0, :, f:f + P], w[:, f:f + P]) for f in range(c, c + 4 * P, P)])
            yield 0.5
        yield lead
        yt = _dot_nt(eye, acc * gate[:, :GE])
        yield lead
        h = h_v[span(e, GE), :].astype(F32) + _dot(yt, oh_v[...])
        s = jnp.concatenate([s_v[e * (GE // GD) + 1 + n] for n in range(GE // GD)], axis=0)
        q = s * h
        out = (x_v[span(e, GE), :].astype(F32) + q) + q * jnp.tanh(h)
        if debug:
            out = s
        o_v[span(e, GE), :] = out.astype(o_v.dtype)

    def finish_step(e, _):
        cwd(e).wait()
        c_step(e + NG + NF, CS[2], (finish(e, 3.0), (FF // (4 * P) + 6.0) * CS[2]))
        cout(e).start()
        return 0

    with jax.named_scope("conv2"):
        jax.lax.fori_loop(0, ND - NG - NF, finish_step, 0)

    with jax.named_scope("tail"):
        _zip(c_inverse(ND, 0, NB // 2), c_inverse(ND, NB // 2, NB // 2))
        row_v[1, :, :P] = functools.reduce(jnp.add, [hat_v[i, q, NB - 1, GD - 8:, :] for i in (ND,) for q in range(6)])
        for e in range(ND - NG - NF, NE):
            cwd(e).wait()
            _zip(finish(e, 0.0))
            cout(e).start()
        for e in range(NE):
            cout(e).wait()


def run(A_u, A_A_re, A_A_im, A_B_re, A_B_im, A_C_re, A_C_im, A_log_dt, A_Dskip, B_x, B_w_r,
        B_w_gate, B_w_up, B_w_down, GS=64, GA=96, GD=32, NG=4, NF=6, GE=64, CS=(1.12, 1.12, 1.0), UB=2,
        debug=False, interpret=False, flags=None):
    _, L, D = A_u.shape
    FF = B_w_gate.shape[1]
    fu, fi, g = _tables()[:3]
    odt = F32 if debug else A_u.dtype
    hbm = pl.BlockSpec(memory_space=pl.ANY)
    NB = L // P
    out = pl.pallas_call(
        functools.partial(_kernel, GS=GS, GA=GA, GD=GD, NG=NG, NF=NF, GE=GE, CS=CS, UB=UB, debug=debug),
        out_shape=jax.ShapeDtypeStruct((D, L), odt),
        in_specs=[hbm] * 16,
        out_specs=hbm,
        scratch_shapes=[
            *[pltpu.VMEM((D,), BF16)] * 3,
            pltpu.VMEM((D, L), BF16), pltpu.VMEM((6, D, P), BF16),
            pltpu.VMEM((D, FF), BF16), pltpu.VMEM((D, FF), BF16), pltpu.VMEM((D, FF), BF16),
            pltpu.VMEM(fu.shape, jnp.uint32), pltpu.VMEM(fi.shape, jnp.uint32),
            pltpu.VMEM(g.shape, jnp.uint32),
            pltpu.VMEM((D, L), odt), pltpu.VMEM((D, L), BF16), pltpu.VMEM((D, L), BF16),
            pltpu.VMEM((D // GD + 1, GD, L), F32),
            pltpu.VMEM((10, D, P), F32), pltpu.VMEM((2, D, P), F32),
            pltpu.VMEM((2, 8, L), F32), pltpu.VMEM((8, L), F32), pltpu.VMEM((2, 8, FF), F32),
            pltpu.VMEM((D // GD + 1, 8, NB, GD, P), F32),
            pltpu.VMEM((25, D, P), F32),
            pltpu.SemaphoreType.DMA((7 + 2 * NF + D // GE,)),
            pltpu.SemaphoreType.DMA((12,)),
            pltpu.SemaphoreType.DMA((D // GE,)),
        ],
        compiler_params=pltpu.CompilerParams(vmem_limit_bytes=112 * 2**20, flags=flags),
        interpret=interpret,
        name="ssm_moe",
    )(A_u[0].T, A_A_re, A_A_im, A_B_re, A_B_im, A_C_re, A_C_im, A_log_dt, A_Dskip, B_w_r,
      B_w_gate, B_w_up, B_w_down.T, fu, fi, g)
    return out.T[None]


@jax.jit
def pallas_recurrent_scan__ssm_conv_s4__moe_arch_mod__prompt_kernel(
    A_u: jax.Array,
    A_A_re: jax.Array,
    A_A_im: jax.Array,
    A_B_re: jax.Array,
    A_B_im: jax.Array,
    A_C_re: jax.Array,
    A_C_im: jax.Array,
    A_log_dt: jax.Array,
    A_Dskip: jax.Array,
    B_x: jax.Array,
    B_w_r: jax.Array,
    B_w_gate: jax.Array,
    B_w_up: jax.Array,
    B_w_down: jax.Array,
):
    return run(A_u, A_A_re, A_A_im, A_B_re, A_B_im, A_C_re, A_C_im, A_log_dt, A_Dskip, B_x,
               B_w_r, B_w_gate, B_w_up, B_w_down)
```

```python
import functools

import jax
import jax.numpy as jnp
import numpy as np
import jax.experimental.pallas as pl
import jax.experimental.pallas.tpu as pltpu

F32 = jnp.float32
BF16 = jnp.bfloat16
P = 128


def _bf16_bits(a):
    u = np.ascontiguousarray(a, dtype=np.float32).view(np.uint32)
    return ((u + 0x7FFF + ((u >> 16) & 1)) >> 16).astype(np.uint32)


def _round_bf16(a):
    return (_bf16_bits(a) << 16).view(np.float32)


def _pack_rows(a):
    b = _bf16_bits(a)
    return (b[0::2] | (b[1::2] << 16)).astype(np.uint32)


def _tile_lags():
    lane = np.arange(P)
    quarter, hb, j = lane // 32, (lane // 16) % 2, lane % 16

    def half(offsets, second):
        q = (quarter + 2 * second) % 4
        return np.array(offsets)[q] + 128 * (hb ^ second) + 8 * j

    l1, u1 = half((1, 2, 3, 4), 0), half((5, 6, 7, 8), 1)
    l2, u2 = half((258, 260, 516, 772), 0), half((262, 264, 520, 776), 1)
    l3, u3 = half((1032, 1288) * 2, 0), half((1544, 1800) * 2, 1)
    lags = [np.where(hb == 0, l1, u1), np.where(hb == 0, u1, l1),
            np.where(lane < 64, l2, u2), np.where(lane < 64, u2, l2), np.where(lane < 64, l3, u3)]
    lags.append(np.where((lane // 16 == 2) | (lane // 16 == 5), np.roll(lags[3], 16), lags[2]))
    lags.append(np.where(lane < 96, lags[3], lags[2]))
    lags.append(np.where(lane < 32, lags[4], lags[3]))
    return lags


_SRC = ((0,), (0, 1), (1, 2), (2,), (5,), (6,), (3,), (3,), (7,), (7,)) + ((4,),) * 6


@functools.cache
def _tables():
    k = np.arange(P)
    phi = 2 * np.pi * (k + 0.25) / P

    def coords(m):
        z = np.exp(1j * np.outer(m, phi))
        return np.concatenate([z.real + z.imag / np.sqrt(3), 2 * z.imag / np.sqrt(3)], axis=1)

    fu = 2.0 * coords(np.arange(P))
    zi = np.exp(-1j * np.outer(phi, np.arange(P)))
    fi = np.concatenate([zi.real, (np.exp(2j * np.pi / 3) * zi).real], axis=0) / P
    lags = _tile_lags()
    groups, layout = [], []
    for j, src in enumerate(_SRC):
        m = np.arange(-P + 1 + (j == 3), P)
        m = m[P * j + m >= 1]
        rl = _round_bf16(P * j + m)
        hit = np.zeros(len(m), int)
        layout.append([])
        for t in src:
            sel = (lags[t][:, None] == rl[None, :])
            hit += sel.sum(0)
            g = _pack_rows(sel.astype(np.float64) @ coords(m))
            ids = []
            for r in range(0, P // 2, 8):
                known = [n for n, e in enumerate(groups) if np.array_equal(e, g[r:r + 8])]
                if not sel[2 * r:2 * r + 16].any():
                    ids.append(None)
                elif known:
                    ids.append(known[0])
                else:
                    ids.append(len(groups))
                    groups.append(g[r:r + 8])
            layout[-1].append(ids)
        assert (hit == 1).all()
    edge = np.broadcast_to(coords(np.array([-P + 1])).astype(np.float32), (8, 2 * P)).view(np.uint32)
    lane256 = int(np.nonzero(lags[1] == 2 * P)[0][0])
    return _pack_rows(fu), _pack_rows(fi), np.stack(groups + [edge]), layout, lane256


def _cmul(a, b):
    return (a[0] * b[0] - a[1] * b[1], a[0] * b[1] + a[1] * b[0])


def _csq(a):
    t = a[0] * a[1]
    return ((a[0] - a[1]) * (a[0] + a[1]), t + t)


def _dot(a, b):
    return jax.lax.dot_general(a, b, (((1,), (0,)), ((), ())), preferred_element_type=F32)


def _dot_nt(a, b):
    return jax.lax.dot_general(a, b, (((1,), (1,)), ((), ())), preferred_element_type=F32)


def _rbf(x):
    return x.astype(BF16).astype(F32)


def _interleave(*gens):
    state = [[0.0, k, g, total] for k, (g, total) in enumerate(gens)]
    while state:
        cur = min(state, key=lambda e: (e[0], e[1]))
        w = next(cur[2], None)
        if w is None:
            state.remove(cur)
        else:
            cur[0] += w / cur[3]


def _zip(*gens):
    _interleave(*((g, 1.0) for g in gens))


_ZP = (1, 8, 32, 256)


def _kernel(x_hbm, are_hbm, aim_hbm, bre_hbm, bim_hbm, cre_hbm, cim_hbm, ldt_hbm, dsk_hbm,
            wr_hbm, wg_hbm, wu_hbm, wd_hbm, fu_hbm, fi_hbm, g_hbm, o_hbm,
            ldt_v, dsk_v, wr_v, x_v, prm_v, wg_v, wu_v, wd_v, fu_v, fi_v, g_v, o_v, d_v, h_v, s_v,
            kc_v, dt_v, row_v, oh_v, act_v, hat_v, p_v, sems, psem, osem,
            *, GS, GA, GD, NG, NF, GE, CS, UB, debug):
    D, L = x_v.shape
    FF = wg_v.shape[1]
    NB = L // P
    FC = FF // NF
    ND, NE = D // GD, D // GE
    layout, lane256 = _tables()[3:]

    def span(i, n):
        start = i * n
        if not isinstance(start, int):
            start = pl.multiple_of(start, n)
        return pl.ds(start, n)

    prm_hbm = (are_hbm, aim_hbm, bre_hbm, bim_hbm, cre_hbm, cim_hbm)

    def cprm(part, k):
        r = pl.ds(0, 3 * GS) if part == 0 else pl.ds(3 * GS, D - 3 * GS)
        return pltpu.make_async_copy(prm_hbm[k].at[r], prm_v.at[k, r], psem.at[6 * part + k])

    cx, cfu, cfi, cg, *cvec = (
        pltpu.make_async_copy(src, dst, sems.at[k]) for k, (src, dst) in enumerate((
            (x_hbm, x_v), (fu_hbm, fu_v), (fi_hbm, fi_v), (g_hbm, g_v),
            (ldt_hbm, ldt_v), (dsk_hbm, dsk_v), (wr_hbm, wr_v))))

    def cwg(i):
        return pltpu.make_async_copy(wg_hbm.at[:, span(i, FC)], wg_v.at[:, span(i, FC)], sems.at[7 + i])

    def cwu(i):
        return pltpu.make_async_copy(wu_hbm.at[:, span(i, FC)], wu_v.at[:, span(i, FC)], sems.at[7 + NF + i])

    def cwd(i):
        return pltpu.make_async_copy(wd_hbm.at[span(i, GE)], wd_v.at[span(i, GE)], sems.at[7 + 2 * NF + i])

    def cout(i):
        return pltpu.make_async_copy(o_v.at[span(i, GE)], o_hbm.at[span(i, GE)], osem.at[i])

    for c in cvec:
        c.start()
    for k in range(6):
        cprm(0, k).start()

    @pl.loop(0, NF)
    def _(i):
        cwg(i).start(priority=1)
        cwu(i).start(priority=1)

    @pl.loop(0, NE)
    def _(i):
        cwd(i).start(priority=1)

    for k in range(6):
        cprm(1, k).start()
    for c in cvec:
        c.wait()

    dt_row = _rbf(jnp.exp(ldt_v[...].astype(F32)[None, :]))
    dsk_row = dsk_v[...].astype(F32)[None, :] * (1.0 / P)
    for c0 in range(0, D, P):
        n = min(P, D - c0)
        eye = (jax.lax.broadcasted_iota(jnp.int32, (n, n), 0) == jax.lax.broadcasted_iota(jnp.int32, (n, n), 1))
        for k, row in enumerate((dt_row, dsk_row)):
            dt_v[k, c0:c0 + n, :] = _dot(jnp.where(eye, row[:, c0:c0 + n], 0.0), jnp.ones((n, P), BF16))

    lane8 = jax.lax.broadcasted_iota(jnp.int32, (8, P), 1)
    sub8 = jax.lax.broadcasted_iota(jnp.int32, (8, P), 0)

    def k_setup(i, _):
        @pl.when(i == 3)
        def _():
            for k in range(6):
                cprm(1, k).wait()

        low = sub8 < 4
        for g in range(GS // 16):
            sl = slice(16 * g, 16 * g + 16)
            dt, dsk = (dt_v.at[k, span(i, GS)][sl, :] for k in range(2))
            a_re, a_im, b_re, b_im, c_re, c_im = (prm_v.at[k, span(i, GS)][sl, :].astype(F32) for k in range(6))
            dst = p_v.at[:, span(i, GS)]
            w = {0: _cmul((c_re, c_im), (dt * b_re, dt * b_im))}
            dst[24, sl, :] = w[0][0] + dsk
            mag = jnp.exp(dt * a_re)
            z = {1: (mag * jnp.cos(dt * a_im), mag * jnp.sin(dt * a_im))}
            for e in range(10):
                z[2 << e] = _csq(z[1 << e])
            for n, e in enumerate(_ZP):
                for q in range(2):
                    dst[2 * n + q, sl, :] = z[e][q]
            w[4], w[8] = _cmul(w[0], z[4]), _cmul(w[0], z[8])
            w[1032] = _cmul(w[8], z[1024])
            w[1544] = _cmul(w[1032], z[512])
            one = (jnp.ones((16, P), F32), jnp.zeros((16, P), F32))
            for n, (a, b) in enumerate(((one, z[128]), (w[0], w[4]), (w[4], w[8]), (w[1032], w[1544]))):
                for q in range(2):
                    for t in range(2):
                        x, y = a[q][8 * t:8 * t + 8], pltpu.roll(b[q][8 * t:8 * t + 8], 4, 0)
                        r = slice(16 * g + 8 * t, 16 * g + 8 * t + 8)
                        dst[8 + 4 * n + q, r, :] = jnp.where(low, x, y)
                        dst[10 + 4 * n + q, r, :] = jnp.where(low, y, x)
        return 0

    def k_lags(i, _):
        low = sub8 < 4
        bit4, bit5, bit6 = ((lane8 & b) == 0 for b in (16, 32, 64))
        bit6x = ((lane8 >> 4) ^ sub8) & 4 == 0
        diag = (lane8 & 15) * 8 + (((lane8 >> 2) & 4) ^ sub8)
        src, dst = p_v.at[:, span(i, GA)], kc_v.at[:, span(i, GA)]
        for g in range(GA // 8):
            sl = slice(8 * g, 8 * g + 8)
            out = []
            for h in range(2):
                off = (4 if h else 0) if g + 1 < GA // 8 else (0 if h else -4)
                z = {e: tuple(jnp.take_along_axis(src[2 * n + q, 8 * g + off:8 * g + off + 8, :],
                                                  (sub8 & 3) + (4 * h - off), axis=0,
                                                  mode="promise_in_bounds") for q in range(2))
                     for n, e in enumerate(_ZP)}
                b0, r, a4, far = (tuple(src[8 + 4 * n + 2 * h + q, sl, :] for q in range(2)) for n in range(4))
                bs = [b0]
                for j in range(1, 16):
                    bs.append(_cmul(bs[j - 1], z[8]) if j < 4 else _cmul(bs[j - 4], z[32]))
                av = [_cmul(r, z[1])]
                av += [_cmul(av[0], z[1])]
                av += [_cmul(av[1], z[1]), a4, _cmul(av[1], z[256]), _cmul(a4, z[256])]
                av.append(_cmul(av[-1], z[256]))
                av.append(_cmul(av[-1], z[256]))
                av += [far, _cmul(far, z[256])]
                out.append([_dot_nt(jnp.concatenate([v[q] for v in av], axis=0),
                                    jnp.concatenate([v[q] for v in reversed(bs)], axis=0).astype(BF16))
                            for q in range(2)])
            v = [[None] * 10, [None] * 10]
            for n in range(10):
                for h in range(2):
                    v[h][n] = jnp.take_along_axis(out[h][0][8 * n:8 * n + 8] - out[h][1][8 * n:8 * n + 8],
                                                  diag ^ 120, axis=1, mode="promise_in_bounds")
            halves = []
            for lo, hi in ((0, 4), (4, 8), (8, 10)):
                xs = []
                for h in range(2):
                    u = [jnp.where(bit5, v[h][n], v[h][n + 1]) for n in range(lo, hi, 2)]
                    xs.append(jnp.where(bit6x, u[h], u[1 - h]) if len(u) == 2 else u[0])
                halves.append((jnp.where(low, xs[0], xs[1]), pltpu.roll(jnp.where(low, xs[1], xs[0]), 4, 0)))
            (l1, u1), (l2, u2), (l3, u3) = halves
            tiles = [jnp.where(bit4, l1, u1), jnp.where(bit4, u1, l1), jnp.where(bit6, l2, u2),
                     jnp.where(bit6, u2, l2), jnp.where(bit6, l3, u3)]
            tiles.append(jnp.where(((lane8 >> 4) == 2) | ((lane8 >> 4) == 5), pltpu.roll(tiles[3], 16, 1), tiles[2]))
            tiles.append(jnp.where(lane8 < 96, tiles[3], tiles[2]))
            tiles.append(jnp.where(lane8 < 32, tiles[4], tiles[3]))
            for u in (src[24, sl, :], jnp.where(lane8 == lane256, tiles[1], 0.0)):
                tiles.append(jnp.broadcast_to(jnp.sum(u, axis=1, keepdims=True), (8, P)))
            for t, tile in enumerate(tiles):
                dst[t, sl, :] = tile
        return 0

    with jax.named_scope("setup"):
        for k in range(6):
            cprm(0, k).wait()
        for c in (cx, cg, cfu, cfi):
            c.start()
        jax.lax.fori_loop(0, D // GS, k_setup, 0)
    with jax.named_scope("lags"):
        jax.lax.fori_loop(0, D // GA, k_lags, 0)

    LB = 2 * P

    def col_sum(parts):
        acc = [functools.reduce(jnp.add, parts[k::4]) for k in range(4)]
        return (acc[0] + acc[1]) + (acc[2] + acc[3])

    def ln_sum(c, _):
        src = x_v.at[:, span(c, LB)]
        row_v[0, :, span(c, LB)] = col_sum([src[r:r + 8, :].astype(F32) for r in range(0, D, 8)])
        return 0

    def ln_centre(c, _):
        src, dst = x_v.at[:, span(c, LB)], d_v.at[:, span(c, LB)]
        mb = row_v[0, :, span(c, LB)]
        acc = [0.0] * 4
        for r in range(0, D, 8):
            d = src[r:r + 8, :].astype(F32) - mb
            dst[r:r + 8, :] = d.astype(BF16)
            acc[r // 8 % 4] += d * d
        row_v[1, :, span(c, LB)] = col_sum(acc)
        return 0

    def ln_scale(c, _):
        src, dst = d_v.at[:, span(c, LB)], h_v.at[:, span(c, LB)]
        inv = row_v[0, :, span(c, LB)]
        for r in range(0, D, 8):
            dst[r:r + 8, :] = (src[r:r + 8, :].astype(F32) * inv).astype(BF16)
        return 0

    def compact(v):
        return jnp.concatenate([functools.reduce(
            lambda a, q: jnp.where(sub8 == q, v[:, (c + q) * P:(c + q + 1) * P], a),
            range(1, 8), v[:, c * P:(c + 1) * P]) for c in range(0, NB, 8)], axis=0)

    def spread(v):
        return jnp.concatenate([jnp.broadcast_to(v[c:c + 1], (8, P)) for c in range(NB)], axis=1)

    def total(k):
        return compact(jnp.broadcast_to(jnp.sum(row_v[k], axis=0, keepdims=True), (8, L)))

    with jax.named_scope("lnorm"):
        cx.wait()
        jax.lax.fori_loop(0, L // LB, ln_sum, 0)
        m = total(0) / D
        mb = _rbf(m)
        row_v[0] = spread(mb)
        jax.lax.fori_loop(0, L // LB, ln_centre, 0)
        var = jnp.maximum(total(1) / D - (m - mb) * (m - mb), 0.0)
        row_v[0] = spread(0.5 / _rbf(jnp.sqrt(_rbf(_rbf(var) + _rbf(jnp.full_like(var, 1e-5))))))
        jax.lax.fori_loop(0, L // LB, ln_scale, 0)

    def put(dst, kind, c, g, a, b):
        for q, v in enumerate((a, b, a - b)):
            hat_v[dst, 3 * kind + q, c, 8 * g:8 * g + 8, :] = v

    def c_signal(src, dst, c0, n):
        lhs = jnp.concatenate([h_v[span(src, GD), c * P:(c + 1) * P] for c in range(c0, c0 + n)], axis=0)
        uh = _dot(lhs, pltpu.bitcast(fu_v[...], BF16))
        for c in range(n):
            for g in range(GD // 8):
                r = slice(c * GD + 8 * g, c * GD + 8 * g + 8)
                put(dst, 0, c0 + c, g, uh[r, :P], uh[r, P:])
                yield 1

    def c_window(src, dst, j):
        tiles = kc_v.at[:, span(src, GD)]
        kh = None
        for t, ids in zip(_SRC[j], layout[j]):
            rhs = jnp.concatenate([jnp.zeros((8, 2 * P), jnp.uint32) if n is None else g_v[n] for n in ids], axis=0)
            part = _dot(tiles[t], pltpu.bitcast(rhs, BF16))
            kh = part if kh is None else kh + part
        for g in range(GD // 8):
            sl = slice(8 * g, 8 * g + 8)
            a, b = kh[sl, :P], kh[sl, P:]
            if j == 0:
                a = a + tiles[8, sl, :]
            if j == 3:
                edge = pltpu.bitcast(g_v[g_v.shape[0] - 1], F32)
                a, b = a + tiles[9, sl, :] * edge[:, :P], b + tiles[9, sl, :] * edge[:, P:]
            put(dst, 1, j, g, a, b)
            yield 1

    def c_inverse(i, c0, n):
        lhs = jnp.concatenate([jnp.concatenate([hat_v[i, 6 + q, c] for q in range(2)], axis=1)
                               for c in range(c0, c0 + n)], axis=0)
        y = _dot(lhs, pltpu.bitcast(fi_v[...], BF16))
        for c in range(n):
            for g in range(GD // 8):
                s_v[i, 8 * g:8 * g + 8, (c0 + c) * P:(c0 + c + 1) * P] = y[c * GD + 8 * g:c * GD + 8 * g + 8]
                yield 1

    window_pairs = ((14, 15), (12, 13), (10, 11), (8, 9), (6, 7), (4, 5), (0, 3), (1, 2))

    def c_transforms(i):
        nxt = jnp.minimum(i, ND - 2) + 1
        for c0 in range(0, NB, UB):
            _zip(c_signal(nxt, i + 1, c0, UB), c_inverse(i, c0, UB))
            yield UB
            for pair in window_pairs[c0 // 2:(c0 + UB) // 2]:
                _zip(*(c_window(nxt, i + 1, j) for j in pair))
                yield len(_SRC[pair[0]])

    def c_product(i):
        for g in range(GD // 8):
            sl = slice(8 * g, 8 * g + 8)
            for cs in (range(8, 16), range(8)):
                m0 = {}
                for q in range(3):
                    acc = dict(m0)
                    for j in reversed(range(max(cs) + 1)):
                        k = hat_v[i, 3 + q, j, sl, :]
                        live = [c for c in cs if c >= j]
                        for c in live:
                            t = k * hat_v[i, q, c - j, sl, :]
                            acc[c] = t if c not in acc else (acc[c] - t if q else acc[c] + t)
                        yield len(live)
                    if q == 0:
                        m0 = acc
                    else:
                        for c in cs:
                            hat_v[i + 1, 5 + q, c, sl, :] = acc[c]

    def c_step(i, pace, *extra):
        _interleave((c_product(i), GD // 8 * 3 * 136), (c_transforms(i), 25 * pace), *extra)

    with jax.named_scope("topk"):
        for c in (cg, cfu, cfi):
            c.wait()
        wr = jnp.broadcast_to(2.0 * wr_v[...].astype(F32)[None, :], (8, D))
        r = _rbf(compact(_dot(wr, h_v[...])))
        bits = pltpu.bitcast(jnp.where(r == 0.0, 0.0, r), jnp.int32)
        ordered = jnp.where(bits < 0, ~bits, bits ^ jnp.int32(-2**31))
        idx = (jax.lax.broadcasted_iota(jnp.int32, (NB, P), 0) * P
               + jax.lax.broadcasted_iota(jnp.int32, (NB, P), 1))
        key = pltpu.bitcast((jax.lax.shift_right_logical(ordered, 16) << 11) + (0x20000000 + L - 1 - idx), F32)
        rest, top = key, jnp.zeros((8, P), F32)
        for q in range(8):
            mx = jnp.max(jnp.max(rest, axis=0, keepdims=True), axis=1, keepdims=True)
            top = jnp.where(sub8 == q, mx, top)
            rest = jnp.where(rest == mx, 0.0, rest)
        _zip(c_signal(0, 0, 0, NB // 2), c_signal(0, 0, NB // 2, NB // 2))
        for pair in window_pairs:
            _zip(*(c_window(0, 0, j) for j in pair))
        hat_v[0, 6:8] = jnp.zeros((2,) + hat_v.shape[2:], F32)
        oh_v[...] = jnp.where(spread(key) == jnp.concatenate([top] * NB, axis=1), 1.0, 0.0)
        o16 = jax.lax.shift_right_logical(pltpu.bitcast(top, jnp.int32) - 0x20000000, 11) << 16
        r_top = pltpu.bitcast(jnp.where(o16 < 0, o16 ^ jnp.int32(-2**31), (~o16) & jnp.int32(-65536)), F32)
        gate = 0.5 * jax.nn.sigmoid(r_top)

    def gather_step(i, acc):
        n = L // NG
        oh, h = oh_v.at[:, span(i, n)], h_v.at[:, span(i, n)]
        parts = []

        def gather():
            for r in range(0, D, P):
                yield 0.5
                parts.append(functools.reduce(jnp.add, [
                    _dot_nt(oh[:, c:c + P], h[r:min(r + P, D), c:c + P]) for c in range(0, n, P)]))
                yield 0.5

        c_step(i, CS[0], (gather(), 5 * CS[0]))
        return acc + jnp.concatenate(parts, axis=1)

    with jax.named_scope("conv0"):
        x_sel = 2.0 * jax.lax.fori_loop(0, NG, gather_step, jnp.zeros((8, D), F32))
        row_v[0, :, :D] = x_sel

    def gate_up_step(item, _):
        i = item - NG
        ws, dst = (wg_v.at[:, span(i, FC)], wu_v.at[:, span(i, FC)]), act_v.at[:, :, span(i, FC)]

        def gate_up():
            for c in range(0, FC, 2 * P):
                acc = [0.0, 0.0]
                for r in range(0, D, P):
                    yield 0.5
                    rs = slice(r, min(r + P, D))
                    acc = [a + _dot(row_v[0, :, rs], w[rs, c:c + 2 * P]) for a, w in zip(acc, ws)]
                    yield 0.5
                for k in range(2):
                    dst[k, :, c:c + 2 * P] = acc[k]

        c_step(item, CS[1], (gate_up(), FC // (2 * P) * 5 * CS[1]))

        @pl.when(i + 1 < NF)
        def _():
            cwg(i + 1).wait()
            cwu(i + 1).wait()

        return 0

    with jax.named_scope("conv1"):
        cwg(0).wait()
        cwu(0).wait()
        jax.lax.fori_loop(NG, NG + NF, gate_up_step, 0)
        a = 0.5 * act_v[0]
        act_v[0] = (a + a * jnp.tanh(a)) * act_v[1]

    eye = (jax.lax.broadcasted_iota(jnp.int32, (GE, GE), 0)
           == jax.lax.broadcasted_iota(jnp.int32, (GE, GE), 1)).astype(F32)

    def finish(e, lead):
        w = wd_v.at[span(e, GE)]
        acc = 0.0
        for c in range(0, FF, 4 * P):
            yield 0.5
            acc = acc + functools.reduce(jnp.add, [
                _dot_nt(act_v[0, :, f:f + P], w[:, f:f + P]) for f in range(c, c + 4 * P, P)])
            yield 0.5
        yield lead
        yt = _dot_nt(eye, acc * gate[:, :GE])
        yield lead
        h = h_v[span(e, GE), :].astype(F32) + _dot(yt, oh_v[...])
        s = jnp.concatenate([s_v[e * (GE // GD) + 1 + n] for n in range(GE // GD)], axis=0)
        q = s * h
        out = (x_v[span(e, GE), :].astype(F32) + q) + q * jnp.tanh(h)
        if debug:
            out = s
        o_v[span(e, GE), :] = out.astype(o_v.dtype)

    def finish_step(item, _):
        e = item - (NG + NF)
        c_step(item, CS[2], (finish(e, 3.0), (FF // (4 * P) + 6.0) * CS[2]))
        cout(e).start()
        cwd(e + 1).wait()
        return 0

    with jax.named_scope("conv2"):
        cwd(0).wait()
        jax.lax.fori_loop(NG + NF, ND, finish_step, 0)

    with jax.named_scope("tail"):
        _zip(c_inverse(ND, 0, NB // 2), c_inverse(ND, NB // 2, NB // 2))
        row_v[1, :, :P] = functools.reduce(jnp.add, [hat_v[i, q, NB - 1, GD - 8:, :] for i in (ND,) for q in range(6)])
        for e in range(ND - NG - NF, NE):
            if e > ND - NG - NF:
                cwd(e).wait()
            _zip(finish(e, 0.0))
            cout(e).start()
        for e in range(NE):
            cout(e).wait()


def run(A_u, A_A_re, A_A_im, A_B_re, A_B_im, A_C_re, A_C_im, A_log_dt, A_Dskip, B_x, B_w_r,
        B_w_gate, B_w_up, B_w_down, GS=64, GA=96, GD=32, NG=4, NF=6, GE=64, CS=(1.12, 1.12, 1.0), UB=2,
        debug=False, interpret=False, flags=None):
    _, L, D = A_u.shape
    FF = B_w_gate.shape[1]
    fu, fi, g = _tables()[:3]
    odt = F32 if debug else A_u.dtype
    hbm = pl.BlockSpec(memory_space=pl.ANY)
    NB = L // P
    out = pl.pallas_call(
        functools.partial(_kernel, GS=GS, GA=GA, GD=GD, NG=NG, NF=NF, GE=GE, CS=CS, UB=UB, debug=debug),
        out_shape=jax.ShapeDtypeStruct((D, L), odt),
        in_specs=[hbm] * 16,
        out_specs=hbm,
        scratch_shapes=[
            *[pltpu.VMEM((D,), BF16)] * 3,
            pltpu.VMEM((D, L), BF16), pltpu.VMEM((6, D, P), BF16),
            pltpu.VMEM((D, FF), BF16), pltpu.VMEM((D, FF), BF16), pltpu.VMEM((D, FF), BF16),
            pltpu.VMEM(fu.shape, jnp.uint32), pltpu.VMEM(fi.shape, jnp.uint32),
            pltpu.VMEM(g.shape, jnp.uint32),
            pltpu.VMEM((D, L), odt), pltpu.VMEM((D, L), BF16), pltpu.VMEM((D, L), BF16),
            pltpu.VMEM((D // GD + 1, GD, L), F32),
            pltpu.VMEM((10, D, P), F32), pltpu.VMEM((2, D, P), F32),
            pltpu.VMEM((2, 8, L), F32), pltpu.VMEM((8, L), F32), pltpu.VMEM((2, 8, FF), F32),
            pltpu.VMEM((D // GD + 1, 8, NB, GD, P), F32),
            pltpu.VMEM((25, D, P), F32),
            pltpu.SemaphoreType.DMA((7 + 2 * NF + D // GE,)),
            pltpu.SemaphoreType.DMA((12,)),
            pltpu.SemaphoreType.DMA((D // GE,)),
        ],
        compiler_params=pltpu.CompilerParams(vmem_limit_bytes=112 * 2**20, flags=flags),
        interpret=interpret,
        name="ssm_moe",
    )(A_u[0].T, A_A_re, A_A_im, A_B_re, A_B_im, A_C_re, A_C_im, A_log_dt, A_Dskip, B_w_r,
      B_w_gate, B_w_up, B_w_down.T, fu, fi, g)
    return out.T[None]


@jax.jit
def pallas_recurrent_scan__ssm_conv_s4__moe_arch_mod__prompt_kernel(
    A_u: jax.Array,
    A_A_re: jax.Array,
    A_A_im: jax.Array,
    A_B_re: jax.Array,
    A_B_im: jax.Array,
    A_C_re: jax.Array,
    A_C_im: jax.Array,
    A_log_dt: jax.Array,
    A_Dskip: jax.Array,
    B_x: jax.Array,
    B_w_r: jax.Array,
    B_w_gate: jax.Array,
    B_w_up: jax.Array,
    B_w_down: jax.Array,
):
    return run(A_u, A_A_re, A_A_im, A_B_re, A_B_im, A_C_re, A_C_im, A_log_dt, A_Dskip, B_x,
               B_w_r, B_w_gate, B_w_up, B_w_down)
```

```python
import contextlib
import functools

import jax
import jax.numpy as jnp
import numpy as np
import jax.experimental.pallas as pl
import jax.experimental.pallas.tpu as pltpu

F32 = jnp.float32
BF16 = jnp.bfloat16
P = 128


def _bf16_bits(a):
    u = np.ascontiguousarray(a, dtype=np.float32).view(np.uint32)
    return ((u + 0x7FFF + ((u >> 16) & 1)) >> 16).astype(np.uint32)


def _round_bf16(a):
    return (_bf16_bits(a) << 16).view(np.float32)


def _pack_rows(a):
    b = _bf16_bits(a)
    return (b[0::2] | (b[1::2] << 16)).astype(np.uint32)


def _tile_lags():
    lane = np.arange(P)
    quarter, hb, j = lane // 32, (lane // 16) % 2, lane % 16

    def half(offsets, second):
        q = (quarter + 2 * second) % 4
        return np.array(offsets)[q] + 128 * (hb ^ second) + 8 * j

    l1, u1 = half((1, 2, 3, 4), 0), half((5, 6, 7, 8), 1)
    l2, u2 = half((258, 260, 516, 772), 0), half((262, 264, 520, 776), 1)
    l3, u3 = half((1032, 1288) * 2, 0), half((1544, 1800) * 2, 1)
    lags = [np.where(hb == 0, l1, u1), np.where(hb == 0, u1, l1),
            np.where(lane < 64, l2, u2), np.where(lane < 64, u2, l2), np.where(lane < 64, l3, u3)]
    lags.append(np.where(lane // 16 == 0, half((516,) * 4, 0),
                         np.where(lane // 16 == 5, half((520,) * 4, 1), lags[2])))
    lags.append(np.where(lane < 96, lags[3], lags[2]))
    lags.append(np.where(lane < 32, lags[4], lags[3]))
    return lags


_SRC = ((0,), (0, 1), (1, 2), (2,), (5,), (6,), (3,), (3,), (7,), (7,)) + ((4,),) * 6


@functools.cache
def _tables():
    k = np.arange(P)
    phi = 2 * np.pi * (k + 0.25) / P

    def coords(m):
        z = np.exp(1j * np.outer(m, phi))
        return np.concatenate([z.real + z.imag / np.sqrt(3), 2 * z.imag / np.sqrt(3)], axis=1)

    fu = 2.0 * coords(np.arange(P))
    zi = np.exp(-1j * np.outer(phi, np.arange(P)))
    fi = np.concatenate([zi.real, (np.exp(2j * np.pi / 3) * zi).real], axis=0) / P
    lags = _tile_lags()
    groups, layout = [], []
    for j, src in enumerate(_SRC):
        m = np.arange(-P + 1 + (j == 3), P)
        m = m[P * j + m >= 1]
        rl = _round_bf16(P * j + m)
        hit = np.zeros(len(m), int)
        layout.append([])
        for t in src:
            sel = (lags[t][:, None] == rl[None, :])
            hit += sel.sum(0)
            g = _pack_rows(sel.astype(np.float64) @ coords(m))
            ids = []
            for r in range(0, P // 2, 8):
                known = [n for n, e in enumerate(groups) if np.array_equal(e, g[r:r + 8])]
                if not sel[2 * r:2 * r + 16].any():
                    ids.append(None)
                elif known:
                    ids.append(known[0])
                else:
                    ids.append(len(groups))
                    groups.append(g[r:r + 8])
            layout[-1].append(ids)
        assert (hit == 1).all()
    edge = np.broadcast_to(coords(np.array([-P + 1])).astype(np.float32), (8, 2 * P)).view(np.uint32)
    return _pack_rows(fu), _pack_rows(fi), np.stack(groups + [edge]), layout


def _cmul(a, b):
    return (a[0] * b[0] - a[1] * b[1], a[0] * b[1] + a[1] * b[0])


def _csq(a):
    t = a[0] * a[1]
    return ((a[0] - a[1]) * (a[0] + a[1]), t + t)


def _dot(a, b):
    return jax.lax.dot_general(a, b, (((1,), (0,)), ((), ())), preferred_element_type=F32)


def _dot_nt(a, b):
    return jax.lax.dot_general(a, b, (((1,), (1,)), ((), ())), preferred_element_type=F32)


def _rbf(x):
    return x.astype(BF16).astype(F32)


def _interleave(*gens):
    state = [[0.0, k, g, total] for k, (g, total) in enumerate(gens)]
    while state:
        cur = min(state, key=lambda e: (e[0], e[1]))
        w = next(cur[2], None)
        if w is None:
            state.remove(cur)
        else:
            cur[0] += w / cur[3]


def _zip(*gens):
    _interleave(*((g, 1.0) for g in gens))


_ZP = (1, 8, 32, 256)


def _kernel(x_hbm, are_hbm, aim_hbm, bre_hbm, bim_hbm, cre_hbm, cim_hbm, ldt_hbm, dsk_hbm,
            wr_hbm, wg_hbm, wu_hbm, wd_hbm, fu_hbm, fi_hbm, g_hbm, o_hbm,
            ldt_v, dsk_v, wr_v, x_v, prm_v, wg_v, wu_v, wd_v, fu_v, fi_v, g_v, o_v, d_v, h_v, s_v,
            kc_v, dt_v, row_v, oh_v, act_v, hat_v, p_v, sems, psem, osem,
            *, GS, GA, GD, NG, NF, GE, GT, LD, CS, UB, SC, debug):
    scope = jax.named_scope if SC else (lambda _: contextlib.nullcontext())
    D, L = x_v.shape
    FF = wg_v.shape[1]
    NB = L // P
    FC = FF // NF
    ND = D // GD
    NL = ND - NG - NF
    tails = tuple(range(NL * GE, D, GT))
    layout = _tables()[3]

    def span(i, n):
        start = i * n
        if not isinstance(start, int):
            start = pl.multiple_of(start, n)
        return pl.ds(start, n)

    prm_hbm = (are_hbm, aim_hbm, bre_hbm, bim_hbm, cre_hbm, cim_hbm)

    def cprm(part, k):
        r = pl.ds(0, 3 * GS) if part == 0 else pl.ds(3 * GS, D - 3 * GS)
        return pltpu.make_async_copy(prm_hbm[k].at[r], prm_v.at[k, r], psem.at[6 * part + k])

    cx, cfu, cfi, cg, *cvec = (
        pltpu.make_async_copy(src, dst, sems.at[k]) for k, (src, dst) in enumerate((
            (x_hbm, x_v), (fu_hbm, fu_v), (fi_hbm, fi_v), (g_hbm, g_v),
            (ldt_hbm, ldt_v), (dsk_hbm, dsk_v), (wr_hbm, wr_v))))

    def cwg(i):
        return pltpu.make_async_copy(wg_hbm.at[:, span(i, FC)], wg_v.at[:, span(i, FC)], sems.at[7 + i])

    def cwu(i):
        return pltpu.make_async_copy(wu_hbm.at[:, span(i, FC)], wu_v.at[:, span(i, FC)], sems.at[7 + NF + i])

    def out_rows(i):
        if isinstance(i, int) and i >= NL:
            return pl.ds(tails[i - NL], GT)
        return pl.ds(i * GE if isinstance(i, int) else pl.multiple_of(i * GE, 16), GE)

    def cwd(i):
        return pltpu.make_async_copy(wd_hbm.at[out_rows(i)], wd_v.at[out_rows(i)], sems.at[7 + 2 * NF + i])

    def cout(i):
        return pltpu.make_async_copy(o_v.at[out_rows(i)], o_hbm.at[out_rows(i)], osem.at[i])

    for c in cvec:
        c.start()
    for k in range(6):
        cprm(0, k).start()

    @pl.loop(0, NF)
    def _(i):
        cwg(i).start(priority=1)
        cwu(i).start(priority=1)

    @pl.loop(0, NL)
    def _(i):
        cwd(i).start(priority=1)

    for i in range(len(tails)):
        cwd(NL + i).start(priority=1)

    for k in range(6):
        cprm(1, k).start()
    for c in cvec:
        c.wait()

    dt_row = _rbf(jnp.exp(ldt_v[...].astype(F32)[None, :]))
    dsk_row = dsk_v[...].astype(F32)[None, :] * (1.0 / P)
    for c0 in range(0, D, P):
        n = min(P, D - c0)
        eye = (jax.lax.broadcasted_iota(jnp.int32, (n, n), 0) == jax.lax.broadcasted_iota(jnp.int32, (n, n), 1))
        for k, row in enumerate((dt_row, dsk_row)):
            dt_v[k, c0:c0 + n, :] = _dot(jnp.where(eye, row[:, c0:c0 + n], 0.0), jnp.ones((n, P), BF16))

    lane8 = jax.lax.broadcasted_iota(jnp.int32, (8, P), 1)
    sub8 = jax.lax.broadcasted_iota(jnp.int32, (8, P), 0)

    def k_setup(i, _):
        @pl.when(i == 3)
        def _():
            for k in range(6):
                cprm(1, k).wait()

        low = sub8 < 4
        for g in range(GS // 16):
            sl = slice(16 * g, 16 * g + 16)
            dt, dsk = (dt_v.at[k, span(i, GS)][sl, :] for k in range(2))
            a_re, a_im, b_re, b_im, c_re, c_im = (prm_v.at[k, span(i, GS)][sl, :].astype(F32) for k in range(6))
            dst = p_v.at[:, span(i, GS)]
            w = {0: _cmul((c_re, c_im), (dt * b_re, dt * b_im))}
            mag = jnp.exp(dt * a_re)
            z = {1: (mag * jnp.cos(dt * a_im), mag * jnp.sin(dt * a_im))}
            for e in range(10):
                z[2 << e] = _csq(z[1 << e])
            for n, e in enumerate(_ZP):
                for q in range(2):
                    dst[2 * n + q, sl, :] = z[e][q]
            dst[24, sl, :] = w[0][0] + dsk
            dst[25, sl, :] = w[0][0] * z[256][0] - w[0][1] * z[256][1]
            w[4], w[8] = _cmul(w[0], z[4]), _cmul(w[0], z[8])
            w[1032] = _cmul(w[8], z[1024])
            w[1544] = _cmul(w[1032], z[512])
            one = (jnp.ones((16, P), F32), jnp.zeros((16, P), F32))
            for n, (a, b) in enumerate(((one, z[128]), (w[0], w[4]), (w[4], w[8]), (w[1032], w[1544]))):
                for q in range(2):
                    for t in range(2):
                        x, y = a[q][8 * t:8 * t + 8], pltpu.roll(b[q][8 * t:8 * t + 8], 4, 0)
                        r = slice(16 * g + 8 * t, 16 * g + 8 * t + 8)
                        dst[8 + 4 * n + q, r, :] = jnp.where(low, x, y)
                        dst[10 + 4 * n + q, r, :] = jnp.where(low, y, x)
        return 0

    def k_lags(i, _):
        low = sub8 < 4
        bit4, bit5, bit6 = ((lane8 & b) == 0 for b in (16, 32, 64))
        bit6x = ((lane8 >> 4) ^ sub8) & 4 == 0
        diag = (lane8 & 15) * 8 + (((lane8 >> 2) & 4) ^ sub8)
        src, dst = p_v.at[:, span(i, GA)], kc_v.at[:, span(i, GA)]
        for g in range(GA // 8):
            sl = slice(8 * g, 8 * g + 8)
            out = []
            for h in range(2):
                off = (4 if h else 0) if g + 1 < GA // 8 else (0 if h else -4)
                z = {e: tuple(jnp.take_along_axis(src[2 * n + q, 8 * g + off:8 * g + off + 8, :],
                                                  (sub8 & 3) + (4 * h - off), axis=0,
                                                  mode="promise_in_bounds") for q in range(2))
                     for n, e in enumerate(_ZP)}
                b0, r, a4, far = (tuple(src[8 + 4 * n + 2 * h + q, sl, :] for q in range(2)) for n in range(4))
                bs = [b0]
                for j in range(1, 16):
                    bs.append(_cmul(bs[j - 1], z[8]) if j < 4 else _cmul(bs[j - 4], z[32]))
                av = [_cmul(r, z[1])]
                av += [_cmul(av[0], z[1])]
                av += [_cmul(av[1], z[1]), a4, _cmul(av[1], z[256]), _cmul(a4, z[256])]
                av.append(_cmul(av[-1], z[256]))
                av.append(_cmul(av[-1], z[256]))
                av += [far, _cmul(far, z[256])]
                out.append([_dot_nt(jnp.concatenate([v[q] for v in av], axis=0),
                                    jnp.concatenate([v[q] for v in reversed(bs)], axis=0).astype(BF16))
                            for q in range(2)])
            d = [[out[h][0][8 * n:8 * n + 8] - out[h][1][8 * n:8 * n + 8] for n in range(10)] for h in range(2)]
            v = [[None] * 10, [None] * 10]
            for n in range(10):
                for h in range(2):
                    v[h][n] = jnp.take_along_axis(d[h][n], diag ^ 120, axis=1, mode="promise_in_bounds")

            def unzip(xs):
                return jnp.where(low, xs[0], xs[1]), pltpu.roll(jnp.where(low, xs[1], xs[0]), 4, 0)

            halves = []
            for lo, hi in ((0, 4), (4, 8), (8, 10)):
                xs = []
                for h in range(2):
                    u = [jnp.where(bit5, v[h][n], v[h][n + 1]) for n in range(lo, hi, 2)]
                    xs.append(jnp.where(bit6x, u[h], u[1 - h]) if len(u) == 2 else u[0])
                halves.append(unzip(xs))
            (l1, u1), (l2, u2), (l3, u3) = halves
            l6, u6 = unzip((v[0][6], v[1][6]))
            tiles = [jnp.where(bit4, l1, u1), jnp.where(bit4, u1, l1), jnp.where(bit6, l2, u2),
                     jnp.where(bit6, u2, l2), jnp.where(bit6, l3, u3)]
            tiles.append(jnp.where(lane8 < 16, l6, jnp.where((lane8 >> 4) == 5, u6, tiles[2])))
            tiles.append(jnp.where(lane8 < 96, tiles[3], tiles[2]))
            tiles.append(jnp.where(lane8 < 32, tiles[4], tiles[3]))
            for t, tile in enumerate(tiles):
                dst[t, sl, :] = tile
        return 0

    with scope("setup"):
        for k in range(6):
            cprm(0, k).wait()
        for c in (cx, cg, cfu, cfi):
            c.start()
        jax.lax.fori_loop(0, D // GS, k_setup, 0)
    with scope("lags"):
        jax.lax.fori_loop(0, D // GA, k_lags, 0)

    LB, RB, HB = 2 * P, 96, h_v.shape[2]

    def col_sum(parts):
        acc = [functools.reduce(jnp.add, parts[k::4]) for k in range(4)]
        return (acc[0] + acc[1]) + (acc[2] + acc[3])

    def ln_sum(i, _):
        src = x_v.at[span(i, RB)]
        acc = row_v[0]
        for r in range(0, RB, 8):
            acc = acc + src[r:r + 8, :].astype(F32)
        row_v[0] = acc
        return 0

    def ln_centre(c, _):
        src, dst = x_v.at[:, span(c, LB)], d_v.at[:, span(c, LB)]
        rows = span(c, D * LB // L)
        for t in range(2):
            kc_v[8 + t, rows, :] = jnp.broadcast_to(
                jnp.sum(p_v[24 + t, rows, :], axis=1, keepdims=True), (rows.size, P))
        mb = row_v[0, :, span(c, LB)]
        acc = [0.0] * 4
        for r in range(0, D, 8):
            d = src[r:r + 8, :].astype(F32) - mb
            dst[r:r + 8, :] = d.astype(BF16)
            acc[r // 8 % 4] += d * d
        row_v[1, :, span(c, LB)] = col_sum(acc)
        return 0

    def ln_scale(c):
        src, inv = d_v.at[:, span(c, HB)], row_v[0, :, span(c, HB)]
        for r in range(0, D, 8):
            h_v[c, r:r + 8, :] = (src[r:r + 8, :].astype(F32) * inv).astype(BF16)

    def ln_route(c, _):
        oh_v[:, span(c, HB)] = _dot(wr, h_v[c])
        ln_scale(c + 1)
        return 0

    def h_block(rows, c):
        return h_v[c * P // HB, rows, c * P % HB:c * P % HB + P]

    def compact(v):
        return jnp.concatenate([functools.reduce(
            lambda a, q: jnp.where(sub8 == q, v[:, (c + q) * P:(c + q + 1) * P], a),
            range(1, 8), v[:, c * P:(c + 1) * P]) for c in range(0, NB, 8)], axis=0)

    def spread(v):
        return jnp.concatenate([jnp.broadcast_to(v[c:c + 1], (8, P)) for c in range(NB)], axis=1)

    def total(k):
        return compact(jnp.broadcast_to(jnp.sum(row_v[k], axis=0, keepdims=True), (8, L)))

    with scope("lnorm"):
        for c in (cx, cg, cfu, cfi):
            c.wait()
        row_v[0] = jnp.zeros((8, L), F32)
        jax.lax.fori_loop(0, D // RB, ln_sum, 0)
        m = total(0) / D
        mb = _rbf(m)
        row_v[0] = spread(mb)
        jax.lax.fori_loop(0, L // LB, ln_centre, 0)
        var = jnp.maximum(total(1) / D - (m - mb) * (m - mb), 0.0)
        row_v[0] = spread(0.5 / _rbf(jnp.sqrt(_rbf(_rbf(var) + _rbf(jnp.full_like(var, 1e-5))))))
        wr = jnp.broadcast_to(2.0 * wr_v[...].astype(F32)[None, :], (8, D))
        ln_scale(0)
        jax.lax.fori_loop(0, L // HB - 1, ln_route, 0)
        oh_v[:, L - HB:] = _dot(wr, h_v[L // HB - 1])

    def put(dst, kind, c, g, a, b):
        for q, v in enumerate((a, b, a - b)):
            hat_v[dst, 3 * kind + q, c, 8 * g:8 * g + 8, :] = v

    def c_signal(src, dst, c0, n):
        lhs = jnp.concatenate([h_block(span(src, GD), c) for c in range(c0, c0 + n)], axis=0)
        uh = _dot(lhs, pltpu.bitcast(fu_v[...], BF16))
        for c in range(n):
            for g in range(GD // 8):
                r = slice(c * GD + 8 * g, c * GD + 8 * g + 8)
                put(dst, 0, c0 + c, g, uh[r, :P], uh[r, P:])
                yield 1

    def c_window(src, dst, j):
        tiles = kc_v.at[:, span(src, GD)]
        kh = None
        for t, ids in zip(_SRC[j], layout[j]):
            rhs = jnp.concatenate([jnp.zeros((8, 2 * P), jnp.uint32) if n is None else g_v[n] for n in ids], axis=0)
            part = _dot(tiles[t], pltpu.bitcast(rhs, BF16))
            kh = part if kh is None else kh + part
        for g in range(GD // 8):
            sl = slice(8 * g, 8 * g + 8)
            a, b = kh[sl, :P], kh[sl, P:]
            if j == 0:
                a = a + tiles[8, sl, :]
            if j == 3:
                edge = pltpu.bitcast(g_v[g_v.shape[0] - 1], F32)
                a, b = a + tiles[9, sl, :] * edge[:, :P], b + tiles[9, sl, :] * edge[:, P:]
            put(dst, 1, j, g, a, b)
            yield 1

    def c_inverse(i, c0, n):
        lhs = jnp.concatenate([jnp.concatenate([hat_v[i, 6 + q, c] for q in range(2)], axis=1)
                               for c in range(c0, c0 + n)], axis=0)
        y = _dot(lhs, pltpu.bitcast(fi_v[...], BF16))
        for c in range(n):
            for g in range(GD // 8):
                s_v.at[span(i, GD)][8 * g:8 * g + 8, (c0 + c) * P:(c0 + c + 1) * P] = y[c * GD + 8 * g:c * GD + 8 * g + 8]
                yield 1

    window_pairs = ((14, 15), (12, 13), (10, 11), (8, 9), (6, 7), (4, 5), (0, 3), (1, 2))

    def c_transforms(i):
        nxt = jnp.minimum(i, ND - 2) + 1
        for c0 in range(0, NB, UB):
            _zip(c_signal(nxt, i + 1, c0, UB), c_inverse(i, c0, UB))
            yield UB
            for pair in window_pairs[c0 // 2:(c0 + UB) // 2]:
                _zip(*(c_window(nxt, i + 1, j) for j in pair))
                yield len(_SRC[pair[0]])

    def c_product(i):
        for g in range(GD // 8):
            sl = slice(8 * g, 8 * g + 8)
            for cs in (range(8, 16), range(8)):
                m0 = {}
                for q in range(3):
                    acc = dict(m0)
                    for j in reversed(range(max(cs) + 1)):
                        k = hat_v[i, 3 + q, j, sl, :]
                        live = [c for c in cs if c >= j]
                        for c in live:
                            t = k * hat_v[i, q, c - j, sl, :]
                            acc[c] = t if c not in acc else (acc[c] - t if q else acc[c] + t)
                        yield len(live)
                    if q == 0:
                        m0 = acc
                    else:
                        for c in cs:
                            hat_v[i + 1, 5 + q, c, sl, :] = acc[c]

    def c_step(i, pace, *extra):
        _interleave((c_product(i), GD // 8 * 3 * 136), (c_transforms(i), 25 * pace), *extra)

    with scope("topk"):
        r = _rbf(compact(oh_v[...]))
        bits = pltpu.bitcast(jnp.where(r == 0.0, 0.0, r), jnp.int32)
        ordered = jnp.where(bits < 0, ~bits, bits ^ jnp.int32(-2**31))
        idx = (jax.lax.broadcasted_iota(jnp.int32, (NB, P), 0) * P
               + jax.lax.broadcasted_iota(jnp.int32, (NB, P), 1))
        key = pltpu.bitcast((jax.lax.shift_right_logical(ordered, 16) << 11) + (0x20000000 + L - 1 - idx), F32)
        rest, top = key, jnp.zeros((8, P), F32)
        for q in range(8):
            mx = jnp.max(jnp.max(rest, axis=0, keepdims=True), axis=1, keepdims=True)
            top = jnp.where(sub8 == q, mx, top)
            rest = jnp.where(rest == mx, 0.0, rest)
        _zip(c_signal(0, 0, 0, NB // 2), c_signal(0, 0, NB // 2, NB // 2))
        for pair in window_pairs:
            _zip(*(c_window(0, 0, j) for j in pair))
        hat_v[0, 6:8] = jnp.zeros((2,) + hat_v.shape[2:], F32)
        oh_v[...] = jnp.where(spread(key) == jnp.concatenate([top] * NB, axis=1), 1.0, 0.0)
        o16 = jax.lax.shift_right_logical(pltpu.bitcast(top, jnp.int32) - 0x20000000, 11) << 16
        r_top = pltpu.bitcast(jnp.where(o16 < 0, o16 ^ jnp.int32(-2**31), (~o16) & jnp.int32(-65536)), F32)
        gate = 0.5 * jax.nn.sigmoid(r_top)

    def gather_step(i, acc):
        n = L // NG
        oh = oh_v.at[:, span(i, n)]
        parts = []

        def gather():
            for r in range(0, D, P):
                part = 0.0
                for c0 in range(0, n, 4 * P):
                    yield 0.5
                    part = part + functools.reduce(jnp.add, [
                        _dot_nt(oh[:, c:c + P], h_v[i * (n // HB) + c // HB, r:min(r + P, D), c % HB:c % HB + P]) for c in range(c0, c0 + 4 * P, P)])
                    yield 0.5
                parts.append(part)

        c_step(i, CS[0], (gather(), n // (4 * P) * 5 * CS[0]))
        return acc + jnp.concatenate(parts, axis=1)

    with scope("conv0"):
        x_sel = 2.0 * jax.lax.fori_loop(0, NG, gather_step, jnp.zeros((8, D), F32))
        row_v[0, :, :D] = x_sel

    def gate_up_step(item, _):
        i = item - NG
        ws, dst = (wg_v.at[:, span(i, FC)], wu_v.at[:, span(i, FC)]), act_v.at[:, :, span(i, FC)]

        def gate_up():
            for c in range(0, FC, 2 * P):
                acc = [0.0, 0.0]
                for r in range(0, D, P):
                    yield 0.5
                    rs = slice(r, min(r + P, D))
                    acc = [a + _dot(row_v[0, :, rs], w[rs, c:c + 2 * P]) for a, w in zip(acc, ws)]
                    yield 0.5
                for k in range(2):
                    dst[k, :, c:c + 2 * P] = acc[k]

        c_step(item, CS[1], (gate_up(), FC // (2 * P) * 5 * CS[1]))

        @pl.when(i + 1 < NF)
        def _():
            cwg(i + 1).wait()
            cwu(i + 1).wait()

        return 0

    with scope("conv1"):
        cwg(0).wait()
        cwu(0).wait()
        jax.lax.fori_loop(NG, NG + NF, gate_up_step, 0)
        a = 0.5 * act_v[0]
        act_v[0] = (a + a * jnp.tanh(a)) * act_v[1]

    def finish(e, lead):
        rows = out_rows(e)
        n = rows.size
        w = wd_v.at[rows]
        acc = 0.0
        for c in range(0, FF, 4 * P):
            yield 0.5
            acc = acc + functools.reduce(jnp.add, [
                _dot_nt(act_v[0, :, f:f + P], w[:, f:f + P]) for f in range(c, c + 4 * P, P)])
            yield 0.5
        yield lead
        eye = jax.lax.broadcasted_iota(jnp.int32, (n, n), 0) == jax.lax.broadcasted_iota(jnp.int32, (n, n), 1)
        yt = _dot_nt(eye.astype(F32), acc * gate[:, :n])
        yield lead
        h = jnp.concatenate([h_v[c, rows, :].astype(F32) for c in range(L // HB)], axis=1) + _dot(yt, oh_v[...])
        s = s_v.at[GD:][rows, :]
        q = s * h
        out = (x_v[rows, :].astype(F32) + q) + q * jnp.tanh(h)
        if debug:
            out = s
        o_v[rows, :] = out.astype(o_v.dtype)

    def finish_step(item, _):
        e = item - (NG + NF)
        c_step(item, CS[2], (finish(e, LD), (FF // (4 * P) + 2 * LD) * CS[2]))
        cout(e).start()

        @pl.when(e + 1 < NL)
        def _():
            cwd(e + 1).wait()

        return 0

    with scope("conv2"):
        cwd(0).wait()
        jax.lax.fori_loop(NG + NF, ND, finish_step, 0)

    with scope("tail"):
        last = [finish(NL + i, 0.0) for i in range(len(tails))]
        for i, gen in enumerate(last):
            cwd(NL + i).wait()
        for gen in last:
            for _ in range(FF // (2 * P)):
                next(gen)
        for c0 in range(0, NB, 4):
            _zip(c_inverse(ND, c0, 2), c_inverse(ND, c0 + 2, 2))
            if c0 == 4:
                for gen in last:
                    next(gen), next(gen)
        row_v[1, :, :P] = functools.reduce(jnp.add, [hat_v[ND, q, NB - 1, GD - 8:, :] for q in range(6)])
        for i, gen in enumerate(last):
            _zip(gen)
            cout(NL + i).start()
        for e in range(NL + len(tails)):
            cout(e).wait()


def run(A_u, A_A_re, A_A_im, A_B_re, A_B_im, A_C_re, A_C_im, A_log_dt, A_Dskip, B_x, B_w_r,
        B_w_gate, B_w_up, B_w_down, GS=64, GA=192, GD=64, NG=2, NF=3, GE=112, GT=64, LD=2.0, CS=(1.1, 1.1, 1.0), UB=1, SC=0,
        debug=False, interpret=False, flags=None):
    _, L, D = A_u.shape
    FF = B_w_gate.shape[1]
    fu, fi, g = _tables()[:3]
    odt = F32 if debug else A_u.dtype
    hbm = pl.BlockSpec(memory_space=pl.ANY)
    NB = L // P
    NL = D // GD - NG - NF
    NE = NL + (D - NL * GE) // GT
    out = pl.pallas_call(
        functools.partial(_kernel, GS=GS, GA=GA, GD=GD, NG=NG, NF=NF, GE=GE, GT=GT, LD=LD, CS=CS, UB=UB, SC=SC, debug=debug),
        out_shape=jax.ShapeDtypeStruct((D, L), odt),
        in_specs=[hbm] * 16,
        out_specs=hbm,
        scratch_shapes=[
            *[pltpu.VMEM((D,), BF16)] * 3,
            pltpu.VMEM((D, L), BF16), pltpu.VMEM((6, D, P), BF16),
            pltpu.VMEM((D, FF), BF16), pltpu.VMEM((D, FF), BF16), pltpu.VMEM((D, FF), BF16),
            pltpu.VMEM(fu.shape, jnp.uint32), pltpu.VMEM(fi.shape, jnp.uint32),
            pltpu.VMEM(g.shape, jnp.uint32),
            pltpu.VMEM((D, L), odt), pltpu.VMEM((D, L), BF16), pltpu.VMEM((4, D, L // 4), BF16),
            pltpu.VMEM((D + GD, L), F32),
            pltpu.VMEM((10, D, P), F32), pltpu.VMEM((2, D, P), F32),
            pltpu.VMEM((2, 8, L), F32), pltpu.VMEM((8, L), F32), pltpu.VMEM((2, 8, FF), F32),
            pltpu.VMEM((D // GD + 1, 8, NB, GD, P), F32),
            pltpu.VMEM((26, D, P), F32),
            pltpu.SemaphoreType.DMA((7 + 2 * NF + NE,)),
            pltpu.SemaphoreType.DMA((12,)),
            pltpu.SemaphoreType.DMA((NE,)),
        ],
        compiler_params=pltpu.CompilerParams(vmem_limit_bytes=112 * 2**20, flags=flags),
        interpret=interpret,
        name="ssm_moe",
    )(A_u[0].T, A_A_re, A_A_im, A_B_re, A_B_im, A_C_re, A_C_im, A_log_dt, A_Dskip, B_w_r,
      B_w_gate, B_w_up, B_w_down.T, fu, fi, g)
    return out.T[None]


@jax.jit
def pallas_recurrent_scan__ssm_conv_s4__moe_arch_mod__prompt_kernel(
    A_u: jax.Array,
    A_A_re: jax.Array,
    A_A_im: jax.Array,
    A_B_re: jax.Array,
    A_B_im: jax.Array,
    A_C_re: jax.Array,
    A_C_im: jax.Array,
    A_log_dt: jax.Array,
    A_Dskip: jax.Array,
    B_x: jax.Array,
    B_w_r: jax.Array,
    B_w_gate: jax.Array,
    B_w_up: jax.Array,
    B_w_down: jax.Array,
):
    return run(A_u, A_A_re, A_A_im, A_B_re, A_B_im, A_C_re, A_C_im, A_log_dt, A_Dskip, B_x,
               B_w_r, B_w_gate, B_w_up, B_w_down)
```

```python
import contextlib
import functools

import jax
import jax.numpy as jnp
import numpy as np
import jax.experimental.pallas as pl
import jax.experimental.pallas.tpu as pltpu

F32 = jnp.float32
BF16 = jnp.bfloat16
P = 128


def _bf16_bits(a):
    u = np.ascontiguousarray(a, dtype=np.float32).view(np.uint32)
    return ((u + 0x7FFF + ((u >> 16) & 1)) >> 16).astype(np.uint32)


def _round_bf16(a):
    return (_bf16_bits(a) << 16).view(np.float32)


def _pack_rows(a):
    b = _bf16_bits(a)
    return (b[0::2] | (b[1::2] << 16)).astype(np.uint32)


def _tile_lags():
    lane = np.arange(P)
    quarter, hb, j = lane // 32, (lane // 16) % 2, lane % 16

    def half(offsets, second):
        q = (quarter + 2 * second) % 4
        return np.array(offsets)[q] + 128 * (hb ^ second) + 8 * j

    l1, u1 = half((1, 2, 3, 4), 0), half((5, 6, 7, 8), 1)
    l2, u2 = half((258, 260, 516, 772), 0), half((262, 264, 520, 776), 1)
    l3, u3 = half((1032, 1288) * 2, 0), half((1544, 1800) * 2, 1)
    lags = [np.where(hb == 0, l1, u1), np.where(hb == 0, u1, l1),
            np.where(lane < 64, l2, u2), np.where(lane < 64, u2, l2), np.where(lane < 64, l3, u3)]
    lags.append(np.where(lane // 16 == 0, half((516,) * 4, 0),
                         np.where(lane // 16 == 5, half((520,) * 4, 1), lags[2])))
    lags.append(np.where(lane < 96, lags[3], lags[2]))
    lags.append(np.where(lane < 32, lags[4], lags[3]))
    return lags


_SRC = ((0,), (0, 1), (1, 2), (2,), (5,), (6,), (3,), (3,), (7,), (7,)) + ((4,),) * 6


@functools.cache
def _tables():
    k = np.arange(P)
    phi = 2 * np.pi * (k + 0.25) / P

    def coords(m):
        z = np.exp(1j * np.outer(m, phi))
        return np.concatenate([z.real + z.imag / np.sqrt(3), 2 * z.imag / np.sqrt(3)], axis=1)

    fu = 2.0 * coords(np.arange(P))
    zi = np.exp(-1j * np.outer(phi, np.arange(P)))
    fi = np.concatenate([zi.real, (np.exp(2j * np.pi / 3) * zi).real], axis=0) / P
    lags = _tile_lags()
    groups, layout = [], []
    for j, src in enumerate(_SRC):
        m = np.arange(-P + 1 + (j == 3), P)
        m = m[P * j + m >= 1]
        rl = _round_bf16(P * j + m)
        hit = np.zeros(len(m), int)
        layout.append([])
        for t in src:
            sel = (lags[t][:, None] == rl[None, :])
            hit += sel.sum(0)
            g = _pack_rows(sel.astype(np.float64) @ coords(m))
            ids = []
            for r in range(0, P // 2, 8):
                known = [n for n, e in enumerate(groups) if np.array_equal(e, g[r:r + 8])]
                if not sel[2 * r:2 * r + 16].any():
                    ids.append(None)
                elif known:
                    ids.append(known[0])
                else:
                    ids.append(len(groups))
                    groups.append(g[r:r + 8])
            layout[-1].append(ids)
        assert (hit == 1).all()
    edge = np.broadcast_to(coords(np.array([-P + 1])).astype(np.float32), (8, 2 * P)).view(np.uint32)
    return _pack_rows(fu), _pack_rows(fi), np.stack(groups + [edge]), layout


def _cmul(a, b):
    return (a[0] * b[0] - a[1] * b[1], a[0] * b[1] + a[1] * b[0])


def _csq(a):
    t = a[0] * a[1]
    return ((a[0] - a[1]) * (a[0] + a[1]), t + t)


def _dot(a, b):
    return jax.lax.dot_general(a, b, (((1,), (0,)), ((), ())), preferred_element_type=F32)


def _dot_nt(a, b):
    return jax.lax.dot_general(a, b, (((1,), (1,)), ((), ())), preferred_element_type=F32)


def _rbf(x):
    return x.astype(BF16).astype(F32)


def _interleave(*gens):
    state = [[0.0, k, g, total] for k, (g, total) in enumerate(gens)]
    while state:
        cur = min(state, key=lambda e: (e[0], e[1]))
        w = next(cur[2], None)
        if w is None:
            state.remove(cur)
        else:
            cur[0] += w / cur[3]


def _zip(*gens):
    _interleave(*((g, 1.0) for g in gens))


_ZP = (1, 8, 32, 256)


def _kernel(x_hbm, are_hbm, aim_hbm, bre_hbm, bim_hbm, cre_hbm, cim_hbm, ldt_hbm, dsk_hbm,
            wr_hbm, wg_hbm, wu_hbm, wd_hbm, fu_hbm, fi_hbm, g_hbm, o_hbm,
            ldt_v, dsk_v, wr_v, x_v, prm_v, wg_v, wu_v, wd_v, fu_v, fi_v, g_v, o_v, d_v, h_v, s_v,
            kc_v, dt_v, row_v, oh_v, act_v, hat_v, p_v, yt_v, yu_v, sems, psem, osem,
            *, GS, GA, GD, NG, NF, GE, GT, LD, CS, UB, SC, EO, debug):
    scope = jax.named_scope if SC else (lambda _: contextlib.nullcontext())
    D, L = x_v.shape
    FF = wg_v.shape[1]
    NB = L // P
    FC = FF // NF
    ND = D // GD
    NL = ND - 1 - NG - NF
    tails = ((NL * GE, D - GD - NL * GE),) + tuple((r, GT) for r in range(D - GD, D, GT))
    layout = _tables()[3]

    def span(i, n):
        start = i * n
        if not isinstance(start, int):
            start = pl.multiple_of(start, n)
        return pl.ds(start, n)

    prm_hbm = (are_hbm, aim_hbm, bre_hbm, bim_hbm, cre_hbm, cim_hbm)

    def cprm(part, k):
        r = pl.ds(0, 3 * GS) if part == 0 else pl.ds(3 * GS, D - 3 * GS)
        return pltpu.make_async_copy(prm_hbm[k].at[r], prm_v.at[k, r], psem.at[6 * part + k])

    cx, cfu, cfi, cg, *cvec = (
        pltpu.make_async_copy(src, dst, sems.at[k]) for k, (src, dst) in enumerate((
            (x_hbm, x_v), (fu_hbm, fu_v), (fi_hbm, fi_v), (g_hbm, g_v),
            (ldt_hbm, ldt_v), (dsk_hbm, dsk_v), (wr_hbm, wr_v))))

    def cwg(i):
        return pltpu.make_async_copy(wg_hbm.at[:, span(i, FC)], wg_v.at[:, span(i, FC)], sems.at[7 + i])

    def cwu(i):
        return pltpu.make_async_copy(wu_hbm.at[:, span(i, FC)], wu_v.at[:, span(i, FC)], sems.at[7 + NF + i])

    def out_rows(i):
        if isinstance(i, int) and i >= NL:
            return pl.ds(*tails[i - NL])
        return pl.ds(i * GE if isinstance(i, int) else pl.multiple_of(i * GE, 16), GE)

    def cwd(i):
        return pltpu.make_async_copy(wd_hbm.at[out_rows(i)], wd_v.at[out_rows(i)], sems.at[7 + 2 * NF + i])

    def cout(i):
        return pltpu.make_async_copy(o_v.at[out_rows(i)], o_hbm.at[out_rows(i)], osem.at[i])

    for c in cvec:
        c.start()
    for k in range(6):
        cprm(0, k).start()

    @pl.loop(0, NF)
    def _(i):
        cwg(i).start(priority=1)
        cwu(i).start(priority=1)

    @pl.loop(0, NL)
    def _(i):
        cwd(i).start(priority=1)

    for i in range(len(tails)):
        cwd(NL + i).start(priority=1)

    for k in range(6):
        cprm(1, k).start()
    for c in cvec:
        c.wait()

    dt_row = _rbf(jnp.exp(ldt_v[...].astype(F32)[None, :]))
    dsk_row = dsk_v[...].astype(F32)[None, :] * (1.0 / P)
    for c0 in range(0, D, P):
        n = min(P, D - c0)
        eye = (jax.lax.broadcasted_iota(jnp.int32, (n, n), 0) == jax.lax.broadcasted_iota(jnp.int32, (n, n), 1))
        for k, row in enumerate((dt_row, dsk_row)):
            dt_v[k, c0:c0 + n, :] = _dot(jnp.where(eye, row[:, c0:c0 + n], 0.0), jnp.ones((n, P), BF16))

    lane8 = jax.lax.broadcasted_iota(jnp.int32, (8, P), 1)
    sub8 = jax.lax.broadcasted_iota(jnp.int32, (8, P), 0)

    def k_setup(i, _):
        @pl.when(i == 3)
        def _():
            for k in range(6):
                cprm(1, k).wait()

        low = sub8 < 4
        for g in range(GS // 16):
            sl = slice(16 * g, 16 * g + 16)
            dt, dsk = (dt_v.at[k, span(i, GS)][sl, :] for k in range(2))
            a_re, a_im, b_re, b_im, c_re, c_im = (prm_v.at[k, span(i, GS)][sl, :].astype(F32) for k in range(6))
            dst = p_v.at[:, span(i, GS)]
            w = {0: _cmul((c_re, c_im), (dt * b_re, dt * b_im))}
            mag = jnp.exp(dt * a_re)
            z = {1: (mag * jnp.cos(dt * a_im), mag * jnp.sin(dt * a_im))}
            for e in range(10):
                z[2 << e] = _csq(z[1 << e])
            for n, e in enumerate(_ZP):
                for q in range(2):
                    dst[2 * n + q, sl, :] = z[e][q]
            dst[24, sl, :] = w[0][0] + dsk
            dst[25, sl, :] = w[0][0] * z[256][0] - w[0][1] * z[256][1]
            w[4], w[8] = _cmul(w[0], z[4]), _cmul(w[0], z[8])
            w[1032] = _cmul(w[8], z[1024])
            w[1544] = _cmul(w[1032], z[512])
            one = (jnp.ones((16, P), F32), jnp.zeros((16, P), F32))
            for n, (a, b) in enumerate(((one, z[128]), (w[0], w[4]), (w[4], w[8]), (w[1032], w[1544]))):
                for q in range(2):
                    for t in range(2):
                        x, y = a[q][8 * t:8 * t + 8], pltpu.roll(b[q][8 * t:8 * t + 8], 4, 0)
                        r = slice(16 * g + 8 * t, 16 * g + 8 * t + 8)
                        dst[8 + 4 * n + q, r, :] = jnp.where(low, x, y)
                        dst[10 + 4 * n + q, r, :] = jnp.where(low, y, x)
        return 0

    def k_lags(i, _):
        low = sub8 < 4
        bit4, bit5, bit6 = ((lane8 & b) == 0 for b in (16, 32, 64))
        bit6x = ((lane8 >> 4) ^ sub8) & 4 == 0
        diag = (lane8 & 15) * 8 + (((lane8 >> 2) & 4) ^ sub8)
        src, dst = p_v.at[:, span(i, GA)], kc_v.at[:, span(i, GA)]
        for g in range(GA // 8):
            sl = slice(8 * g, 8 * g + 8)
            out = []
            for h in range(2):
                off = (4 if h else 0) if g + 1 < GA // 8 else (0 if h else -4)
                z = {e: tuple(jnp.take_along_axis(src[2 * n + q, 8 * g + off:8 * g + off + 8, :],
                                                  (sub8 & 3) + (4 * h - off), axis=0,
                                                  mode="promise_in_bounds") for q in range(2))
                     for n, e in enumerate(_ZP)}
                b0, r, a4, far = (tuple(src[8 + 4 * n + 2 * h + q, sl, :] for q in range(2)) for n in range(4))
                bs = [b0]
                for j in range(1, 16):
                    bs.append(_cmul(bs[j - 1], z[8]) if j < 4 else _cmul(bs[j - 4], z[32]))
                av = [_cmul(r, z[1])]
                av += [_cmul(av[0], z[1])]
                av += [_cmul(av[1], z[1]), a4, _cmul(av[1], z[256]), _cmul(a4, z[256])]
                av.append(_cmul(av[-1], z[256]))
                av.append(_cmul(av[-1], z[256]))
                av += [far, _cmul(far, z[256])]
                out.append([_dot_nt(jnp.concatenate([v[q] for v in av], axis=0),
                                    jnp.concatenate([v[q] for v in reversed(bs)], axis=0).astype(BF16))
                            for q in range(2)])
            d = [[out[h][0][8 * n:8 * n + 8] - out[h][1][8 * n:8 * n + 8] for n in range(10)] for h in range(2)]
            v = [[None] * 10, [None] * 10]
            for n in range(10):
                for h in range(2):
                    v[h][n] = jnp.take_along_axis(d[h][n], diag ^ 120, axis=1, mode="promise_in_bounds")

            def unzip(xs):
                return jnp.where(low, xs[0], xs[1]), pltpu.roll(jnp.where(low, xs[1], xs[0]), 4, 0)

            halves = []
            for lo, hi in ((0, 4), (4, 8), (8, 10)):
                xs = []
                for h in range(2):
                    u = [jnp.where(bit5, v[h][n], v[h][n + 1]) for n in range(lo, hi, 2)]
                    xs.append(jnp.where(bit6x, u[h], u[1 - h]) if len(u) == 2 else u[0])
                halves.append(unzip(xs))
            (l1, u1), (l2, u2), (l3, u3) = halves
            l6, u6 = unzip((v[0][6], v[1][6]))
            tiles = [jnp.where(bit4, l1, u1), jnp.where(bit4, u1, l1), jnp.where(bit6, l2, u2),
                     jnp.where(bit6, u2, l2), jnp.where(bit6, l3, u3)]
            tiles.append(jnp.where(lane8 < 16, l6, jnp.where((lane8 >> 4) == 5, u6, tiles[2])))
            tiles.append(jnp.where(lane8 < 96, tiles[3], tiles[2]))
            tiles.append(jnp.where(lane8 < 32, tiles[4], tiles[3]))
            for t, tile in enumerate(tiles):
                dst[t, sl, :] = tile
        return 0

    with scope("setup"):
        for k in range(6):
            cprm(0, k).wait()
        for c in (cx, cg, cfu, cfi):
            c.start()
        jax.lax.fori_loop(0, D // GS, k_setup, 0)
    with scope("lags"):
        jax.lax.fori_loop(0, D // GA, k_lags, 0)

    LB, RB, HB = 2 * P, 96, h_v.shape[2]

    def col_sum(parts):
        acc = [functools.reduce(jnp.add, parts[k::4]) for k in range(4)]
        return (acc[0] + acc[1]) + (acc[2] + acc[3])

    def ln_sum(i, _):
        src = x_v.at[span(i, RB)]
        acc = row_v[0]
        for r in range(0, RB, 8):
            acc = acc + src[r:r + 8, :].astype(F32)
        row_v[0] = acc
        return 0

    def ln_centre(c, _):
        src, dst = x_v.at[:, span(c, LB)], d_v.at[:, span(c, LB)]
        rows = span(c, D * LB // L)
        for t in range(2):
            kc_v[8 + t, rows, :] = jnp.broadcast_to(
                jnp.sum(p_v[24 + t, rows, :], axis=1, keepdims=True), (rows.size, P))
        mb = row_v[0, :, span(c, LB)]
        acc = [0.0] * 4
        for r in range(0, D, 8):
            d = src[r:r + 8, :].astype(F32) - mb
            dst[r:r + 8, :] = d.astype(BF16)
            acc[r // 8 % 4] += d * d
        row_v[1, :, span(c, LB)] = col_sum(acc)
        return 0

    def ln_scale(c):
        src, inv = d_v.at[:, span(c, HB)], row_v[0, :, span(c, HB)]
        for r in range(0, D, 8):
            h_v[c, r:r + 8, :] = (src[r:r + 8, :].astype(F32) * inv).astype(BF16)

    def ln_route(c, _):
        oh_v[:, span(c, HB)] = _dot(wr, h_v[c])
        ln_scale(c + 1)
        return 0

    def h_block(rows, c):
        return h_v[c * P // HB, rows, c * P % HB:c * P % HB + P]

    def compact(v):
        return jnp.concatenate([functools.reduce(
            lambda a, q: jnp.where(sub8 == q, v[:, (c + q) * P:(c + q + 1) * P], a),
            range(1, 8), v[:, c * P:(c + 1) * P]) for c in range(0, NB, 8)], axis=0)

    def spread(v):
        return jnp.concatenate([jnp.broadcast_to(v[c:c + 1], (8, P)) for c in range(NB)], axis=1)

    def total(k):
        return compact(jnp.broadcast_to(jnp.sum(row_v[k], axis=0, keepdims=True), (8, L)))

    with scope("lnorm"):
        for c in (cx, cg, cfu, cfi):
            c.wait()
        row_v[0] = jnp.zeros((8, L), F32)
        jax.lax.fori_loop(0, D // RB, ln_sum, 0)
        m = total(0) / D
        mb = _rbf(m)
        row_v[0] = spread(mb)
        jax.lax.fori_loop(0, L // LB, ln_centre, 0)
        var = jnp.maximum(total(1) / D - (m - mb) * (m - mb), 0.0)
        row_v[0] = spread(0.5 / _rbf(jnp.sqrt(_rbf(_rbf(var) + _rbf(jnp.full_like(var, 1e-5))))))
        wr = jnp.broadcast_to(2.0 * wr_v[...].astype(F32)[None, :], (8, D))
        ln_scale(0)
        jax.lax.fori_loop(0, L // HB - 1, ln_route, 0)
        oh_v[:, L - HB:] = _dot(wr, h_v[L // HB - 1])

    def put(dst, kind, c, g, a, b):
        for q, v in enumerate((a, b, a - b)):
            hat_v[dst, 3 * kind + q, c, 8 * g:8 * g + 8, :] = v

    def c_signal(src, dst, c0, n):
        lhs = jnp.concatenate([h_block(span(src, GD), c) for c in range(c0, c0 + n)], axis=0)
        uh = _dot(lhs, pltpu.bitcast(fu_v[...], BF16))
        for c in range(n):
            for g in range(GD // 8):
                r = slice(c * GD + 8 * g, c * GD + 8 * g + 8)
                put(dst, 0, c0 + c, g, uh[r, :P], uh[r, P:])
                yield 1

    def c_window(src, dst, j):
        tiles = kc_v.at[:, span(src, GD)]
        kh = None
        for t, ids in zip(_SRC[j], layout[j]):
            rhs = jnp.concatenate([jnp.zeros((8, 2 * P), jnp.uint32) if n is None else g_v[n] for n in ids], axis=0)
            part = _dot(tiles[t], pltpu.bitcast(rhs, BF16))
            kh = part if kh is None else kh + part
        for g in range(GD // 8):
            sl = slice(8 * g, 8 * g + 8)
            a, b = kh[sl, :P], kh[sl, P:]
            if j == 0:
                a = a + tiles[8, sl, :]
            if j == 3:
                edge = pltpu.bitcast(g_v[g_v.shape[0] - 1], F32)
                a, b = a + tiles[9, sl, :] * edge[:, :P], b + tiles[9, sl, :] * edge[:, P:]
            put(dst, 1, j, g, a, b)
            yield 1

    def c_inverse(i, c0, n, r0=0, m=GD):
        lhs = jnp.concatenate([jnp.concatenate([hat_v[i, 6 + q, c, r0:r0 + m, :] for q in range(2)], axis=1)
                               for c in range(c0, c0 + n)], axis=0)
        y = _dot(lhs, pltpu.bitcast(fi_v[...], BF16))
        for c in range(n):
            for r in range(0, m, 8):
                s_v.at[span(i, GD)][r0 + r:r0 + r + 8, (c0 + c) * P:(c0 + c + 1) * P] = y[c * m + r:c * m + r + 8]
                yield 1

    window_pairs = ((14, 15), (12, 13), (10, 11), (8, 9), (6, 7), (4, 5), (0, 3), (1, 2))

    def c_transforms(i):
        nxt = i + 1
        for c0 in range(0, NB, UB):
            _zip(c_signal(nxt, i + 1, c0, UB), c_inverse(i, c0, UB))
            yield UB
            for pair in window_pairs[c0 // 2:(c0 + UB) // 2]:
                _zip(*(c_window(nxt, i + 1, j) for j in pair))
                yield len(_SRC[pair[0]])

    def c_product(i, groups=range(GD // 8)):
        for g in groups:
            sl = slice(8 * g, 8 * g + 8)
            for cs in (range(8, 16), range(8)):
                m0 = {}
                for q in range(3):
                    acc = dict(m0)
                    for j in reversed(range(max(cs) + 1)):
                        k = hat_v[i, 3 + q, j, sl, :]
                        live = [c for c in cs if c >= j]
                        for c in live:
                            t = k * hat_v[i, q, c - j, sl, :]
                            acc[c] = t if c not in acc else (acc[c] - t if q else acc[c] + t)
                        yield len(live)
                    if q == 0:
                        m0 = acc
                    else:
                        for c in cs:
                            hat_v[i + 1, 5 + q, c, sl, :] = acc[c]

    def c_step(i, pace, *extra):
        _interleave((c_product(i), GD // 8 * 3 * 136), (c_transforms(i), 25 * pace), *extra)

    with scope("topk"):
        r = _rbf(compact(oh_v[...]))
        bits = pltpu.bitcast(jnp.where(r == 0.0, 0.0, r), jnp.int32)
        ordered = jnp.where(bits < 0, ~bits, bits ^ jnp.int32(-2**31))
        idx = (jax.lax.broadcasted_iota(jnp.int32, (NB, P), 0) * P
               + jax.lax.broadcasted_iota(jnp.int32, (NB, P), 1))
        key = pltpu.bitcast((jax.lax.shift_right_logical(ordered, 16) << 11) + (0x20000000 + L - 1 - idx), F32)
        rest, top = key, jnp.zeros((8, P), F32)
        for q in range(8):
            mx = jnp.max(jnp.max(rest, axis=0, keepdims=True), axis=1, keepdims=True)
            top = jnp.where(sub8 == q, mx, top)
            rest = jnp.where(rest == mx, 0.0, rest)
        _zip(c_signal(0, 0, 0, NB // 2), c_signal(0, 0, NB // 2, NB // 2))
        for pair in window_pairs:
            _zip(*(c_window(0, 0, j) for j in pair))
        hat_v[0, 6:8] = jnp.zeros((2,) + hat_v.shape[2:], F32)
        oh_v[...] = jnp.where(spread(key) == jnp.concatenate([top] * NB, axis=1), 1.0, 0.0)
        o16 = jax.lax.shift_right_logical(pltpu.bitcast(top, jnp.int32) - 0x20000000, 11) << 16
        r_top = pltpu.bitcast(jnp.where(o16 < 0, o16 ^ jnp.int32(-2**31), (~o16) & jnp.int32(-65536)), F32)
        gate = 0.5 * jax.nn.sigmoid(r_top)

    def gather_step(i, acc):
        n = L // NG
        oh = oh_v.at[:, span(i, n)]
        parts = []

        def gather():
            for r in range(0, D, P):
                part = 0.0
                for c0 in range(0, n, 4 * P):
                    yield 0.5
                    part = part + functools.reduce(jnp.add, [
                        _dot_nt(oh[:, c:c + P], h_v[i * (n // HB) + c // HB, r:min(r + P, D), c % HB:c % HB + P]) for c in range(c0, c0 + 4 * P, P)])
                    yield 0.5
                parts.append(part)

        c_step(i, CS[0], (gather(), n // (4 * P) * 5 * CS[0]))
        return acc + jnp.concatenate(parts, axis=1)

    with scope("conv0"):
        x_sel = 2.0 * jax.lax.fori_loop(0, NG, gather_step, jnp.zeros((8, D), F32))
        row_v[0, :, :D] = x_sel

    def gate_up_step(item, _):
        i = item - NG
        ws, dst = (wg_v.at[:, span(i, FC)], wu_v.at[:, span(i, FC)]), act_v.at[:, :, span(i, FC)]

        def gate_up():
            for c in range(0, FC, 2 * P):
                acc = [0.0, 0.0]
                for r in range(0, D, P):
                    yield 0.5
                    rs = slice(r, min(r + P, D))
                    acc = [a + _dot(row_v[0, :, rs], w[rs, c:c + 2 * P]) for a, w in zip(acc, ws)]
                    yield 0.5
                for k in range(2):
                    dst[k, :, c:c + 2 * P] = acc[k]

        c_step(item, CS[1], (gate_up(), FC // (2 * P) * 5 * CS[1]))

        @pl.when(i + 1 < NF)
        def _():
            cwg(i + 1).wait()
            cwu(i + 1).wait()

        return 0

    with scope("conv1"):
        cwg(0).wait()
        cwu(0).wait()
        jax.lax.fori_loop(NG, NG + NF, gate_up_step, 0)
        a = 0.5 * act_v[0]
        act_v[0] = (a + a * jnp.tanh(a)) * act_v[1]

    def project(rows, lead, res):
        n = rows.size
        w = wd_v.at[rows]
        acc = 0.0
        for c in range(0, FF, 4 * P):
            yield 0.5
            acc = acc + functools.reduce(jnp.add, [
                _dot_nt(act_v[0, :, f:f + P], w[:, f:f + P]) for f in range(c, c + 4 * P, P)])
            yield 0.5
        yield lead
        eye = jax.lax.broadcasted_iota(jnp.int32, (n, n), 0) == jax.lax.broadcasted_iota(jnp.int32, (n, n), 1)
        res.append(_dot_nt(eye.astype(F32), acc * gate[:, :n]))
        yield lead

    def emit(e, yt):
        rows = out_rows(e)
        h = jnp.concatenate([h_v[c, rows, :].astype(F32) for c in range(L // HB)], axis=1) + _dot(yt, oh_v[...])
        s = s_v.at[GD:][rows, :]
        q = s * h
        out = (x_v[rows, :].astype(F32) + q) + q * jnp.tanh(h)
        if debug:
            out = s
        o_v[rows, :] = out.astype(o_v.dtype)
        cout(e).start()

    NP = FF // (4 * P) + 2 * LD

    def inverse_all(i, step, *rows):
        for c0 in range(0, NB, 2 * step):
            _zip(c_inverse(i, c0, step, *rows), c_inverse(i, c0 + step, step, *rows))
            yield 2 * step

    def finish_step(item, _):
        e = item - (NG + NF)

        @pl.when(e < NL)
        def _():
            yt = []
            c_step(item, CS[2], (project(out_rows(e), LD, yt), NP * CS[2]))
            emit(e, yt[0])

            @pl.when(e + 1 < NL)
            def _():
                cwd(e + 1).wait()

            @pl.when(e + 1 == NL)
            def _():
                for i in range(len(tails)):
                    cwd(NL + i).wait()

        @pl.when(e == NL)
        def _():
            yt = ([], [])
            _interleave((c_product(item), GD // 8 * 3 * 136), (inverse_all(item, 1), NB * CS[3]),
                        (project(out_rows(NL), LD, yt[0]), NP * CS[3]),
                        (project(pl.ds(D - GD, GD), LD, yt[1]), NP * CS[3]))
            yt_v[...] = yt[1][0]
            if EO:
                emit(NL, yt[0][0])
            else:
                yu_v[...] = yt[0][0]

        return 0

    with scope("conv2"):
        cwd(0).wait()
        jax.lax.fori_loop(NG + NF, ND, finish_step, 0)

    with scope("tail"):
        if not EO:
            emit(NL, yu_v[...])
        for n in range(GD // GT):
            _zip(inverse_all(ND, NB // 2, n * GT, GT))
            emit(NL + 1 + n, yt_v[n * GT:(n + 1) * GT, :])
        for e in range(NL + len(tails)):
            cout(e).wait()


def run(A_u, A_A_re, A_A_im, A_B_re, A_B_im, A_C_re, A_C_im, A_log_dt, A_Dskip, B_x, B_w_r,
        B_w_gate, B_w_up, B_w_down, GS=64, GA=192, GD=64, NG=2, NF=3, GE=128, GT=64, LD=2.0, CS=(1.1, 1.1, 1.0, 1.05), UB=1, SC=0, EO=1,
        debug=False, interpret=False, flags=None, DS=True):
    _, L, D = A_u.shape
    FF = B_w_gate.shape[1]
    fu, fi, g = _tables()[:3]
    odt = F32 if debug else A_u.dtype
    hbm = pl.BlockSpec(memory_space=pl.ANY)
    NB = L // P
    NE = D // GD - NG - NF + GD // GT
    out = pl.pallas_call(
        functools.partial(_kernel, GS=GS, GA=GA, GD=GD, NG=NG, NF=NF, GE=GE, GT=GT, LD=LD, CS=CS, UB=UB, SC=SC, EO=EO, debug=debug),
        out_shape=jax.ShapeDtypeStruct((D, L), odt),
        in_specs=[hbm] * 16,
        out_specs=hbm,
        scratch_shapes=[
            *[pltpu.VMEM((D,), BF16)] * 3,
            pltpu.VMEM((D, L), BF16), pltpu.VMEM((6, D, P), BF16),
            pltpu.VMEM((D, FF), BF16), pltpu.VMEM((D, FF), BF16), pltpu.VMEM((D, FF), BF16),
            pltpu.VMEM(fu.shape, jnp.uint32), pltpu.VMEM(fi.shape, jnp.uint32),
            pltpu.VMEM(g.shape, jnp.uint32),
            pltpu.VMEM((D, L), odt), pltpu.VMEM((D, L), BF16), pltpu.VMEM((4, D, L // 4), BF16),
            pltpu.VMEM((D + GD, L), F32),
            pltpu.VMEM((10, D, P), F32), pltpu.VMEM((2, D, P), F32),
            pltpu.VMEM((2, 8, L), F32), pltpu.VMEM((8, L), F32), pltpu.VMEM((2, 8, FF), F32),
            pltpu.VMEM((D // GD + 1, 8, NB, GD, P), F32),
            pltpu.VMEM((26, D, P), F32), pltpu.VMEM((GD, 8), F32), pltpu.VMEM((128, 8), F32),
            pltpu.SemaphoreType.DMA((7 + 2 * NF + NE,)),
            pltpu.SemaphoreType.DMA((12,)),
            pltpu.SemaphoreType.DMA((NE,)),
        ],
        compiler_params=pltpu.CompilerParams(vmem_limit_bytes=112 * 2**20, flags=flags, disable_semaphore_checks=DS, disable_bounds_checks=DS),
        interpret=interpret,
        name="ssm_moe",
    )(A_u[0].T, A_A_re, A_A_im, A_B_re, A_B_im, A_C_re, A_C_im, A_log_dt, A_Dskip, B_w_r,
      B_w_gate, B_w_up, B_w_down.T, fu, fi, g)
    return out.T[None]


@jax.jit
def pallas_recurrent_scan__ssm_conv_s4__moe_arch_mod__prompt_kernel(
    A_u: jax.Array,
    A_A_re: jax.Array,
    A_A_im: jax.Array,
    A_B_re: jax.Array,
    A_B_im: jax.Array,
    A_C_re: jax.Array,
    A_C_im: jax.Array,
    A_log_dt: jax.Array,
    A_Dskip: jax.Array,
    B_x: jax.Array,
    B_w_r: jax.Array,
    B_w_gate: jax.Array,
    B_w_up: jax.Array,
    B_w_down: jax.Array,
):
    return run(A_u, A_A_re, A_A_im, A_B_re, A_B_im, A_C_re, A_C_im, A_log_dt, A_Dskip, B_x,
               B_w_r, B_w_gate, B_w_up, B_w_down)
```

```python
import contextlib
import functools

import jax
import jax.numpy as jnp
import numpy as np
import jax.experimental.pallas as pl
import jax.experimental.pallas.tpu as pltpu

F32 = jnp.float32
BF16 = jnp.bfloat16
P = 128


def _bf16_bits(a):
    u = np.ascontiguousarray(a, dtype=np.float32).view(np.uint32)
    return ((u + 0x7FFF + ((u >> 16) & 1)) >> 16).astype(np.uint32)


def _round_bf16(a):
    return (_bf16_bits(a) << 16).view(np.float32)


def _pack_rows(a):
    b = _bf16_bits(a)
    return (b[0::2] | (b[1::2] << 16)).astype(np.uint32)


def _tile_lags():
    lane = np.arange(P)
    quarter, hb, j = lane // 32, (lane // 16) % 2, lane % 16

    def half(offsets, second):
        q = (quarter + 2 * second) % 4
        return np.array(offsets)[q] + 128 * (hb ^ second) + 8 * j

    l1, u1 = half((1, 2, 3, 4), 0), half((5, 6, 7, 8), 1)
    l2, u2 = half((258, 260, 516, 772), 0), half((262, 264, 520, 776), 1)
    l3, u3 = half((1032, 1288) * 2, 0), half((1544, 1800) * 2, 1)
    lags = [np.where(hb == 0, l1, u1), np.where(hb == 0, u1, l1),
            np.where(lane < 64, l2, u2), np.where(lane < 64, u2, l2), np.where(lane < 64, l3, u3)]
    lags.append(np.where(lane // 16 == 0, half((516,) * 4, 0),
                         np.where(lane // 16 == 5, half((520,) * 4, 1), lags[2])))
    lags.append(np.where(lane < 96, lags[3], lags[2]))
    lags.append(np.where(lane < 32, lags[4], lags[3]))
    return lags


_SRC = ((0,), (0, 1), (1, 2), (2,), (5,), (6,), (3,), (3,), (7,), (7,)) + ((4,),) * 6


@functools.cache
def _tables():
    k = np.arange(P)
    phi = 2 * np.pi * (k + 0.25) / P

    def coords(m):
        z = np.exp(1j * np.outer(m, phi))
        return np.concatenate([z.real + z.imag / np.sqrt(3), 2 * z.imag / np.sqrt(3)], axis=1)

    fu = 2.0 * coords(np.arange(P))
    zi = np.exp(-1j * np.outer(phi, np.arange(P)))
    fi = np.concatenate([zi.real, (np.exp(2j * np.pi / 3) * zi).real], axis=0) / P
    lags = _tile_lags()
    groups, layout = [], []
    for j, src in enumerate(_SRC):
        m = np.arange(-P + 1 + (j == 3), P)
        m = m[P * j + m >= 1]
        rl = _round_bf16(P * j + m)
        hit = np.zeros(len(m), int)
        layout.append([])
        for t in src:
            sel = (lags[t][:, None] == rl[None, :])
            hit += sel.sum(0)
            g = _pack_rows(sel.astype(np.float64) @ coords(m))
            ids = []
            for r in range(0, P // 2, 8):
                known = [n for n, e in enumerate(groups) if np.array_equal(e, g[r:r + 8])]
                if not sel[2 * r:2 * r + 16].any():
                    ids.append(None)
                elif known:
                    ids.append(known[0])
                else:
                    ids.append(len(groups))
                    groups.append(g[r:r + 8])
            layout[-1].append(ids)
        assert (hit == 1).all()
    edge = np.broadcast_to(coords(np.array([-P + 1])).astype(np.float32), (8, 2 * P)).view(np.uint32)
    return _pack_rows(fu), _pack_rows(fi), np.stack(groups + [edge]), layout


def _cmul(a, b):
    return (a[0] * b[0] - a[1] * b[1], a[0] * b[1] + a[1] * b[0])


def _csq(a):
    t = a[0] * a[1]
    return ((a[0] - a[1]) * (a[0] + a[1]), t + t)


def _dot(a, b):
    return jax.lax.dot_general(a, b, (((1,), (0,)), ((), ())), preferred_element_type=F32)


def _dot_nt(a, b):
    return jax.lax.dot_general(a, b, (((1,), (1,)), ((), ())), preferred_element_type=F32)


def _rbf(x):
    return x.astype(BF16).astype(F32)


def _interleave(*gens):
    state = [[0.0, k, g, total] for k, (g, total) in enumerate(gens)]
    while state:
        cur = min(state, key=lambda e: (e[0], e[1]))
        w = next(cur[2], None)
        if w is None:
            state.remove(cur)
        else:
            cur[0] += w / cur[3]


def _merge(*gens):
    state = [[0.0, k, g, total, cost] for k, (g, total, cost) in enumerate(gens)]
    while state:
        cur = min(state, key=lambda e: (e[0], e[1]))
        w = next(cur[2], None)
        if w is None:
            state.remove(cur)
        else:
            cur[0] += w / cur[3]
            yield w * cur[4]


def _zip(*gens):
    _interleave(*((g, 1.0) for g in gens))


_ZP = (1, 8, 32, 256)


def _kernel(x_hbm, are_hbm, aim_hbm, bre_hbm, bim_hbm, cre_hbm, cim_hbm, ldt_hbm, dsk_hbm,
            wr_hbm, wg_hbm, wu_hbm, wd_hbm, fu_hbm, fi_hbm, g_hbm, o_hbm,
            ldt_v, dsk_v, wr_v, x_v, prm_v, wg_v, wu_v, wd_v, fu_v, fi_v, g_v, o_v, d_v, h_v, s_v,
            kc_v, dt_v, row_v, oh_v, act_v, hat_v, p_v, yt_v, yu_v, sems, psem, osem,
            *, GS, GA, GD, NG, NF, GE, GT, LD, CS, UB, SC, G0, LI, WF, GX, debug):
    scope = jax.named_scope if SC else (lambda _: contextlib.nullcontext())
    D, L = x_v.shape
    FF = wg_v.shape[1]
    NB = L // P
    FC = FF // NF
    ND = D // GD
    NL = ND - 1 - NG - NF
    tails = ((NL * GE, D - GD - NL * GE),) + tuple((r, GT) for r in range(D - GD, D, GT))
    layout = _tables()[3]

    def span(i, n):
        start = i * n
        if not isinstance(start, int):
            start = pl.multiple_of(start, n)
        return pl.ds(start, n)

    prm_hbm = (are_hbm, aim_hbm, bre_hbm, bim_hbm, cre_hbm, cim_hbm)

    def cprm(part, k):
        r = pl.ds(0, GS) if part == 0 else pl.ds(GS, D - GS)
        return pltpu.make_async_copy(prm_hbm[k].at[r], prm_v.at[k, r], psem.at[6 * part + k])

    cx, cfu, cfi, cg, *cvec = (
        pltpu.make_async_copy(src, dst, sems.at[k]) for k, (src, dst) in enumerate((
            (x_hbm, x_v), (fu_hbm, fu_v), (fi_hbm, fi_v), (g_hbm, g_v),
            (ldt_hbm, ldt_v), (dsk_hbm, dsk_v), (wr_hbm, wr_v))))

    def cwg(i):
        return pltpu.make_async_copy(wg_hbm.at[:, span(i, FC)], wg_v.at[:, span(i, FC)], sems.at[7 + i])

    def cwu(i):
        return pltpu.make_async_copy(wu_hbm.at[:, span(i, FC)], wu_v.at[:, span(i, FC)], sems.at[7 + NF + i])

    def out_rows(i):
        if isinstance(i, int) and i >= NL:
            return pl.ds(*tails[i - NL])
        return pl.ds(i * GE if isinstance(i, int) else pl.multiple_of(i * GE, 16), GE)

    def cwd(i):
        return pltpu.make_async_copy(wd_hbm.at[out_rows(i)], wd_v.at[out_rows(i)], sems.at[7 + 2 * NF + i])

    def cout(i):
        return pltpu.make_async_copy(o_v.at[out_rows(i)], o_hbm.at[out_rows(i)], osem.at[i])

    for c in cvec:
        c.start()
    for k in range(6):
        cprm(0, k).start()

    @pl.loop(0, NF)
    def _(i):
        cwg(i).start(priority=1)
        cwu(i).start(priority=1)

    @pl.loop(0, NL)
    def _(i):
        cwd(i).start(priority=1)

    for i in range(len(tails)):
        cwd(NL + i).start(priority=1)

    for k in range(6):
        cprm(1, k).start()
    for c in cvec:
        c.wait()

    dt_row = _rbf(jnp.exp(ldt_v[...].astype(F32)[None, :]))
    dsk_row = dsk_v[...].astype(F32)[None, :] * (1.0 / P)
    for c0 in range(0, D, P):
        n = min(P, D - c0)
        eye = (jax.lax.broadcasted_iota(jnp.int32, (n, n), 0) == jax.lax.broadcasted_iota(jnp.int32, (n, n), 1))
        for k, row in enumerate((dt_row, dsk_row)):
            dt_v[k, c0:c0 + n, :] = _dot(jnp.where(eye, row[:, c0:c0 + n], 0.0), jnp.ones((n, P), BF16))

    lane8 = jax.lax.broadcasted_iota(jnp.int32, (8, P), 1)
    sub8 = jax.lax.broadcasted_iota(jnp.int32, (8, P), 0)

    def k_setup(i, _):
        @pl.when(i == 1)
        def _():
            for k in range(6):
                cprm(1, k).wait()

        low = sub8 < 4
        for g in range(GS // 16):
            sl = slice(16 * g, 16 * g + 16)
            dt, dsk = (dt_v.at[k, span(i, GS)][sl, :] for k in range(2))
            a_re, a_im, b_re, b_im, c_re, c_im = (prm_v.at[k, span(i, GS)][sl, :].astype(F32) for k in range(6))
            dst = p_v.at[:, span(i, GS)]
            w = {0: _cmul((c_re, c_im), (dt * b_re, dt * b_im))}
            mag = jnp.exp(dt * a_re)
            z = {1: (mag * jnp.cos(dt * a_im), mag * jnp.sin(dt * a_im))}
            for e in range(10):
                z[2 << e] = _csq(z[1 << e])
            for n, e in enumerate(_ZP):
                for q in range(2):
                    dst[2 * n + q, sl, :] = z[e][q]
            dst[24, sl, :] = w[0][0] + dsk
            dst[25, sl, :] = w[0][0] * z[256][0] - w[0][1] * z[256][1]
            w[4], w[8] = _cmul(w[0], z[4]), _cmul(w[0], z[8])
            w[1032] = _cmul(w[8], z[1024])
            w[1544] = _cmul(w[1032], z[512])
            one = (jnp.ones((16, P), F32), jnp.zeros((16, P), F32))
            for n, (a, b) in enumerate(((one, z[128]), (w[0], w[4]), (w[4], w[8]), (w[1032], w[1544]))):
                for q in range(2):
                    for t in range(2):
                        x, y = a[q][8 * t:8 * t + 8], pltpu.roll(b[q][8 * t:8 * t + 8], 4, 0)
                        r = slice(16 * g + 8 * t, 16 * g + 8 * t + 8)
                        dst[8 + 4 * n + q, r, :] = jnp.where(low, x, y)
                        dst[10 + 4 * n + q, r, :] = jnp.where(low, y, x)
        return 0

    def k_lags(i, _):
        low = sub8 < 4
        bit4, bit5, bit6 = ((lane8 & b) == 0 for b in (16, 32, 64))
        bit6x = ((lane8 >> 4) ^ sub8) & 4 == 0
        diag = (lane8 & 15) * 8 + (((lane8 >> 2) & 4) ^ sub8)
        src, dst = p_v.at[:, span(i, GA)], kc_v.at[:, span(i, GA)]
        for g in range(GA // 8):
            sl = slice(8 * g, 8 * g + 8)
            out = []
            for h in range(2):
                off = (4 if h else 0) if g + 1 < GA // 8 else (0 if h else -4)
                z = {e: tuple(jnp.take_along_axis(src[2 * n + q, 8 * g + off:8 * g + off + 8, :],
                                                  (sub8 & 3) + (4 * h - off), axis=0,
                                                  mode="promise_in_bounds") for q in range(2))
                     for n, e in enumerate(_ZP)}
                b0, r, a4, far = (tuple(src[8 + 4 * n + 2 * h + q, sl, :] for q in range(2)) for n in range(4))
                bs = [b0]
                for j in range(1, 16):
                    bs.append(_cmul(bs[j - 1], z[8]) if j < 4 else _cmul(bs[j - 4], z[32]))
                av = [_cmul(r, z[1])]
                av += [_cmul(av[0], z[1])]
                av += [_cmul(av[1], z[1]), a4, _cmul(av[1], z[256]), _cmul(a4, z[256])]
                av.append(_cmul(av[-1], z[256]))
                av.append(_cmul(av[-1], z[256]))
                av += [far, _cmul(far, z[256])]
                out.append([_dot_nt(jnp.concatenate([v[q] for v in av], axis=0),
                                    jnp.concatenate([v[q] for v in reversed(bs)], axis=0).astype(BF16))
                            for q in range(2)])
            d = [[out[h][0][8 * n:8 * n + 8] - out[h][1][8 * n:8 * n + 8] for n in range(10)] for h in range(2)]
            v = [[None] * 10, [None] * 10]
            for n in range(10):
                for h in range(2):
                    v[h][n] = jnp.take_along_axis(d[h][n], diag ^ 120, axis=1, mode="promise_in_bounds")

            def unzip(xs):
                return jnp.where(low, xs[0], xs[1]), pltpu.roll(jnp.where(low, xs[1], xs[0]), 4, 0)

            halves = []
            for lo, hi in ((0, 4), (4, 8), (8, 10)):
                xs = []
                for h in range(2):
                    u = [jnp.where(bit5, v[h][n], v[h][n + 1]) for n in range(lo, hi, 2)]
                    xs.append(jnp.where(bit6x, u[h], u[1 - h]) if len(u) == 2 else u[0])
                halves.append(unzip(xs))
            (l1, u1), (l2, u2), (l3, u3) = halves
            l6, u6 = unzip((v[0][6], v[1][6]))
            tiles = [jnp.where(bit4, l1, u1), jnp.where(bit4, u1, l1), jnp.where(bit6, l2, u2),
                     jnp.where(bit6, u2, l2), jnp.where(bit6, l3, u3)]
            tiles.append(jnp.where(lane8 < 16, l6, jnp.where((lane8 >> 4) == 5, u6, tiles[2])))
            tiles.append(jnp.where(lane8 < 96, tiles[3], tiles[2]))
            tiles.append(jnp.where(lane8 < 32, tiles[4], tiles[3]))
            for t, tile in enumerate(tiles):
                dst[t, sl, :] = tile
        return 0

    with scope("setup"):
        for k in range(6):
            cprm(0, k).wait()
        for c in (cx, cg, cfu, cfi):
            c.start()
        jax.lax.fori_loop(0, D // GS, k_setup, 0)
    with scope("lags"):
        jax.lax.fori_loop(0, D // GA, k_lags, 0)

    LB, RB, HB = 2 * P, 96, h_v.shape[2]

    def col_sum(parts):
        acc = [functools.reduce(jnp.add, parts[k::4]) for k in range(4)]
        return (acc[0] + acc[1]) + (acc[2] + acc[3])

    def ln_sum(i, _):
        src = x_v.at[span(i, RB)]
        acc = row_v[0]
        for r in range(0, RB, 8):
            acc = acc + src[r:r + 8, :].astype(F32)
        row_v[0] = acc
        return 0

    def ln_centre(c, _):
        src, dst = x_v.at[:, span(c, LB)], d_v.at[:, span(c, LB)]
        rows = span(c, D * LB // L)
        for t in range(2):
            kc_v[8 + t, rows, :] = jnp.broadcast_to(
                jnp.sum(p_v[24 + t, rows, :], axis=1, keepdims=True), (rows.size, P))
        mb = row_v[0, :, span(c, LB)]
        acc = [0.0] * 4
        for r in range(0, D, 8):
            d = src[r:r + 8, :].astype(F32) - mb
            dst[r:r + 8, :] = d.astype(BF16)
            acc[r // 8 % 4] += d * d
        row_v[1, :, span(c, LB)] = col_sum(acc)
        return 0

    def ln_scale(c):
        src, inv = d_v.at[:, span(c, HB)], row_v[0, :, span(c, HB)]
        for r in range(0, D, 8):
            h_v[c, r:r + 8, :] = (src[r:r + 8, :].astype(F32) * inv).astype(BF16)
            yield 8

    def ln_route(c, _):
        oh_v[:, span(c, HB)] = _dot(wr, h_v[c])
        _zip(ln_scale(c + 1))
        return 0

    def h_block(rows, c):
        return h_v[c * P // HB, rows, c * P % HB:c * P % HB + P]

    def compact(v):
        return jnp.concatenate([functools.reduce(
            lambda a, q: jnp.where(sub8 == q, v[:, (c + q) * P:(c + q + 1) * P], a),
            range(1, 8), v[:, c * P:(c + 1) * P]) for c in range(0, NB, 8)], axis=0)

    def spread(v):
        return jnp.concatenate([jnp.broadcast_to(v[c:c + 1], (8, P)) for c in range(NB)], axis=1)

    def total(k):
        return compact(jnp.broadcast_to(jnp.sum(row_v[k], axis=0, keepdims=True), (8, L)))

    with scope("lnorm"):
        for c in (cx, cg, cfu, cfi):
            c.wait()
        row_v[0] = jnp.zeros((8, L), F32)
        jax.lax.fori_loop(0, D // RB, ln_sum, 0)
        m = total(0) / D
        mb = _rbf(m)
        row_v[0] = spread(mb)
        jax.lax.fori_loop(0, L // LB, ln_centre, 0)
        var = jnp.maximum(total(1) / D - (m - mb) * (m - mb), 0.0)
        row_v[0] = spread(0.5 / _rbf(jnp.sqrt(_rbf(_rbf(var) + _rbf(jnp.full_like(var, 1e-5))))))
        wr = jnp.broadcast_to(2.0 * wr_v[...].astype(F32)[None, :], (8, D))
        _zip(ln_scale(0))
        jax.lax.fori_loop(0, L // HB - 1, ln_route, 0)
        oh_v[:, L - HB:] = _dot(wr, h_v[L // HB - 1])

    def put(dst, kind, c, g, a, b):
        for q, v in enumerate((a, b, a - b)):
            hat_v[dst, 3 * kind + q, c, 8 * g:8 * g + 8, :] = v

    def c_signal(src, dst, c0, n):
        lhs = jnp.concatenate([h_block(span(src, GD), c) for c in range(c0, c0 + n)], axis=0)
        uh = _dot(lhs, pltpu.bitcast(fu_v[...], BF16))
        for c in range(n):
            for g in range(GD // 8):
                r = slice(c * GD + 8 * g, c * GD + 8 * g + 8)
                put(dst, 0, c0 + c, g, uh[r, :P], uh[r, P:])
                yield 1

    def c_window(src, dst, j):
        tiles = kc_v.at[:, span(src, GD)]
        kh = None
        for t, ids in zip(_SRC[j], layout[j]):
            rhs = jnp.concatenate([jnp.zeros((8, 2 * P), jnp.uint32) if n is None else g_v[n] for n in ids], axis=0)
            part = _dot(tiles[t], pltpu.bitcast(rhs, BF16))
            kh = part if kh is None else kh + part
        for g in range(GD // 8):
            sl = slice(8 * g, 8 * g + 8)
            a, b = kh[sl, :P], kh[sl, P:]
            if j == 0:
                a = a + tiles[8, sl, :]
            if j == 3:
                edge = pltpu.bitcast(g_v[g_v.shape[0] - 1], F32)
                a, b = a + tiles[9, sl, :] * edge[:, :P], b + tiles[9, sl, :] * edge[:, P:]
            put(dst, 1, j, g, a, b)
            yield 1

    def c_inverse(i, c0, n, r0=0, m=GD):
        lhs = jnp.concatenate([jnp.concatenate([hat_v[i, 6 + q, c, r0:r0 + m, :] for q in range(2)], axis=1)
                               for c in range(c0, c0 + n)], axis=0)
        y = _dot(lhs, pltpu.bitcast(fi_v[...], BF16))
        for c in range(n):
            for r in range(0, m, 8):
                s_v.at[span(i, GD)][r0 + r:r0 + r + 8, (c0 + c) * P:(c0 + c + 1) * P] = y[c * m + r:c * m + r + 8]
                yield 1

    window_pairs = ((14, 15), (12, 13), (10, 11), (1, 2), (8, 9), (6, 7), (4, 5), (0, 3))

    def c_transforms(i, first=False):
        nxt = i + 1
        for c0 in range(0, NB, UB):
            if not first:
                _zip(c_signal(nxt, nxt, c0, UB), c_inverse(i, c0, UB))
                yield UB
            elif c0 % 2 == 0:
                _zip(c_signal(nxt, nxt, c0, UB), c_signal(nxt, nxt, c0 + UB, UB))
                yield UB
            for pair in window_pairs[c0 // 2:(c0 + UB) // 2]:
                _zip(*(c_window(nxt, i + 1, j) for j in pair))
                yield len(_SRC[pair[0]])

    def c_product(i, groups=range(GD // 8)):
        for g in groups:
            sl = slice(8 * g, 8 * g + 8)
            for cs in (range(8, 16), range(8)):
                m0 = {}
                for q in range(3):
                    acc = dict(m0)
                    for j in reversed(range(max(cs) + 1)):
                        k = hat_v[i, 3 + q, j, sl, :]
                        live = [c for c in cs if c >= j]
                        for c in live:
                            t = k * hat_v[i, q, c - j, sl, :]
                            acc[c] = t if c not in acc else (acc[c] - t if q else acc[c] + t)
                        yield len(live)
                    if q == 0:
                        m0 = acc
                    else:
                        for c in cs:
                            hat_v[i + 1, 5 + q, c, sl, :] = acc[c]

    def c_step(i, pace, *side):
        _interleave((c_product(i), GD // 8 * 3 * 136),
                    (_merge(*side), sum(total * cost for _, total, cost in side) * pace))

    with scope("topk"):
        r = _rbf(compact(oh_v[...]))
        bits = pltpu.bitcast(jnp.where(r == 0.0, 0.0, r), jnp.int32)
        ordered = jnp.where(bits < 0, ~bits, bits ^ jnp.int32(-2**31))
        idx = (jax.lax.broadcasted_iota(jnp.int32, (NB, P), 0) * P
               + jax.lax.broadcasted_iota(jnp.int32, (NB, P), 1))
        key = pltpu.bitcast((jax.lax.shift_right_logical(ordered, 16) << 11) + (0x20000000 + L - 1 - idx), F32)
        rest, top = key, jnp.zeros((8, P), F32)
        for q in range(8):
            mx = jnp.max(jnp.max(rest, axis=0, keepdims=True), axis=1, keepdims=True)
            top = jnp.where(sub8 == q, mx, top)
            rest = jnp.where(rest == mx, 0.0, rest)
        _zip(c_signal(0, 0, 0, NB // 2), c_signal(0, 0, NB // 2, NB // 2))
        for pair in window_pairs:
            _zip(*(c_window(0, 0, j) for j in pair))
        oh_v[...] = jnp.where(spread(key) == jnp.concatenate([top] * NB, axis=1), 1.0, 0.0)
        o16 = jax.lax.shift_right_logical(pltpu.bitcast(top, jnp.int32) - 0x20000000, 11) << 16
        r_top = pltpu.bitcast(jnp.where(o16 < 0, o16 ^ jnp.int32(-2**31), (~o16) & jnp.int32(-65536)), F32)
        gate = 0.5 * jax.nn.sigmoid(r_top)

    def gather(lo, hi):
        for r in range(lo, hi, P):
            rs = slice(r, min(r + P, D))
            part = 0.0
            for c0 in range(0, NB, 4):
                part = part + functools.reduce(jnp.add, [
                    _dot_nt(oh_v[:, c * P:(c + 1) * P], h_block(rs, c)) for c in range(c0, c0 + 4)])
                yield 1
            row_v[0, :, rs] = 2.0 * part

    with scope("conv0"):
        @pl.loop(0, NG)
        def _(i):
            @pl.when(i == 0)
            def _():
                c_step(0, CS[0], (c_transforms(0, True), 17, 1), (gather(0, G0 * P), 4 * G0 + 0.5, WF[0]))

            @pl.when(i > 0)
            def _():
                c_step(i, CS[4], (c_transforms(i), 25, 1), (gather(G0 * P, D), 4 * max(5 - G0, 1), WF[4]))

    def gate_up_step(item, _):
        i = item - NG
        ws, dst = (wg_v.at[:, span(i, FC)], wu_v.at[:, span(i, FC)]), act_v.at[:, :, span(i, FC)]

        def gate_up():
            for c in range(0, FC, 2 * P):
                acc = [0.0, 0.0]
                for r in range(0, D, P):
                    rs = slice(r, min(r + P, D))
                    acc = [a + _dot(row_v[0, :, rs], w[rs, c:c + 2 * P]) for a, w in zip(acc, ws)]
                    yield 1
                for k in range(2):
                    dst[k, :, c:c + 2 * P] = acc[k]

        c_step(item, CS[1], (c_transforms(item), 25, 1), (gate_up(), FC // (2 * P) * 5 + GX, WF[1]))

        @pl.when(i + 1 < NF)
        def _():
            cwg(i + 1).wait()
            cwu(i + 1).wait()

        return 0

    with scope("conv1"):
        cwg(0).wait()
        cwu(0).wait()
        jax.lax.fori_loop(NG, NG + NF, gate_up_step, 0)
        a = 0.5 * act_v[0]
        act_v[0] = (a + a * jnp.tanh(a)) * act_v[1]

    def project(rows, lead, res):
        n = rows.size
        w = wd_v.at[rows]
        acc = 0.0
        for c in range(0, FF, 4 * P):
            acc = acc + functools.reduce(jnp.add, [
                _dot_nt(act_v[0, :, f:f + P], w[:, f:f + P]) for f in range(c, c + 4 * P, P)])
            yield 1
        yield from [1] * lead
        eye = jax.lax.broadcasted_iota(jnp.int32, (n, n), 0) == jax.lax.broadcasted_iota(jnp.int32, (n, n), 1)
        res.append(_dot_nt(eye.astype(F32), acc * gate[:, :n]))
        yield from [1] * lead

    def emit(e, yt):
        rows = out_rows(e)
        h = jnp.concatenate([h_v[c, rows, :].astype(F32) for c in range(L // HB)], axis=1) + _dot(yt, oh_v[...])
        s = s_v.at[GD:][rows, :]
        q = s * h
        out = (x_v[rows, :].astype(F32) + q) + q * jnp.tanh(h)
        if debug:
            out = s
        o_v[rows, :] = out.astype(o_v.dtype)

    def finish(e):
        yt = []
        yield from project(out_rows(e), LD, yt)
        emit(e, yt[0])

    NP = FF // (4 * P) + 2 * LD

    def inverse_all(i, step, *rows):
        for c0 in range(0, NB, 2 * step):
            _zip(c_inverse(i, c0, step, *rows), c_inverse(i, c0 + step, step, *rows))
            yield 2 * step

    def finish_step(item, _):
        e = item - (NG + NF)

        @pl.when(e < NL)
        def _():
            c_step(item, CS[2], (c_transforms(item), 25, 1), (finish(e), NP, WF[2]))
            cout(e).start()

            @pl.when(e + 1 < NL)
            def _():
                cwd(e + 1).wait()

            @pl.when(e + 1 == NL)
            def _():
                for i in range(len(tails)):
                    cwd(NL + i).wait()

        @pl.when(e == NL)
        def _():
            yt = []
            c_step(ND - 1, CS[3], (inverse_all(ND - 1, 1), NB * LI, 0.5), (finish(NL), NP, WF[3]),
                   (project(pl.ds(D - GD, GD), LD, yt), NP + 0.5, WF[3] * 0.5))
            yt_v[...] = yt[0]
            cout(NL).start()

        return 0

    with scope("conv2"):
        cwd(0).wait()
        jax.lax.fori_loop(NG + NF, ND, finish_step, 0)

    with scope("tail"):
        for n in range(GD // GT):
            _zip(inverse_all(ND, NB // 2, n * GT, GT))
            emit(NL + 1 + n, yt_v[n * GT:(n + 1) * GT, :])
            cout(NL + 1 + n).start()
        for e in range(NL + len(tails)):
            cout(e).wait()


def run(A_u, A_A_re, A_A_im, A_B_re, A_B_im, A_C_re, A_C_im, A_log_dt, A_Dskip, B_x, B_w_r,
        B_w_gate, B_w_up, B_w_down, GS=144, GA=288, GD=64, NG=2, NF=3, GE=128, GT=64, LD=3, CS=(1.1, 1.04, 0.99, 1.01, 1.1), UB=1, SC=0, G0=4, LI=1.29, WF=(1.09, 0.57, 0.67, 1.14, 0.23), GX=3.07,
        debug=False, interpret=False, flags=None, DS=3):
    _, L, D = A_u.shape
    FF = B_w_gate.shape[1]
    fu, fi, g = _tables()[:3]
    odt = F32 if debug else A_u.dtype
    hbm = pl.BlockSpec(memory_space=pl.ANY)
    NB = L // P
    NE = D // GD - NG - NF + GD // GT
    out = pl.pallas_call(
        functools.partial(_kernel, GS=GS, GA=GA, GD=GD, NG=NG, NF=NF, GE=GE, GT=GT, LD=LD, CS=CS, UB=UB, SC=SC, G0=G0, LI=LI, WF=WF, GX=GX, debug=debug),
        out_shape=jax.ShapeDtypeStruct((D, L), odt),
        in_specs=[hbm] * 16,
        out_specs=hbm,
        scratch_shapes=[
            *[pltpu.VMEM((D,), BF16)] * 3,
            pltpu.VMEM((D, L), BF16), pltpu.VMEM((6, D, P), BF16),
            pltpu.VMEM((D, FF), BF16), pltpu.VMEM((D, FF), BF16), pltpu.VMEM((D, FF), BF16),
            pltpu.VMEM(fu.shape, jnp.uint32), pltpu.VMEM(fi.shape, jnp.uint32),
            pltpu.VMEM(g.shape, jnp.uint32),
            pltpu.VMEM((D, L), odt), pltpu.VMEM((D, L), BF16), pltpu.VMEM((4, D, L // 4), BF16),
            pltpu.VMEM((D + GD, L), F32),
            pltpu.VMEM((10, D, P), F32), pltpu.VMEM((2, D, P), F32),
            pltpu.VMEM((2, 8, L), F32), pltpu.VMEM((8, L), F32), pltpu.VMEM((2, 8, FF), F32),
            pltpu.VMEM((D // GD + 1, 8, NB, GD, P), F32),
            pltpu.VMEM((26, D, P), F32), pltpu.VMEM((GD, 8), F32), pltpu.VMEM((128, 8), F32),
            pltpu.SemaphoreType.DMA((7 + 2 * NF + NE,)),
            pltpu.SemaphoreType.DMA((12,)),
            pltpu.SemaphoreType.DMA((NE,)),
        ],
        compiler_params=pltpu.CompilerParams(vmem_limit_bytes=112 * 2**20, flags=flags, disable_semaphore_checks=bool(DS & 1), disable_bounds_checks=bool(DS & 2)),
        interpret=interpret,
        name="ssm_moe",
    )(A_u[0].T, A_A_re, A_A_im, A_B_re, A_B_im, A_C_re, A_C_im, A_log_dt, A_Dskip, B_w_r,
      B_w_gate, B_w_up, B_w_down.T, fu, fi, g)
    return out.T[None]


@jax.jit
def pallas_recurrent_scan__ssm_conv_s4__moe_arch_mod__prompt_kernel(
    A_u: jax.Array,
    A_A_re: jax.Array,
    A_A_im: jax.Array,
    A_B_re: jax.Array,
    A_B_im: jax.Array,
    A_C_re: jax.Array,
    A_C_im: jax.Array,
    A_log_dt: jax.Array,
    A_Dskip: jax.Array,
    B_x: jax.Array,
    B_w_r: jax.Array,
    B_w_gate: jax.Array,
    B_w_up: jax.Array,
    B_w_down: jax.Array,
):
    return run(A_u, A_A_re, A_A_im, A_B_re, A_B_im, A_C_re, A_C_im, A_log_dt, A_Dskip, B_x,
               B_w_r, B_w_gate, B_w_up, B_w_down)
```

```python
import contextlib
import functools

import jax
import jax.numpy as jnp
import numpy as np
import jax.experimental.pallas as pl
import jax.experimental.pallas.tpu as pltpu

F32 = jnp.float32
BF16 = jnp.bfloat16
P = 128


def _bf16_bits(a):
    u = np.ascontiguousarray(a, dtype=np.float32).view(np.uint32)
    return ((u + 0x7FFF + ((u >> 16) & 1)) >> 16).astype(np.uint32)


def _round_bf16(a):
    return (_bf16_bits(a) << 16).view(np.float32)


def _pack_rows(a):
    b = _bf16_bits(a)
    return (b[0::2] | (b[1::2] << 16)).astype(np.uint32)


def _tile_lags():
    lane = np.arange(P)
    quarter, hb, j = lane // 32, (lane // 16) % 2, lane % 16

    def half(offsets, second):
        q = (quarter + 2 * second) % 4
        return np.array(offsets)[q] + 128 * (hb ^ second) + 8 * j

    l1, u1 = half((1, 2, 3, 4), 0), half((5, 6, 7, 8), 1)
    l2, u2 = half((258, 260, 516, 772), 0), half((262, 264, 520, 776), 1)
    l3, u3 = half((1032, 1288) * 2, 0), half((1544, 1800) * 2, 1)
    lags = [np.where(hb == 0, l1, u1), np.where(hb == 0, u1, l1),
            np.where(lane < 64, l2, u2), np.where(lane < 64, u2, l2), np.where(lane < 64, l3, u3)]
    lags.append(np.where(lane // 16 == 0, half((516,) * 4, 0),
                         np.where(lane // 16 == 5, half((520,) * 4, 1), lags[2])))
    lags.append(np.where(lane < 96, lags[3], lags[2]))
    lags.append(np.where(lane < 32, lags[4], lags[3]))
    return lags


_SRC = ((0,), (0, 1), (1, 2), (2,), (5,), (6,), (3,), (3,), (7,), (7,)) + ((4,),) * 6


@functools.cache
def _tables():
    k = np.arange(P)
    phi = 2 * np.pi * (k + 0.25) / P

    def coords(m):
        z = np.exp(1j * np.outer(m, phi))
        return np.concatenate([z.real + z.imag / np.sqrt(3), 2 * z.imag / np.sqrt(3)], axis=1)

    fu = 2.0 * coords(np.arange(P))
    zi = np.exp(-1j * np.outer(phi, np.arange(P)))
    fi = np.concatenate([zi.real, (np.exp(2j * np.pi / 3) * zi).real], axis=0) / P
    lags = _tile_lags()
    groups, layout = [], []
    for j, src in enumerate(_SRC):
        m = np.arange(-P + 1 + (j == 3), P)
        m = m[P * j + m >= 1]
        rl = _round_bf16(P * j + m)
        hit = np.zeros(len(m), int)
        layout.append([])
        for t in src:
            sel = (lags[t][:, None] == rl[None, :])
            hit += sel.sum(0)
            g = _pack_rows(sel.astype(np.float64) @ coords(m))
            ids = []
            for r in range(0, P // 2, 8):
                known = [n for n, e in enumerate(groups) if np.array_equal(e, g[r:r + 8])]
                if not sel[2 * r:2 * r + 16].any():
                    ids.append(None)
                elif known:
                    ids.append(known[0])
                else:
                    ids.append(len(groups))
                    groups.append(g[r:r + 8])
            layout[-1].append(ids)
        assert (hit == 1).all()
    edge = np.broadcast_to(coords(np.array([-P + 1])).astype(np.float32), (8, 2 * P)).view(np.uint32)
    return _pack_rows(fu), _pack_rows(fi), np.stack(groups + [edge]), layout


def _cmul(a, b):
    return (a[0] * b[0] - a[1] * b[1], a[0] * b[1] + a[1] * b[0])


def _csq(a):
    t = a[0] * a[1]
    return ((a[0] - a[1]) * (a[0] + a[1]), t + t)


def _dot(a, b):
    return jax.lax.dot_general(a, b, (((1,), (0,)), ((), ())), preferred_element_type=F32)


def _dot_nt(a, b):
    return jax.lax.dot_general(a, b, (((1,), (1,)), ((), ())), preferred_element_type=F32)


def _rbf(x):
    return x.astype(BF16).astype(F32)


def _interleave(*gens):
    state = [[0.0, k, g, total] for k, (g, total) in enumerate(gens)]
    while state:
        cur = min(state, key=lambda e: (e[0], e[1]))
        w = next(cur[2], None)
        if w is None:
            state.remove(cur)
        else:
            cur[0] += w / cur[3]


def _merge(*gens):
    state = [[0.0, k, g, total, cost] for k, (g, total, cost) in enumerate(gens)]
    while state:
        cur = min(state, key=lambda e: (e[0], e[1]))
        w = next(cur[2], None)
        if w is None:
            state.remove(cur)
        else:
            cur[0] += w / cur[3]
            yield w * cur[4]


def _zip(*gens):
    _interleave(*((g, 1.0) for g in gens))


_ZP = (1, 8, 32, 256)


def _kernel(x_hbm, are_hbm, aim_hbm, bre_hbm, bim_hbm, cre_hbm, cim_hbm, ldt_hbm, dsk_hbm,
            wr_hbm, wg_hbm, wu_hbm, wd_hbm, fu_hbm, fi_hbm, g_hbm, o_hbm,
            ldt_v, dsk_v, wr_v, x_v, prm_v, wg_v, wu_v, wd_v, fu_v, fi_v, g_v, o_v, d_v, h_v, s_v,
            kc_v, dt_v, row_v, oh_v, act_v, hat_v, p_v, yt_v, yu_v, sems, psem, osem,
            *, GS, GA, GD, NG, NF, GE, GT, LD, CS, UB, SC, G0, LI, WF, GX, OP, debug):
    scope = jax.named_scope if SC else (lambda _: contextlib.nullcontext())
    D, L = x_v.shape
    FF = wg_v.shape[1]
    NB = L // P
    FC = FF // NF
    ND = D // GD
    NL = ND - 1 - NG - NF
    tails = ((NL * GE, D - GD - NL * GE),) + tuple((r, GT) for r in range(D - GD, D, GT))
    layout = _tables()[3]

    def span(i, n):
        start = i * n
        if not isinstance(start, int):
            start = pl.multiple_of(start, n)
        return pl.ds(start, n)

    prm_hbm = (are_hbm, aim_hbm, bre_hbm, bim_hbm, cre_hbm, cim_hbm)

    def cprm(part, k):
        r = pl.ds(0, GS) if part == 0 else pl.ds(GS, D - GS)
        return pltpu.make_async_copy(prm_hbm[k].at[r], prm_v.at[k, r], psem.at[6 * part + k])

    cx, cfu, cfi, cg, *cvec = (
        pltpu.make_async_copy(src, dst, sems.at[k]) for k, (src, dst) in enumerate((
            (x_hbm, x_v), (fu_hbm, fu_v), (fi_hbm, fi_v), (g_hbm, g_v),
            (ldt_hbm, ldt_v), (dsk_hbm, dsk_v), (wr_hbm, wr_v))))

    def cwg(i):
        return pltpu.make_async_copy(wg_hbm.at[:, span(i, FC)], wg_v.at[:, span(i, FC)], sems.at[7 + i])

    def cwu(i):
        return pltpu.make_async_copy(wu_hbm.at[:, span(i, FC)], wu_v.at[:, span(i, FC)], sems.at[7 + NF + i])

    def out_rows(i):
        if isinstance(i, int) and i >= NL:
            return pl.ds(*tails[i - NL])
        return pl.ds(i * GE if isinstance(i, int) else pl.multiple_of(i * GE, 16), GE)

    def cwd(i):
        return pltpu.make_async_copy(wd_hbm.at[out_rows(i)], wd_v.at[out_rows(i)], sems.at[7 + 2 * NF + i])

    def cout(i):
        return pltpu.make_async_copy(o_v.at[out_rows(i)], o_hbm.at[out_rows(i)], osem.at[i])

    for c in cvec:
        c.start()
    for k in range(6):
        cprm(0, k).start()

    @pl.loop(0, NF)
    def _(i):
        cwg(i).start(priority=1)
        cwu(i).start(priority=1)

    @pl.loop(0, NL)
    def _(i):
        cwd(i).start(priority=1)

    for i in range(len(tails)):
        cwd(NL + i).start(priority=1)

    for k in range(6):
        cprm(1, k).start()
    for c in cvec:
        c.wait()

    dt_row = _rbf(jnp.exp(ldt_v[...].astype(F32)[None, :]))
    dsk_row = dsk_v[...].astype(F32)[None, :] * (1.0 / P)
    for c0 in range(0, D, P):
        n = min(P, D - c0)
        eye = (jax.lax.broadcasted_iota(jnp.int32, (n, n), 0) == jax.lax.broadcasted_iota(jnp.int32, (n, n), 1))
        for k, row in enumerate((dt_row, dsk_row)):
            dt_v[k, c0:c0 + n, :] = _dot(jnp.where(eye, row[:, c0:c0 + n], 0.0), jnp.ones((n, P), BF16))

    lane8 = jax.lax.broadcasted_iota(jnp.int32, (8, P), 1)
    sub8 = jax.lax.broadcasted_iota(jnp.int32, (8, P), 0)

    def k_setup(i, _):
        @pl.when(i == 1)
        def _():
            for k in range(6):
                cprm(1, k).wait()

        low = sub8 < 4
        for g in range(GS // 16):
            sl = slice(16 * g, 16 * g + 16)
            dt, dsk = (dt_v.at[k, span(i, GS)][sl, :] for k in range(2))
            a_re, a_im, b_re, b_im, c_re, c_im = (prm_v.at[k, span(i, GS)][sl, :].astype(F32) for k in range(6))
            dst = p_v.at[:, span(i, GS)]
            w = {0: _cmul((c_re, c_im), (dt * b_re, dt * b_im))}
            mag = jnp.exp(dt * a_re)
            z = {1: (mag * jnp.cos(dt * a_im), mag * jnp.sin(dt * a_im))}
            for e in range(10):
                z[2 << e] = _csq(z[1 << e])
            for n, e in enumerate(_ZP):
                for q in range(2):
                    dst[2 * n + q, sl, :] = z[e][q]
            dst[24, sl, :] = w[0][0] + dsk
            dst[25, sl, :] = w[0][0] * z[256][0] - w[0][1] * z[256][1]
            w[4], w[8] = _cmul(w[0], z[4]), _cmul(w[0], z[8])
            w[1032] = _cmul(w[8], z[1024])
            w[1544] = _cmul(w[1032], z[512])
            one = (jnp.ones((16, P), F32), jnp.zeros((16, P), F32))
            for n, (a, b) in enumerate(((one, z[128]), (w[0], w[4]), (w[4], w[8]), (w[1032], w[1544]))):
                for q in range(2):
                    for t in range(2):
                        x, y = a[q][8 * t:8 * t + 8], pltpu.roll(b[q][8 * t:8 * t + 8], 4, 0)
                        r = slice(16 * g + 8 * t, 16 * g + 8 * t + 8)
                        dst[8 + 4 * n + q, r, :] = jnp.where(low, x, y)
                        dst[10 + 4 * n + q, r, :] = jnp.where(low, y, x)
        return 0

    def k_lags(i, _):
        low = sub8 < 4
        bit4, bit5, bit6 = ((lane8 & b) == 0 for b in (16, 32, 64))
        bit6x = ((lane8 >> 4) ^ sub8) & 4 == 0
        diag = (lane8 & 15) * 8 + (((lane8 >> 2) & 4) ^ sub8)
        src, dst = p_v.at[:, span(i, GA)], kc_v.at[:, span(i, GA)]
        for g in range(GA // 8):
            sl = slice(8 * g, 8 * g + 8)
            out = []
            for h in range(2):
                off = (4 if h else 0) if g + 1 < GA // 8 else (0 if h else -4)
                z = {e: tuple(jnp.take_along_axis(src[2 * n + q, 8 * g + off:8 * g + off + 8, :],
                                                  (sub8 & 3) + (4 * h - off), axis=0,
                                                  mode="promise_in_bounds") for q in range(2))
                     for n, e in enumerate(_ZP)}
                b0, r, a4, far = (tuple(src[8 + 4 * n + 2 * h + q, sl, :] for q in range(2)) for n in range(4))
                bs = [b0]
                for j in range(1, 16):
                    bs.append(_cmul(bs[j - 1], z[8]) if j < 4 else _cmul(bs[j - 4], z[32]))
                av = [_cmul(r, z[1])]
                av += [_cmul(av[0], z[1])]
                av += [_cmul(av[1], z[1]), a4, _cmul(av[1], z[256]), _cmul(a4, z[256])]
                av.append(_cmul(av[-1], z[256]))
                av.append(_cmul(av[-1], z[256]))
                av += [far, _cmul(far, z[256])]
                out.append([_dot_nt(jnp.concatenate([v[q] for v in av], axis=0),
                                    jnp.concatenate([v[q] for v in reversed(bs)], axis=0).astype(BF16))
                            for q in range(2)])
            d = [[out[h][0][8 * n:8 * n + 8] - out[h][1][8 * n:8 * n + 8] for n in range(10)] for h in range(2)]
            v = [[None] * 10, [None] * 10]
            for n in range(10):
                for h in range(2):
                    v[h][n] = jnp.take_along_axis(d[h][n], diag ^ 120, axis=1, mode="promise_in_bounds")

            def unzip(xs):
                return jnp.where(low, xs[0], xs[1]), pltpu.roll(jnp.where(low, xs[1], xs[0]), 4, 0)

            halves = []
            for lo, hi in ((0, 4), (4, 8), (8, 10)):
                xs = []
                for h in range(2):
                    u = [jnp.where(bit5, v[h][n], v[h][n + 1]) for n in range(lo, hi, 2)]
                    xs.append(jnp.where(bit6x, u[h], u[1 - h]) if len(u) == 2 else u[0])
                halves.append(unzip(xs))
            (l1, u1), (l2, u2), (l3, u3) = halves
            l6, u6 = unzip((v[0][6], v[1][6]))
            tiles = [jnp.where(bit4, l1, u1), jnp.where(bit4, u1, l1), jnp.where(bit6, l2, u2),
                     jnp.where(bit6, u2, l2), jnp.where(bit6, l3, u3)]
            tiles.append(jnp.where(lane8 < 16, l6, jnp.where((lane8 >> 4) == 5, u6, tiles[2])))
            tiles.append(jnp.where(lane8 < 96, tiles[3], tiles[2]))
            tiles.append(jnp.where(lane8 < 32, tiles[4], tiles[3]))
            for t, tile in enumerate(tiles):
                dst[t, sl, :] = tile
        return 0

    with scope("setup"):
        for k in range(6):
            cprm(0, k).wait()
        for c in (cx, cg, cfu, cfi):
            c.start()
        jax.lax.fori_loop(0, D // GS, k_setup, 0)
    with scope("lags"):
        jax.lax.fori_loop(0, D // GA, k_lags, 0)

    LB, RB, HB = 2 * P, 96, h_v.shape[2]

    def col_sum(parts):
        acc = [functools.reduce(jnp.add, parts[k::4]) for k in range(4)]
        return (acc[0] + acc[1]) + (acc[2] + acc[3])

    def ln_sum(i, _):
        src = x_v.at[span(i, RB)]
        acc = row_v[0]
        for r in range(0, RB, 8):
            acc = acc + src[r:r + 8, :].astype(F32)
        row_v[0] = acc
        return 0

    def ln_centre(c, _):
        src, dst = x_v.at[:, span(c, LB)], d_v.at[:, span(c, LB)]
        rows = span(c, D * LB // L)
        for t in range(2):
            kc_v[8 + t, rows, :] = jnp.broadcast_to(
                jnp.sum(p_v[24 + t, rows, :], axis=1, keepdims=True), (rows.size, P))
        mb = row_v[0, :, span(c, LB)]
        acc = [0.0] * 4
        for r in range(0, D, 8):
            d = src[r:r + 8, :].astype(F32) - mb
            dst[r:r + 8, :] = d.astype(BF16)
            acc[r // 8 % 4] += d * d
        row_v[1, :, span(c, LB)] = col_sum(acc)
        return 0

    def ln_scale(c):
        src, inv = d_v.at[:, span(c, HB)], row_v[0, :, span(c, HB)]
        for r in range(0, D, 8):
            h_v[c, r:r + 8, :] = (src[r:r + 8, :].astype(F32) * inv).astype(BF16)
            yield 8

    def ln_route(c, _):
        oh_v[:, span(c, HB)] = _dot(wr, h_v[c])
        _zip(ln_scale(c + 1))
        return 0

    def h_block(rows, c):
        return h_v[c * P // HB, rows, c * P % HB:c * P % HB + P]

    def compact(v):
        return jnp.concatenate([functools.reduce(
            lambda a, q: jnp.where(sub8 == q, v[:, (c + q) * P:(c + q + 1) * P], a),
            range(1, 8), v[:, c * P:(c + 1) * P]) for c in range(0, NB, 8)], axis=0)

    def spread(v):
        return jnp.concatenate([jnp.broadcast_to(v[c:c + 1], (8, P)) for c in range(NB)], axis=1)

    def total(k):
        return compact(jnp.broadcast_to(jnp.sum(row_v[k], axis=0, keepdims=True), (8, L)))

    with scope("lnorm"):
        for c in (cx, cg, cfu, cfi):
            c.wait()
        row_v[0] = jnp.zeros((8, L), F32)
        jax.lax.fori_loop(0, D // RB, ln_sum, 0)
        m = total(0) / D
        mb = _rbf(m)
        row_v[0] = spread(mb)
        jax.lax.fori_loop(0, L // LB, ln_centre, 0)
        var = jnp.maximum(total(1) / D - (m - mb) * (m - mb), 0.0)
        row_v[0] = spread(0.5 / _rbf(jnp.sqrt(_rbf(_rbf(var) + _rbf(jnp.full_like(var, 1e-5))))))
        wr = jnp.broadcast_to(2.0 * wr_v[...].astype(F32)[None, :], (8, D))
        _zip(ln_scale(0))
        jax.lax.fori_loop(0, L // HB - 1, ln_route, 0)
        oh_v[:, L - HB:] = _dot(wr, h_v[L // HB - 1])

    def put(dst, kind, c, g, a, b):
        for q, v in enumerate((a, b, a - b)):
            hat_v[dst, g, 3 * kind + q, c] = v

    def c_signal(src, dst, c0, n):
        lhs = jnp.concatenate([h_block(span(src, GD), c) for c in range(c0, c0 + n)], axis=0)
        uh = _dot(lhs, pltpu.bitcast(fu_v[...], BF16))
        for c in range(n):
            for g in range(GD // 8):
                r = slice(c * GD + 8 * g, c * GD + 8 * g + 8)
                put(dst, 0, c0 + c, g, uh[r, :P], uh[r, P:])
                yield 1

    def c_window(src, dst, j):
        tiles = kc_v.at[:, span(src, GD)]
        kh = None
        for t, ids in zip(_SRC[j], layout[j]):
            rhs = jnp.concatenate([jnp.zeros((8, 2 * P), jnp.uint32) if n is None else g_v[n] for n in ids], axis=0)
            part = _dot(tiles[t], pltpu.bitcast(rhs, BF16))
            kh = part if kh is None else kh + part
        for g in range(GD // 8):
            sl = slice(8 * g, 8 * g + 8)
            a, b = kh[sl, :P], kh[sl, P:]
            if j == 0:
                a = a + tiles[8, sl, :]
            if j == 3:
                edge = pltpu.bitcast(g_v[g_v.shape[0] - 1], F32)
                a, b = a + tiles[9, sl, :] * edge[:, :P], b + tiles[9, sl, :] * edge[:, P:]
            put(dst, 1, j, g, a, b)
            yield 1

    def c_inverse(i, c0, n, r0=0, m=GD):
        lhs = jnp.concatenate([jnp.concatenate([hat_v[i, g, 6 + q, c] for q in range(2)], axis=1)
                               for c in range(c0, c0 + n) for g in range(r0 // 8, (r0 + m) // 8)], axis=0)
        y = _dot(lhs, pltpu.bitcast(fi_v[...], BF16))
        for c in range(n):
            for r in range(0, m, 8):
                s_v.at[span(i, GD)][r0 + r:r0 + r + 8, (c0 + c) * P:(c0 + c + 1) * P] = y[c * m + r:c * m + r + 8]
                yield 1

    window_pairs = ((14, 15), (12, 13), (10, 11), (1, 2), (8, 9), (6, 7), (4, 5), (0, 3))

    def c_transforms(i, first=False):
        nxt = i + 1
        for c0 in range(0, NB, UB):
            if not first:
                _zip(c_signal(nxt, nxt, c0, UB), c_inverse(i, c0, UB))
                yield UB
            elif c0 % 2 == 0:
                _zip(c_signal(nxt, nxt, c0, UB), c_signal(nxt, nxt, c0 + UB, UB))
                yield UB
            for pair in window_pairs[c0 // 2:(c0 + UB) // 2]:
                _zip(*(c_window(nxt, i + 1, j) for j in pair))
                yield len(_SRC[pair[0]])

    def c_product(i, groups=range(GD // 8)):
        for g in groups:
            sl = slice(8 * g, 8 * g + 8)
            for cs in (range(8, 16), range(8)):
                m0 = {}
                for q in range(3):
                    acc = dict(m0)
                    for j in reversed(range(max(cs) + 1)):
                        k = hat_v[i, g, 3 + q, j]
                        live = [c for c in cs if c >= j]
                        for c in live:
                            t = k * hat_v[i, g, q, c - j]
                            acc[c] = t if c not in acc else (acc[c] - t if q else acc[c] + t)
                        yield len(live)
                    if q == 0:
                        m0 = acc
                    else:
                        for c in cs:
                            hat_v[i + 1, g, 5 + q, c] = acc[c]

    def c_step(i, pace, *side):
        _interleave((c_product(i), GD // 8 * 3 * 136),
                    (_merge(*side), sum(total * cost for _, total, cost in side) * pace))

    with scope("topk"):
        r = _rbf(compact(oh_v[...]))
        bits = pltpu.bitcast(jnp.where(r == 0.0, 0.0, r), jnp.int32)
        ordered = jnp.where(bits < 0, ~bits, bits ^ jnp.int32(-2**31))
        idx = (jax.lax.broadcasted_iota(jnp.int32, (NB, P), 0) * P
               + jax.lax.broadcasted_iota(jnp.int32, (NB, P), 1))
        key = pltpu.bitcast((jax.lax.shift_right_logical(ordered, 16) << 11) + (0x20000000 + L - 1 - idx), F32)
        rest, top = key, jnp.zeros((8, P), F32)
        for q in range(8):
            mx = jnp.max(jnp.max(rest, axis=0, keepdims=True), axis=1, keepdims=True)
            top = jnp.where(sub8 == q, mx, top)
            rest = jnp.where(rest == mx, 0.0, rest)
        _zip(c_signal(0, 0, 0, NB // 2), c_signal(0, 0, NB // 2, NB // 2))
        for pair in window_pairs:
            _zip(*(c_window(0, 0, j) for j in pair))
        oh_v[...] = jnp.where(spread(key) == jnp.concatenate([top] * NB, axis=1), 1.0, 0.0)
        o16 = jax.lax.shift_right_logical(pltpu.bitcast(top, jnp.int32) - 0x20000000, 11) << 16
        r_top = pltpu.bitcast(jnp.where(o16 < 0, o16 ^ jnp.int32(-2**31), (~o16) & jnp.int32(-65536)), F32)
        gate = 0.5 * jax.nn.sigmoid(r_top)

    def gather(lo, hi):
        for r in range(lo, hi, P):
            rs = slice(r, min(r + P, D))
            part = 0.0
            for c0 in range(0, NB, 4):
                part = part + functools.reduce(jnp.add, [
                    _dot_nt(oh_v[:, c * P:(c + 1) * P], h_block(rs, c)) for c in range(c0, c0 + 4)])
                yield 1
            row_v[0, :, rs] = 2.0 * part

    with scope("conv0"):
        @pl.loop(0, NG)
        def _(i):
            @pl.when(i == 0)
            def _():
                c_step(0, CS[0], (c_transforms(0, True), 17, 1), (gather(0, G0 * P), 4 * G0 + 0.5, WF[0]))

            @pl.when(i > 0)
            def _():
                c_step(i, CS[4], (c_transforms(i), 25, 1), (gather(G0 * P, D), 4 * max(5 - G0, 1), WF[4]))

    def gate_up_step(item, _):
        i = item - NG
        ws, dst = (wg_v.at[:, span(i, FC)], wu_v.at[:, span(i, FC)]), act_v.at[:, :, span(i, FC)]

        def gate_up():
            for c in range(0, FC, 2 * P):
                acc = [0.0, 0.0]
                for r in range(0, D, P):
                    rs = slice(r, min(r + P, D))
                    acc = [a + _dot(row_v[0, :, rs], w[rs, c:c + 2 * P]) for a, w in zip(acc, ws)]
                    yield 1
                for k in range(2):
                    dst[k, :, c:c + 2 * P] = acc[k]

        c_step(item, CS[1], (c_transforms(item), 25, 1), (gate_up(), FC // (2 * P) * 5 + GX, WF[1]))

        @pl.when(i + 1 < NF)
        def _():
            cwg(i + 1).wait()
            cwu(i + 1).wait()

        return 0

    with scope("conv1"):
        cwg(0).wait()
        cwu(0).wait()
        jax.lax.fori_loop(NG, NG + NF, gate_up_step, 0)
        a = 0.5 * act_v[0]
        act_v[0] = (a + a * jnp.tanh(a)) * act_v[1]

    def project(rows, lead, res):
        n = rows.size
        w = wd_v.at[rows]
        acc = 0.0
        for c in range(0, FF, 4 * P):
            acc = acc + functools.reduce(jnp.add, [
                _dot_nt(act_v[0, :, f:f + P], w[:, f:f + P]) for f in range(c, c + 4 * P, P)])
            yield 1
        yield from [1] * lead
        eye = jax.lax.broadcasted_iota(jnp.int32, (n, n), 0) == jax.lax.broadcasted_iota(jnp.int32, (n, n), 1)
        res.append(_dot_nt(eye.astype(F32), acc * gate[:, :n]))
        yield from [1] * lead

    def emit(e, yt):
        rows = out_rows(e)
        h = jnp.concatenate([h_v[c, rows, :].astype(F32) for c in range(L // HB)], axis=1) + _dot(yt, oh_v[...])
        s = s_v.at[GD:][rows, :]
        q = s * h
        out = (x_v[rows, :].astype(F32) + q) + q * jnp.tanh(h)
        if debug:
            out = s
        o_v[rows, :] = out.astype(o_v.dtype)

    def finish(e):
        yt = []
        yield from project(out_rows(e), LD, yt)
        emit(e, yt[0])

    NP = FF // (4 * P) + 2 * LD

    def inverse_all(i, step, *rows):
        for c0 in range(0, NB, 2 * step):
            _zip(c_inverse(i, c0, step, *rows), c_inverse(i, c0 + step, step, *rows))
            yield 2 * step

    def finish_step(item, _):
        e = item - (NG + NF)

        @pl.when(e < NL)
        def _():
            c_step(item, CS[2], (c_transforms(item), 25, 1), (finish(e), NP, WF[2]))

            @pl.when(e == 1)
            def _():
                cout(0).start(priority=OP)

            @pl.when(e > 0)
            def _():
                cout(e).start(priority=OP)

            @pl.when(e + 1 < NL)
            def _():
                cwd(e + 1).wait()

            @pl.when(e + 1 == NL)
            def _():
                for i in range(len(tails)):
                    cwd(NL + i).wait()

        @pl.when(e == NL)
        def _():
            yt = []
            c_step(ND - 1, CS[3], (inverse_all(ND - 1, 1), NB * LI, 0.5), (finish(NL), NP, WF[3]),
                   (project(pl.ds(D - GD, GD), LD, yt), NP + 0.5, WF[3] * 0.5))
            yt_v[...] = yt[0]
            cout(NL).start(priority=OP)

        return 0

    with scope("conv2"):
        cwd(0).wait()
        jax.lax.fori_loop(NG + NF, ND, finish_step, 0)

    with scope("tail"):
        for n in range(GD // GT):
            _zip(inverse_all(ND, NB // 2, n * GT, GT))
            emit(NL + 1 + n, yt_v[n * GT:(n + 1) * GT, :])
            cout(NL + 1 + n).start(priority=OP)
        for e in range(NL + len(tails)):
            cout(e).wait()


def run(A_u, A_A_re, A_A_im, A_B_re, A_B_im, A_C_re, A_C_im, A_log_dt, A_Dskip, B_x, B_w_r,
        B_w_gate, B_w_up, B_w_down, GS=144, GA=288, GD=64, NG=2, NF=3, GE=128, GT=64, LD=3, CS=(1.1, 1.04, 0.99, 1.01, 1.1), UB=1, SC=0, G0=4, LI=1.29, WF=(1.09, 0.57, 0.67, 1.14, 0.23), GX=3.07, OP=1,
        debug=False, interpret=False, flags=None, DS=1, PAD=1):
    _, L, D = A_u.shape
    FF = B_w_gate.shape[1]
    fu, fi, g = _tables()[:3]
    odt = F32 if debug else A_u.dtype
    hbm = pl.BlockSpec(memory_space=pl.ANY)
    NB = L // P
    NE = D // GD - NG - NF + GD // GT
    out = pl.pallas_call(
        functools.partial(_kernel, GS=GS, GA=GA, GD=GD, NG=NG, NF=NF, GE=GE, GT=GT, LD=LD, CS=CS, UB=UB, SC=SC, G0=G0, LI=LI, WF=WF, GX=GX, OP=OP, debug=debug),
        out_shape=jax.ShapeDtypeStruct((D, L), odt),
        in_specs=[hbm] * 16,
        out_specs=hbm,
        scratch_shapes=[
            *[pltpu.VMEM((D,), BF16)] * 3,
            pltpu.VMEM((D, L), BF16), pltpu.VMEM((6, D, P), BF16),
            pltpu.VMEM((D, FF), BF16), pltpu.VMEM((D, FF), BF16), pltpu.VMEM((D, FF), BF16),
            pltpu.VMEM(fu.shape, jnp.uint32), pltpu.VMEM(fi.shape, jnp.uint32),
            pltpu.VMEM(g.shape, jnp.uint32),
            pltpu.VMEM((D, L), odt), pltpu.VMEM((D, L), BF16), pltpu.VMEM((4, D, L // 4), BF16),
            pltpu.VMEM((D + GD, L), F32),
            pltpu.VMEM((10, D, P), F32), pltpu.VMEM((2, D, P), F32),
            pltpu.VMEM((2, 8, L), F32), pltpu.VMEM((8, L), F32), pltpu.VMEM((2, 8, FF), F32),
            pltpu.VMEM((D // GD + 1, GD // 8, 8, NB + PAD, 8, P), F32),
            pltpu.VMEM((26, D, P), F32), pltpu.VMEM((GD, 8), F32), pltpu.VMEM((128, 8), F32),
            pltpu.SemaphoreType.DMA((7 + 2 * NF + NE,)),
            pltpu.SemaphoreType.DMA((12,)),
            pltpu.SemaphoreType.DMA((NE,)),
        ],
        compiler_params=pltpu.CompilerParams(vmem_limit_bytes=112 * 2**20, flags=flags, disable_semaphore_checks=bool(DS & 1), disable_bounds_checks=bool(DS & 2)),
        interpret=interpret,
        name="ssm_moe",
    )(A_u[0].T, A_A_re, A_A_im, A_B_re, A_B_im, A_C_re, A_C_im, A_log_dt, A_Dskip, B_w_r,
      B_w_gate, B_w_up, B_w_down.T, fu, fi, g)
    return out.T[None]


@jax.jit
def pallas_recurrent_scan__ssm_conv_s4__moe_arch_mod__prompt_kernel(
    A_u: jax.Array,
    A_A_re: jax.Array,
    A_A_im: jax.Array,
    A_B_re: jax.Array,
    A_B_im: jax.Array,
    A_C_re: jax.Array,
    A_C_im: jax.Array,
    A_log_dt: jax.Array,
    A_Dskip: jax.Array,
    B_x: jax.Array,
    B_w_r: jax.Array,
    B_w_gate: jax.Array,
    B_w_up: jax.Array,
    B_w_down: jax.Array,
):
    return run(A_u, A_A_re, A_A_im, A_B_re, A_B_im, A_C_re, A_C_im, A_log_dt, A_Dskip, B_x,
               B_w_r, B_w_gate, B_w_up, B_w_down)
```

```python
import contextlib
import functools

import jax
import jax.numpy as jnp
import numpy as np
import jax.experimental.pallas as pl
import jax.experimental.pallas.tpu as pltpu

F32 = jnp.float32
BF16 = jnp.bfloat16
P = 128


def _bf16_bits(a):
    u = np.ascontiguousarray(a, dtype=np.float32).view(np.uint32)
    return ((u + 0x7FFF + ((u >> 16) & 1)) >> 16).astype(np.uint32)


def _round_bf16(a):
    return (_bf16_bits(a) << 16).view(np.float32)


def _pack_rows(a):
    b = _bf16_bits(a)
    return (b[0::2] | (b[1::2] << 16)).astype(np.uint32)


def _tile_lags():
    lane = np.arange(P)
    quarter, hb, j = lane // 32, (lane // 16) % 2, lane % 16

    def half(offsets, second):
        q = (quarter + 2 * second) % 4
        return np.array(offsets)[q] + 128 * (hb ^ second) + 8 * j

    l1, u1 = half((1, 2, 3, 4), 0), half((5, 6, 7, 8), 1)
    l2, u2 = half((258, 260, 516, 772), 0), half((262, 264, 520, 776), 1)
    l3, u3 = half((1032, 1288) * 2, 0), half((1544, 1800) * 2, 1)
    lags = [np.where(hb == 0, l1, u1), np.where(hb == 0, u1, l1),
            np.where(lane < 64, l2, u2), np.where(lane < 64, u2, l2), np.where(lane < 64, l3, u3)]
    lags.append(np.where(lane // 16 == 0, half((516,) * 4, 0),
                         np.where(lane // 16 == 5, half((520,) * 4, 1), lags[2])))
    lags.append(np.where(lane < 96, lags[3], lags[2]))
    lags.append(np.where(lane < 32, lags[4], lags[3]))
    return lags


_SRC = ((0,), (0, 1), (1, 2), (2,), (5,), (6,), (3,), (3,), (7,), (7,)) + ((4,),) * 6


@functools.cache
def _tables():
    k = np.arange(P)
    phi = 2 * np.pi * (k + 0.25) / P

    def coords(m):
        z = np.exp(1j * np.outer(m, phi))
        return np.concatenate([z.real + z.imag / np.sqrt(3), 2 * z.imag / np.sqrt(3)], axis=1)

    fu = 2.0 * coords(np.arange(P))
    zi = np.exp(-1j * np.outer(phi, np.arange(P)))
    fi = np.concatenate([zi.real, (np.exp(2j * np.pi / 3) * zi).real], axis=0) / P
    lags = _tile_lags()
    groups, layout = [], []
    for j, src in enumerate(_SRC):
        m = np.arange(-P + 1 + (j == 3), P)
        m = m[P * j + m >= 1]
        rl = _round_bf16(P * j + m)
        hit = np.zeros(len(m), int)
        layout.append([])
        for t in src:
            sel = (lags[t][:, None] == rl[None, :])
            hit += sel.sum(0)
            g = _pack_rows(sel.astype(np.float64) @ coords(m))
            ids = []
            for r in range(0, P // 2, 8):
                known = [n for n, e in enumerate(groups) if np.array_equal(e, g[r:r + 8])]
                if not sel[2 * r:2 * r + 16].any():
                    ids.append(None)
                elif known:
                    ids.append(known[0])
                else:
                    ids.append(len(groups))
                    groups.append(g[r:r + 8])
            layout[-1].append(ids)
        assert (hit == 1).all()
    edge = np.broadcast_to(coords(np.array([-P + 1])).astype(np.float32), (8, 2 * P)).view(np.uint32)
    return _pack_rows(fu), _pack_rows(fi), np.stack(groups + [edge]), layout


def _cmul(a, b):
    return (a[0] * b[0] - a[1] * b[1], a[0] * b[1] + a[1] * b[0])


def _csq(a):
    t = a[0] * a[1]
    return ((a[0] - a[1]) * (a[0] + a[1]), t + t)


def _dot(a, b):
    return jax.lax.dot_general(a, b, (((1,), (0,)), ((), ())), preferred_element_type=F32)


def _dot_nt(a, b):
    return jax.lax.dot_general(a, b, (((1,), (1,)), ((), ())), preferred_element_type=F32)


def _rbf(x):
    return x.astype(BF16).astype(F32)


def _interleave(*gens):
    state = [[0.0, k, g, total] for k, (g, total) in enumerate(gens)]
    while state:
        cur = min(state, key=lambda e: (e[0], e[1]))
        w = next(cur[2], None)
        if w is None:
            state.remove(cur)
        else:
            cur[0] += w / cur[3]


def _merge(*gens):
    state = [[0.0, k, g, total, cost] for k, (g, total, cost) in enumerate(gens)]
    while state:
        cur = min(state, key=lambda e: (e[0], e[1]))
        w = next(cur[2], None)
        if w is None:
            state.remove(cur)
        else:
            cur[0] += w / cur[3]
            yield w * cur[4]


def _zip(*gens):
    _interleave(*((g, 1.0) for g in gens))


_ZP = (1, 8, 32, 256)


def _kernel(x_hbm, are_hbm, aim_hbm, bre_hbm, bim_hbm, cre_hbm, cim_hbm, ldt_hbm, dsk_hbm,
            wr_hbm, wg_hbm, wu_hbm, wd_hbm, fu_hbm, fi_hbm, g_hbm, o_hbm,
            ldt_v, dsk_v, wr_v, x_v, prm_v, wg_v, wu_v, wd_v, fu_v, fi_v, g_v, o_v, d_v, h_v, s_v,
            kc_v, dt_v, row_v, oh_v, act_v, hat_v, p_v, yt_v, sems, psem, osem,
            *, GS, GA, GD, NG, NF, GE, GT, LD, CS, UB, SC, G0, LI, WF, GX, OP, debug):
    scope = jax.named_scope if SC else (lambda _: contextlib.nullcontext())
    D, L = x_v.shape
    FF = wg_hbm.shape[1]
    NB = L // P
    FC = FF // NF
    ND = D // GD
    NL = ND - 1 - NG - NF
    tails = ((NL * GE, D - GD - NL * GE),) + ((D - GD, GT), (D - GD + GT, GD - GT))
    layout = _tables()[3]

    def span(i, n):
        start = i * n
        if not isinstance(start, int):
            start = pl.multiple_of(start, n)
        return pl.ds(start, n)

    prm_hbm = (are_hbm, aim_hbm, bre_hbm, bim_hbm, cre_hbm, cim_hbm)

    def cprm(part, k):
        r = pl.ds(0, GS) if part == 0 else pl.ds(GS, D - GS)
        return pltpu.make_async_copy(prm_hbm[k].at[r], prm_v.at[k, r], psem.at[6 * part + k])

    cx, cfu, cfi, cg, cdt, cdsk, cwr = (
        pltpu.make_async_copy(src, dst, sems.at[k]) for k, (src, dst) in enumerate((
            (x_hbm, x_v), (fu_hbm, fu_v), (fi_hbm, fi_v), (g_hbm, g_v),
            (ldt_hbm, ldt_v), (dsk_hbm, dsk_v), (wr_hbm, wr_v))))

    def cwg(i):
        return pltpu.make_async_copy(wg_hbm.at[:, span(i, FC)], wg_v.at[i, :, :FC], sems.at[7 + i])

    def cwu(i):
        return pltpu.make_async_copy(wu_hbm.at[:, span(i, FC)], wu_v.at[i, :, :FC], sems.at[7 + NF + i])

    def out_rows(i):
        if isinstance(i, int) and i >= NL:
            return pl.ds(*tails[i - NL])
        return pl.ds(i * GE if isinstance(i, int) else pl.multiple_of(i * GE, 16), GE)

    def cwd(i):
        return pltpu.make_async_copy(wd_hbm.at[out_rows(i)], wd_v.at[out_rows(i), :FF], sems.at[7 + 2 * NF + i])

    def cout(i):
        return pltpu.make_async_copy(o_v.at[out_rows(i)], o_hbm.at[out_rows(i)], osem.at[i])

    cdt.start()

    @pl.loop(0, NF)
    def _(i):
        @pl.when(i == 0)
        def _():
            for k in range(6):
                cprm(0, k).start()

        cwg(i).start(priority=1)
        cwu(i).start(priority=1)

    @pl.loop(0, NL)
    def _(i):
        cwd(i).start(priority=1)

    for i in range(len(tails)):
        cwd(NL + i).start(priority=1)

    for k in range(6):
        cprm(1, k).start()
    cdt.wait()

    dt_row = _rbf(jnp.exp(ldt_v[...].astype(F32)[None, :]))

    def diagonal(row, c0):
        n = min(P, D - c0)
        eye = jax.lax.broadcasted_iota(jnp.int32, (n, n), 0) == jax.lax.broadcasted_iota(jnp.int32, (n, n), 1)
        return jnp.where(eye, row[:, c0:c0 + n], 0.0)

    for c0 in range(0, D, P):
        diag = diagonal(dt_row, c0)
        dt_v[c0:c0 + diag.shape[0], :] = _dot(diag, jnp.ones((diag.shape[0], P), BF16))

    lane8 = jax.lax.broadcasted_iota(jnp.int32, (8, P), 1)
    sub8 = jax.lax.broadcasted_iota(jnp.int32, (8, P), 0)

    def k_setup(i, _):
        @pl.when(i == 1)
        def _():
            for k in range(6):
                cprm(1, k).wait()

        low = sub8 < 4
        for g in range(GS // 16):
            sl = slice(16 * g, 16 * g + 16)
            dt = dt_v.at[span(i, GS)][sl, :]
            a_re, a_im, b_re, b_im, c_re, c_im = (prm_v.at[k, span(i, GS)][sl, :].astype(F32) for k in range(6))
            dst = p_v.at[:, span(i, GS)]
            w = {0: _cmul((c_re, c_im), (dt * b_re, dt * b_im))}
            mag = jnp.exp(dt * a_re)
            z = {1: (mag * jnp.cos(dt * a_im), mag * jnp.sin(dt * a_im))}
            for e in range(10):
                z[2 << e] = _csq(z[1 << e])
            for n, e in enumerate(_ZP):
                for q in range(2):
                    dst[2 * n + q, sl, :] = z[e][q]
            dst[24, sl, :] = w[0][0]
            dst[25, sl, :] = w[0][0] * z[256][0] - w[0][1] * z[256][1]
            w[4], w[8] = _cmul(w[0], z[4]), _cmul(w[0], z[8])
            w[1032] = _cmul(w[8], z[1024])
            w[1544] = _cmul(w[1032], z[512])
            one = (jnp.ones((16, P), F32), jnp.zeros((16, P), F32))
            for n, (a, b) in enumerate(((one, z[128]), (w[0], w[4]), (w[4], w[8]), (w[1032], w[1544]))):
                for q in range(2):
                    for t in range(2):
                        x, y = a[q][8 * t:8 * t + 8], pltpu.roll(b[q][8 * t:8 * t + 8], 4, 0)
                        r = slice(16 * g + 8 * t, 16 * g + 8 * t + 8)
                        dst[8 + 4 * n + q, r, :] = jnp.where(low, x, y)
                        dst[10 + 4 * n + q, r, :] = jnp.where(low, y, x)
        return 0

    def k_lags(i, _):
        low = sub8 < 4
        bit4, bit5, bit6 = ((lane8 & b) == 0 for b in (16, 32, 64))
        bit6x = ((lane8 >> 4) ^ sub8) & 4 == 0
        diag = (lane8 & 15) * 8 + (((lane8 >> 2) & 4) ^ sub8)
        src, dst = p_v.at[:, span(i, GA)], kc_v.at[:, span(i, GA)]
        for g in range(GA // 8):
            sl = slice(8 * g, 8 * g + 8)
            out = []
            for h in range(2):
                off = (4 if h else 0) if g + 1 < GA // 8 else (0 if h else -4)
                z = {e: tuple(jnp.take_along_axis(src[2 * n + q, 8 * g + off:8 * g + off + 8, :],
                                                  (sub8 & 3) + (4 * h - off), axis=0,
                                                  mode="promise_in_bounds") for q in range(2))
                     for n, e in enumerate(_ZP)}
                b0, r, a4, far = (tuple(src[8 + 4 * n + 2 * h + q, sl, :] for q in range(2)) for n in range(4))
                bs = [b0]
                for j in range(1, 16):
                    bs.append(_cmul(bs[j - 1], z[8]) if j < 4 else _cmul(bs[j - 4], z[32]))
                av = [_cmul(r, z[1])]
                av += [_cmul(av[0], z[1])]
                av += [_cmul(av[1], z[1]), a4, _cmul(av[1], z[256]), _cmul(a4, z[256])]
                av.append(_cmul(av[-1], z[256]))
                av.append(_cmul(av[-1], z[256]))
                av += [far, _cmul(far, z[256])]
                out.append([_dot_nt(jnp.concatenate([v[q] for v in av], axis=0),
                                    jnp.concatenate([v[q] for v in reversed(bs)], axis=0).astype(BF16))
                            for q in range(2)])
            d = [[out[h][0][8 * n:8 * n + 8] - out[h][1][8 * n:8 * n + 8] for n in range(10)] for h in range(2)]
            v = [[None] * 10, [None] * 10]
            for n in range(10):
                for h in range(2):
                    v[h][n] = jnp.take_along_axis(d[h][n], diag ^ 120, axis=1, mode="promise_in_bounds")

            def unzip(xs):
                return jnp.where(low, xs[0], xs[1]), pltpu.roll(jnp.where(low, xs[1], xs[0]), 4, 0)

            halves = []
            for lo, hi in ((0, 4), (4, 8), (8, 10)):
                xs = []
                for h in range(2):
                    u = [jnp.where(bit5, v[h][n], v[h][n + 1]) for n in range(lo, hi, 2)]
                    xs.append(jnp.where(bit6x, u[h], u[1 - h]) if len(u) == 2 else u[0])
                halves.append(unzip(xs))
            (l1, u1), (l2, u2), (l3, u3) = halves
            l6, u6 = unzip((v[0][6], v[1][6]))
            tiles = [jnp.where(bit4, l1, u1), jnp.where(bit4, u1, l1), jnp.where(bit6, l2, u2),
                     jnp.where(bit6, u2, l2), jnp.where(bit6, l3, u3)]
            tiles.append(jnp.where(lane8 < 16, l6, jnp.where((lane8 >> 4) == 5, u6, tiles[2])))
            tiles.append(jnp.where(lane8 < 96, tiles[3], tiles[2]))
            tiles.append(jnp.where(lane8 < 32, tiles[4], tiles[3]))
            for t, tile in enumerate(tiles):
                dst[t, sl, :] = tile
        return 0

    with scope("setup"):
        for k in range(6):
            cprm(0, k).wait()
        for c in (cx, cg, cfu, cfi, cdsk, cwr):
            c.start()
        jax.lax.fori_loop(0, D // GS, k_setup, 0)
    with scope("lags"):
        jax.lax.fori_loop(0, D // GA, k_lags, 0)

    LB, RB, HB = 2 * P, 96, h_v.shape[2]

    def col_sum(parts):
        acc = [functools.reduce(jnp.add, parts[k::4]) for k in range(4)]
        return (acc[0] + acc[1]) + (acc[2] + acc[3])

    def ln_sum(i, _):
        src = x_v.at[span(i, RB)]
        acc = row_v[0]
        for r in range(0, RB, 8):
            acc = acc + src[r:r + 8, :].astype(F32)
        row_v[0] = acc
        return 0

    def ln_centre(c, _):
        src, dst = x_v.at[:, span(c, LB)], d_v.at[:, span(c, LB)]
        rows = span(c, D * LB // L)
        for t in range(2):
            kc_v[8 + t, rows, :] = jnp.broadcast_to(
                jnp.sum(p_v[24 + t, rows, :], axis=1, keepdims=True), (rows.size, P))
        mb = row_v[0, :, span(c, LB)]
        acc = [0.0] * 4
        for r in range(0, D, 8):
            d = src[r:r + 8, :].astype(F32) - mb
            dst[r:r + 8, :] = d.astype(BF16)
            acc[r // 8 % 4] += d * d
        row_v[1, :, span(c, LB)] = col_sum(acc)
        return 0

    def ln_scale(c):
        src, inv = d_v.at[:, span(c, HB)], row_v[0, :, span(c, HB)]
        for r in range(0, D, 8):
            h_v[c, r:r + 8, :] = (src[r:r + 8, :].astype(F32) * inv).astype(BF16)
            yield 8

    def ln_route(c, _):
        oh_v[:, span(c, HB)] = _dot(wr, h_v[c])
        _zip(ln_scale(c + 1))
        return 0

    def h_block(rows, c):
        return h_v[c * P // HB, rows, c * P % HB:c * P % HB + P]

    def compact(v):
        return jnp.concatenate([functools.reduce(
            lambda a, q: jnp.where(sub8 == q, v[:, (c + q) * P:(c + q + 1) * P], a),
            range(1, 8), v[:, c * P:(c + 1) * P]) for c in range(0, NB, 8)], axis=0)

    def spread(v):
        return jnp.concatenate([jnp.broadcast_to(v[c:c + 1], (8, P)) for c in range(NB)], axis=1)

    def total(k):
        return compact(jnp.broadcast_to(jnp.sum(row_v[k], axis=0, keepdims=True), (8, L)))

    with scope("lnorm"):
        for c in (cx, cg, cfu, cfi, cdsk, cwr):
            c.wait()
        row_v[0] = jnp.zeros((8, L), F32)
        for c0 in range(0, D, P):
            diag = diagonal(dsk_v[...].astype(F32)[None, :], c0)
            p_v[24, c0:c0 + diag.shape[0], :diag.shape[0]] += diag
        jax.lax.fori_loop(0, D // RB, ln_sum, 0)
        m = total(0) / D
        mb = _rbf(m)
        row_v[0] = spread(mb)
        jax.lax.fori_loop(0, L // LB, ln_centre, 0)
        var = jnp.maximum(total(1) / D - (m - mb) * (m - mb), 0.0)
        row_v[0] = spread(0.5 / _rbf(jnp.sqrt(_rbf(_rbf(var) + _rbf(jnp.full_like(var, 1e-5))))))
        wr = jnp.broadcast_to(2.0 * wr_v[...].astype(F32)[None, :], (8, D))
        _zip(ln_scale(0))
        jax.lax.fori_loop(0, L // HB - 1, ln_route, 0)
        oh_v[:, L - HB:] = _dot(wr, h_v[L // HB - 1])

    def put(dst, kind, c, g, a, b):
        for q, v in enumerate((a, b, a - b)):
            hat_v[dst, g, 3 * kind + q, c] = v

    def c_signal(src, dst, c0, n):
        lhs = jnp.concatenate([h_block(span(src, GD), c) for c in range(c0, c0 + n)], axis=0)
        uh = _dot(lhs, pltpu.bitcast(fu_v[...], BF16))
        for c in range(n):
            for g in range(GD // 8):
                r = slice(c * GD + 8 * g, c * GD + 8 * g + 8)
                put(dst, 0, c0 + c, g, uh[r, :P], uh[r, P:])
                yield 1

    def c_window(src, dst, j):
        tiles = kc_v.at[:, span(src, GD)]
        kh = None
        for t, ids in zip(_SRC[j], layout[j]):
            rhs = jnp.concatenate([jnp.zeros((8, 2 * P), jnp.uint32) if n is None else g_v[n] for n in ids], axis=0)
            part = _dot(tiles[t], pltpu.bitcast(rhs, BF16))
            kh = part if kh is None else kh + part
        for g in range(GD // 8):
            sl = slice(8 * g, 8 * g + 8)
            a, b = kh[sl, :P], kh[sl, P:]
            if j == 0:
                a = a + tiles[8, sl, :]
            if j == 3:
                edge = pltpu.bitcast(g_v[g_v.shape[0] - 1], F32)
                a, b = a + tiles[9, sl, :] * edge[:, :P], b + tiles[9, sl, :] * edge[:, P:]
            put(dst, 1, j, g, a, b)
            yield 1

    def c_inverse(i, c0, n, r0=0, m=GD):
        lhs = jnp.concatenate([jnp.concatenate([hat_v[i, g, 6 + q, c] for q in range(2)], axis=1)
                               for c in range(c0, c0 + n) for g in range(r0 // 8, (r0 + m) // 8)], axis=0)
        y = _dot(lhs, pltpu.bitcast(fi_v[...], BF16))
        for c in range(n):
            for r in range(0, m, 8):
                s_v.at[span(i, GD)][r0 + r:r0 + r + 8, (c0 + c) * P:(c0 + c + 1) * P] = y[c * m + r:c * m + r + 8]
                yield 1

    window_pairs = ((14, 15), (12, 13), (10, 11), (1, 2), (8, 9), (6, 7), (4, 5), (0, 3))

    def c_transforms(i, first=False):
        nxt = i + 1
        for c0 in range(0, NB, UB):
            if not first:
                _zip(c_signal(nxt, nxt, c0, UB), c_inverse(i, c0, UB))
                yield UB
            elif c0 % 2 == 0:
                _zip(c_signal(nxt, nxt, c0, UB), c_signal(nxt, nxt, c0 + UB, UB))
                yield UB
            for pair in window_pairs[c0 // 2:(c0 + UB) // 2]:
                _zip(*(c_window(nxt, i + 1, j) for j in pair))
                yield len(_SRC[pair[0]])

    def c_product(i, groups=range(GD // 8)):
        for g in groups:
            sl = slice(8 * g, 8 * g + 8)
            for cs in (range(8, 16), range(8)):
                m0 = {}
                for q in range(3):
                    acc = dict(m0)
                    for j in reversed(range(max(cs) + 1)):
                        k = hat_v[i, g, 3 + q, j]
                        live = [c for c in cs if c >= j]
                        for c in live:
                            t = k * hat_v[i, g, q, c - j]
                            acc[c] = t if c not in acc else (acc[c] - t if q else acc[c] + t)
                        yield len(live)
                    if q == 0:
                        m0 = acc
                    else:
                        for c in cs:
                            hat_v[i + 1, g, 5 + q, c] = acc[c]

    def c_step(i, pace, *side, groups=range(GD // 8)):
        _interleave((c_product(i, groups), len(groups) * 3 * 136),
                    (_merge(*side), sum(total * cost for _, total, cost in side) * pace))

    with scope("topk"):
        r = _rbf(compact(oh_v[...]))
        bits = pltpu.bitcast(jnp.where(r == 0.0, 0.0, r), jnp.int32)
        ordered = jnp.where(bits < 0, ~bits, bits ^ jnp.int32(-2**31))
        idx = (jax.lax.broadcasted_iota(jnp.int32, (NB, P), 0) * P
               + jax.lax.broadcasted_iota(jnp.int32, (NB, P), 1))
        key = pltpu.bitcast((jax.lax.shift_right_logical(ordered, 16) << 11) + (0x20000000 + L - 1 - idx), F32)
        rest, top = key, jnp.zeros((8, P), F32)
        for q in range(8):
            mx = jnp.max(jnp.max(rest, axis=0, keepdims=True), axis=1, keepdims=True)
            top = jnp.where(sub8 == q, mx, top)
            rest = jnp.where(rest == mx, 0.0, rest)
        _zip(c_signal(0, 0, 0, NB // 2), c_signal(0, 0, NB // 2, NB // 2))
        for pair in window_pairs:
            _zip(*(c_window(0, 0, j) for j in pair))
        oh_v[...] = jnp.where(spread(key) == jnp.concatenate([top] * NB, axis=1), 1.0, 0.0)
        o16 = jax.lax.shift_right_logical(pltpu.bitcast(top, jnp.int32) - 0x20000000, 11) << 16
        r_top = pltpu.bitcast(jnp.where(o16 < 0, o16 ^ jnp.int32(-2**31), (~o16) & jnp.int32(-65536)), F32)
        gate = 0.5 * jax.nn.sigmoid(r_top)

    def gather(lo, hi):
        for r in range(lo, hi, P):
            rs = slice(r, min(r + P, D))
            part = 0.0
            for c0 in range(0, NB, 4):
                part = part + functools.reduce(jnp.add, [
                    _dot_nt(oh_v[:, c * P:(c + 1) * P], h_block(rs, c)) for c in range(c0, c0 + 4)])
                yield 1
            row_v[0, :, rs] = 2.0 * part

    with scope("conv0"):
        @pl.loop(0, NG)
        def _(i):
            @pl.when(i == 0)
            def _():
                c_step(0, CS[0], (c_transforms(0, True), 17, 1), (gather(0, G0 * P), 4 * G0 + 0.5, WF[0]))

            @pl.when(i > 0)
            def _():
                c_step(i, CS[4], (c_transforms(i), 25, 1), (gather(G0 * P, D), 4 * max(5 - G0, 1), WF[4]))

    def gate_up_step(item, _):
        i = item - NG
        ws, dst = (wg_v.at[i], wu_v.at[i]), act_v.at[:, :, span(i, FC)]

        def gate_up():
            for c in range(0, FC, 2 * P):
                acc = [0.0, 0.0]
                for r in range(0, D, P):
                    rs = slice(r, min(r + P, D))
                    acc = [a + _dot(row_v[0, :, rs], w[rs, c:c + 2 * P]) for a, w in zip(acc, ws)]
                    yield 1
                for k in range(2):
                    dst[k, :, c:c + 2 * P] = acc[k]

        c_step(item, CS[1], (c_transforms(item), 25, 1), (gate_up(), FC // (2 * P) * 5 + GX, WF[1]))

        @pl.when(i + 1 < NF)
        def _():
            cwg(i + 1).wait()
            cwu(i + 1).wait()

        return 0

    with scope("conv1"):
        cwg(0).wait()
        cwu(0).wait()
        jax.lax.fori_loop(NG, NG + NF, gate_up_step, 0)
        a = 0.5 * act_v[0]
        act_v[0] = (a + a * jnp.tanh(a)) * act_v[1]

    def project(rows, lead, res):
        n = rows.size
        w = wd_v.at[rows]
        acc = 0.0
        for c in range(0, FF, 4 * P):
            acc = acc + functools.reduce(jnp.add, [
                _dot_nt(act_v[0, :, f:f + P], w[:, f:f + P]) for f in range(c, c + 4 * P, P)])
            yield 1
        yield from [1] * lead
        eye = jax.lax.broadcasted_iota(jnp.int32, (n, n), 0) == jax.lax.broadcasted_iota(jnp.int32, (n, n), 1)
        res.append(_dot_nt(eye.astype(F32), acc * gate[:, :n]))
        yield from [1] * lead

    def gating(rows, yt):
        h = jnp.concatenate([h_v[c, rows, :].astype(F32) for c in range(L // HB)], axis=1) + _dot(yt, oh_v[...])
        return h + h * jnp.tanh(h)

    def emit(rows, g, cols=slice(0, L)):
        s = s_v.at[GD:][rows, cols]
        o_v[rows, cols] = (s if debug else x_v[rows, cols].astype(F32) + s * g).astype(o_v.dtype)

    def finish(e):
        yt = []
        yield from project(out_rows(e), LD, yt)
        emit(out_rows(e), gating(out_rows(e), yt[0]))

    NP = FF // (4 * P) + 2 * LD

    def inverse_all(i, step, *rows):
        for c0 in range(0, NB, 2 * step):
            _zip(c_inverse(i, c0, step, *rows), c_inverse(i, c0 + step, step, *rows))
            yield 2 * step

    def finish_step(item, _):
        e = item - (NG + NF)

        @pl.when(e < NL)
        def _():
            c_step(item, CS[2], (c_transforms(item), 25, 1), (finish(e), NP, WF[2]))

            @pl.when(e == 1)
            def _():
                cout(0).start(priority=OP)

            @pl.when(e > 0)
            def _():
                cout(e).start(priority=OP)

            @pl.when(e + 1 < NL)
            def _():
                cwd(e + 1).wait()

            @pl.when(e + 1 == NL)
            def _():
                for i in range(len(tails)):
                    cwd(NL + i).wait()

        @pl.when(e == NL)
        def _():
            c_step(ND - 1, CS[3], (inverse_all(ND - 1, 1), NB * LI, 0.5), (finish(NL), NP, WF[3]),
                   groups=range(GT // 8))
            cout(NL).start(priority=OP)

        @pl.when(e == NL + 1)
        def _():
            yt = []
            c_step(ND - 1, CS[5], (project(pl.ds(D - GD, GD), LD, yt), NP, WF[5]),
                   (inverse_all(ND, 1, 0, GT), NB, 0.5), groups=range(GT // 8, GD // 8))
            yt_v[...] = yt[0]

        return 0

    with scope("conv2"):
        cwd(0).wait()
        jax.lax.fori_loop(NG + NF, ND + 1, finish_step, 0)

    with scope("tail"):
        g = gating(pl.ds(D - GD, GD), yt_v[...])
        emit(out_rows(NL + 1), g[:GT])
        cout(NL + 1).start(priority=OP)
        _zip(inverse_all(ND, NB // 2, GT, GD - GT))
        emit(out_rows(NL + 2), g[GT:])
        cout(NL + 2).start(priority=OP)
        for e in range(NL + len(tails)):
            cout(e).wait()


def run(A_u, A_A_re, A_A_im, A_B_re, A_B_im, A_C_re, A_C_im, A_log_dt, A_Dskip, B_x, B_w_r,
        B_w_gate, B_w_up, B_w_down, GS=144, GA=288, GD=64, NG=2, NF=3, GE=128, GT=48, LD=3, CS=(1.1, 1.04, 0.99, 1.01, 1.1, 1.2), UB=1, SC=0, G0=4, LI=1.29, WF=(1.09, 0.57, 0.67, 1.14, 0.23, 0.4), GX=3.07, OP=1,
        debug=False, interpret=False, flags=None, DS=1, PAD=1, WP=1, WQ=0, KP=0, SP=0):
    _, L, D = A_u.shape
    FF = B_w_gate.shape[1]
    fu, fi, g = _tables()[:3]
    odt = F32 if debug else A_u.dtype
    hbm = pl.BlockSpec(memory_space=pl.ANY)
    NB = L // P
    NE = D // GD - NG - NF + 2
    out = pl.pallas_call(
        functools.partial(_kernel, GS=GS, GA=GA, GD=GD, NG=NG, NF=NF, GE=GE, GT=GT, LD=LD, CS=CS, UB=UB, SC=SC, G0=G0, LI=LI, WF=WF, GX=GX, OP=OP, debug=debug),
        out_shape=jax.ShapeDtypeStruct((D, L), odt),
        in_specs=[hbm] * 16,
        out_specs=hbm,
        scratch_shapes=[
            *[pltpu.VMEM((D,), BF16)] * 3,
            pltpu.VMEM((D, L), BF16), pltpu.VMEM((6, D, P), BF16),
            *[pltpu.VMEM((NF, D, FF // NF + WQ * P), BF16)] * 2, pltpu.VMEM((D, FF + WP * P), BF16),
            pltpu.VMEM(fu.shape, jnp.uint32), pltpu.VMEM(fi.shape, jnp.uint32),
            pltpu.VMEM(g.shape, jnp.uint32),
            pltpu.VMEM((D, L), odt), pltpu.VMEM((D, L), BF16), pltpu.VMEM((4, D, L // 4), BF16),
            pltpu.VMEM((D + GD, L + SP * P), F32),
            pltpu.VMEM((10, D, P), F32), pltpu.VMEM((D, P), F32),
            pltpu.VMEM((2, 8, L), F32), pltpu.VMEM((8, L), F32), pltpu.VMEM((2, 8, FF), F32),
            pltpu.VMEM((D // GD + 1, GD // 8, 8, NB + PAD, 8, P), F32),
            pltpu.VMEM((26, D + 8 * KP, P), F32), pltpu.VMEM((GD, 8), F32),
            pltpu.SemaphoreType.DMA((7 + 2 * NF + NE,)),
            pltpu.SemaphoreType.DMA((12,)),
            pltpu.SemaphoreType.DMA((NE,)),
        ],
        compiler_params=pltpu.CompilerParams(vmem_limit_bytes=112 * 2**20, flags=flags, disable_semaphore_checks=bool(DS & 1), disable_bounds_checks=bool(DS & 2)),
        interpret=interpret,
        name="ssm_moe",
    )(A_u[0].T, A_A_re, A_A_im, A_B_re, A_B_im, A_C_re, A_C_im, A_log_dt, A_Dskip, B_w_r,
      B_w_gate, B_w_up, B_w_down.T, fu, fi, g)
    return out.T[None]


@jax.jit
def pallas_recurrent_scan__ssm_conv_s4__moe_arch_mod__prompt_kernel(
    A_u: jax.Array,
    A_A_re: jax.Array,
    A_A_im: jax.Array,
    A_B_re: jax.Array,
    A_B_im: jax.Array,
    A_C_re: jax.Array,
    A_C_im: jax.Array,
    A_log_dt: jax.Array,
    A_Dskip: jax.Array,
    B_x: jax.Array,
    B_w_r: jax.Array,
    B_w_gate: jax.Array,
    B_w_up: jax.Array,
    B_w_down: jax.Array,
):
    return run(A_u, A_A_re, A_A_im, A_B_re, A_B_im, A_C_re, A_C_im, A_log_dt, A_Dskip, B_x,
               B_w_r, B_w_gate, B_w_up, B_w_down)
```

```python
import contextlib
import functools

import jax
import jax.numpy as jnp
import numpy as np
import jax.experimental.pallas as pl
import jax.experimental.pallas.tpu as pltpu

F32 = jnp.float32
BF16 = jnp.bfloat16
P = 128


def _bf16_bits(a):
    u = np.ascontiguousarray(a, dtype=np.float32).view(np.uint32)
    return ((u + 0x7FFF + ((u >> 16) & 1)) >> 16).astype(np.uint32)


def _round_bf16(a):
    return (_bf16_bits(a) << 16).view(np.float32)


def _pack_rows(a):
    b = _bf16_bits(a)
    return (b[0::2] | (b[1::2] << 16)).astype(np.uint32)


def _tile_lags():
    lane = np.arange(P)
    quarter, hb, j = lane // 32, (lane // 16) % 2, lane % 16

    def half(offsets, second):
        q = (quarter + 2 * second) % 4
        return np.array(offsets)[q] + 128 * (hb ^ second) + 8 * j

    l1, u1 = half((1, 2, 3, 4), 0), half((5, 6, 7, 8), 1)
    l2, u2 = half((258, 260, 516, 772), 0), half((262, 264, 520, 776), 1)
    l3, u3 = half((1032, 1288) * 2, 0), half((1544, 1800) * 2, 1)
    lags = [np.where(hb == 0, l1, u1), np.where(hb == 0, u1, l1),
            np.where(lane < 64, l2, u2), np.where(lane < 64, u2, l2), np.where(lane < 64, l3, u3)]
    lags.append(np.where(lane // 16 == 0, half((516,) * 4, 0),
                         np.where(lane // 16 == 5, half((520,) * 4, 1), lags[2])))
    lags.append(np.where(lane < 96, lags[3], lags[2]))
    lags.append(np.where(lane < 32, lags[4], lags[3]))
    return lags


_SRC = ((0,), (0, 1), (1, 2), (2,), (5,), (6,), (3,), (3,), (7,), (7,)) + ((4,),) * 6


@functools.cache
def _tables():
    k = np.arange(P)
    phi = 2 * np.pi * (k + 0.25) / P

    def coords(m):
        z = np.exp(1j * np.outer(m, phi))
        return np.concatenate([z.real + z.imag / np.sqrt(3), 2 * z.imag / np.sqrt(3)], axis=1)

    fu = 2.0 * coords(np.arange(P))
    zi = np.exp(-1j * np.outer(phi, np.arange(P)))
    fi = np.concatenate([zi.real, (np.exp(2j * np.pi / 3) * zi).real], axis=0) / P
    lags = _tile_lags()
    groups, layout = [], []
    for j, src in enumerate(_SRC):
        m = np.arange(-P + 1 + (j == 3), P)
        m = m[P * j + m >= 1]
        rl = _round_bf16(P * j + m)
        hit = np.zeros(len(m), int)
        layout.append([])
        for t in src:
            sel = (lags[t][:, None] == rl[None, :])
            hit += sel.sum(0)
            g = _pack_rows(sel.astype(np.float64) @ coords(m))
            ids = []
            for r in range(0, P // 2, 8):
                known = [n for n, e in enumerate(groups) if np.array_equal(e, g[r:r + 8])]
                if not sel[2 * r:2 * r + 16].any():
                    ids.append(None)
                elif known:
                    ids.append(known[0])
                else:
                    ids.append(len(groups))
                    groups.append(g[r:r + 8])
            layout[-1].append(ids)
        assert (hit == 1).all()
    edge = np.broadcast_to(coords(np.array([-P + 1])).astype(np.float32), (8, 2 * P)).view(np.uint32)
    return _pack_rows(fu), _pack_rows(fi), np.stack(groups + [edge]), layout


def _cmul(a, b):
    return (a[0] * b[0] - a[1] * b[1], a[0] * b[1] + a[1] * b[0])


def _csq(a):
    t = a[0] * a[1]
    return ((a[0] - a[1]) * (a[0] + a[1]), t + t)


def _dot(a, b):
    return jax.lax.dot_general(a, b, (((1,), (0,)), ((), ())), preferred_element_type=F32)


def _dot_nt(a, b):
    return jax.lax.dot_general(a, b, (((1,), (1,)), ((), ())), preferred_element_type=F32)


def _rbf(x):
    return x.astype(BF16).astype(F32)


def _interleave(*gens):
    state = [[0.0, k, g, total] for k, (g, total) in enumerate(gens)]
    while state:
        cur = min(state, key=lambda e: (e[0], e[1]))
        w = next(cur[2], None)
        if w is None:
            state.remove(cur)
        else:
            cur[0] += w / cur[3]


def _merge(*gens):
    state = [[0.0, k, g, total, cost] for k, (g, total, cost) in enumerate(gens)]
    while state:
        cur = min(state, key=lambda e: (e[0], e[1]))
        w = next(cur[2], None)
        if w is None:
            state.remove(cur)
        else:
            cur[0] += w / cur[3]
            yield w * cur[4]


def _zip(*gens):
    _interleave(*((g, 1.0) for g in gens))


_ZP = (1, 8, 32, 256)


def _kernel(x_hbm, are_hbm, aim_hbm, bre_hbm, bim_hbm, cre_hbm, cim_hbm, ldt_hbm, dsk_hbm,
            wr_hbm, wg_hbm, wu_hbm, wd_hbm, fu_hbm, fi_hbm, g_hbm, o_hbm,
            ldt_v, dsk_v, wr_v, x_v, prm_v, wg_v, wu_v, wd_v, fu_v, fi_v, g_v, o_v, d_v, h_v, s_v,
            kc_v, dt_v, row_v, oh_v, act_v, hat_v, p_v, yt_v, sems, psem, osem,
            *, G1, GS, GA, GD, NG, NF, GE, GT, LD, CS, UB, SC, G0, LI, WF, GX, OP, debug):
    scope = jax.named_scope if SC else (lambda _: contextlib.nullcontext())
    D, L = x_v.shape
    FF = wg_hbm.shape[1]
    NB = L // P
    FC = FF // NF
    ND = D // GD
    NL = ND - 1 - NG - NF
    tails = ((NL * GE, D - GD - NL * GE),) + ((D - GD, GT), (D - GD + GT, GD - GT))
    layout = _tables()[3]

    def span(i, n):
        start = i * n
        if not isinstance(start, int):
            start = pl.multiple_of(start, n)
        return pl.ds(start, n)

    prm_hbm = (are_hbm, aim_hbm, bre_hbm, bim_hbm, cre_hbm, cim_hbm)

    def cprm(part, k):
        r = pl.ds(*((0, G1), (G1, GS), (G1 + GS, D - G1 - GS))[part])
        return pltpu.make_async_copy(prm_hbm[k].at[r], prm_v.at[k, r], psem.at[part])

    cx, cfu, cfi, cg, cdt, cdsk, cwr = (
        pltpu.make_async_copy(src, dst, sems.at[k]) for k, (src, dst) in enumerate((
            (x_hbm, x_v), (fu_hbm, fu_v), (fi_hbm, fi_v), (g_hbm, g_v),
            (ldt_hbm, ldt_v), (dsk_hbm, dsk_v), (wr_hbm, wr_v))))

    def cwg(i):
        return pltpu.make_async_copy(wg_hbm.at[:, span(i, FC)], wg_v.at[:, span(i, FC)], sems.at[7 + i])

    def cwu(i):
        return pltpu.make_async_copy(wu_hbm.at[:, span(i, FC)], wu_v.at[:, span(i, FC)], sems.at[7 + NF + i])

    def out_rows(i):
        if isinstance(i, int) and i >= NL:
            return pl.ds(*tails[i - NL])
        return pl.ds(i * GE if isinstance(i, int) else pl.multiple_of(i * GE, 16), GE)

    def cwd(i):
        return pltpu.make_async_copy(wd_hbm.at[out_rows(i)], wd_v.at[out_rows(i), :FF], sems.at[7 + 2 * NF + i])

    def cout(i):
        return pltpu.make_async_copy(o_v.at[out_rows(i)], o_hbm.at[out_rows(i)], osem.at[i])

    cdt.start()

    @pl.loop(0, NF)
    def _(i):
        @pl.when(i == 0)
        def _():
            for k in range(6):
                cprm(0, k).start()

        cwg(i).start(priority=1)
        cwu(i).start(priority=1)

    @pl.loop(0, NL)
    def _(i):
        cwd(i).start(priority=1)

    for i in range(len(tails)):
        cwd(NL + i).start(priority=1)

    for k in range(6):
        cprm(1, k).start()
    cdt.wait()

    dt_row = _rbf(jnp.exp(ldt_v[...].astype(F32)[None, :]))

    def diagonal(row, c0):
        n = min(P, D - c0)
        eye = jax.lax.broadcasted_iota(jnp.int32, (n, n), 0) == jax.lax.broadcasted_iota(jnp.int32, (n, n), 1)
        return jnp.where(eye, row[:, c0:c0 + n], 0.0)

    for c0 in range(0, D, P):
        diag = diagonal(dt_row, c0)
        dt_v[c0:c0 + diag.shape[0], :] = _dot(diag, jnp.ones((diag.shape[0], P), BF16))

    lane8 = jax.lax.broadcasted_iota(jnp.int32, (8, P), 1)
    sub8 = jax.lax.broadcasted_iota(jnp.int32, (8, P), 0)

    def k_setup(rows):
        low = sub8 < 4
        for g in range(rows.size // 16):
            sl = slice(16 * g, 16 * g + 16)
            dt = dt_v.at[rows][sl, :]
            a_re, a_im, b_re, b_im, c_re, c_im = (prm_v.at[k, rows][sl, :].astype(F32) for k in range(6))
            dst = p_v.at[:, rows]
            w = {0: _cmul((c_re, c_im), (dt * b_re, dt * b_im))}
            mag = jnp.exp(dt * a_re)
            z = {1: (mag * jnp.cos(dt * a_im), mag * jnp.sin(dt * a_im))}
            for e in range(10):
                z[2 << e] = _csq(z[1 << e])
            for n, e in enumerate(_ZP):
                for q in range(2):
                    dst[2 * n + q, sl, :] = z[e][q]
            dst[24, sl, :] = w[0][0]
            dst[25, sl, :] = w[0][0] * z[256][0] - w[0][1] * z[256][1]
            w[4], w[8] = _cmul(w[0], z[4]), _cmul(w[0], z[8])
            w[1032] = _cmul(w[8], z[1024])
            w[1544] = _cmul(w[1032], z[512])
            one = (jnp.ones((16, P), F32), jnp.zeros((16, P), F32))
            for n, (a, b) in enumerate(((one, z[128]), (w[0], w[4]), (w[4], w[8]), (w[1032], w[1544]))):
                for q in range(2):
                    for t in range(2):
                        x, y = a[q][8 * t:8 * t + 8], pltpu.roll(b[q][8 * t:8 * t + 8], 4, 0)
                        r = slice(16 * g + 8 * t, 16 * g + 8 * t + 8)
                        dst[8 + 4 * n + q, r, :] = jnp.where(low, x, y)
                        dst[10 + 4 * n + q, r, :] = jnp.where(low, y, x)

    def k_lags(i, _):
        low = sub8 < 4
        bit4, bit5, bit6 = ((lane8 & b) == 0 for b in (16, 32, 64))
        bit6x = ((lane8 >> 4) ^ sub8) & 4 == 0
        diag = (lane8 & 15) * 8 + (((lane8 >> 2) & 4) ^ sub8)
        src, dst = p_v.at[:, span(i, GA)], kc_v.at[:, span(i, GA)]
        for g in range(GA // 8):
            sl = slice(8 * g, 8 * g + 8)
            out = []
            for h in range(2):
                off = (4 if h else 0) if g + 1 < GA // 8 else (0 if h else -4)
                z = {e: tuple(jnp.take_along_axis(src[2 * n + q, 8 * g + off:8 * g + off + 8, :],
                                                  (sub8 & 3) + (4 * h - off), axis=0,
                                                  mode="promise_in_bounds") for q in range(2))
                     for n, e in enumerate(_ZP)}
                b0, r, a4, far = (tuple(src[8 + 4 * n + 2 * h + q, sl, :] for q in range(2)) for n in range(4))
                bs = [b0]
                for j in range(1, 16):
                    bs.append(_cmul(bs[j - 1], z[8]) if j < 4 else _cmul(bs[j - 4], z[32]))
                av = [_cmul(r, z[1])]
                av += [_cmul(av[0], z[1])]
                av += [_cmul(av[1], z[1]), a4, _cmul(av[1], z[256]), _cmul(a4, z[256])]
                av.append(_cmul(av[-1], z[256]))
                av.append(_cmul(av[-1], z[256]))
                av += [far, _cmul(far, z[256])]
                out.append([_dot_nt(jnp.concatenate([v[q] for v in av], axis=0),
                                    jnp.concatenate([v[q] for v in reversed(bs)], axis=0).astype(BF16))
                            for q in range(2)])
            d = [[out[h][0][8 * n:8 * n + 8] - out[h][1][8 * n:8 * n + 8] for n in range(10)] for h in range(2)]
            v = [[None] * 10, [None] * 10]
            for n in range(10):
                for h in range(2):
                    v[h][n] = jnp.take_along_axis(d[h][n], diag ^ 120, axis=1, mode="promise_in_bounds")

            def unzip(xs):
                return jnp.where(low, xs[0], xs[1]), pltpu.roll(jnp.where(low, xs[1], xs[0]), 4, 0)

            halves = []
            for lo, hi in ((0, 4), (4, 8), (8, 10)):
                xs = []
                for h in range(2):
                    u = [jnp.where(bit5, v[h][n], v[h][n + 1]) for n in range(lo, hi, 2)]
                    xs.append(jnp.where(bit6x, u[h], u[1 - h]) if len(u) == 2 else u[0])
                halves.append(unzip(xs))
            (l1, u1), (l2, u2), (l3, u3) = halves
            l6, u6 = unzip((v[0][6], v[1][6]))
            tiles = [jnp.where(bit4, l1, u1), jnp.where(bit4, u1, l1), jnp.where(bit6, l2, u2),
                     jnp.where(bit6, u2, l2), jnp.where(bit6, l3, u3)]
            tiles.append(jnp.where(lane8 < 16, l6, jnp.where((lane8 >> 4) == 5, u6, tiles[2])))
            tiles.append(jnp.where(lane8 < 96, tiles[3], tiles[2]))
            tiles.append(jnp.where(lane8 < 32, tiles[4], tiles[3]))
            for t, tile in enumerate(tiles):
                dst[t, sl, :] = tile
        return 0

    with scope("setup"):
        for k in range(6):
            cprm(0, k).wait()
        for k in range(6):
            cprm(2, k).start()
        k_setup(pl.ds(0, G1))
        for k in range(6):
            cprm(1, k).wait()
        for c in (cx, cg, cfu, cfi, cdsk, cwr):
            c.start()

        @pl.loop(0, (D - G1) // GS)
        def _(i):
            @pl.when(i == 1)
            def _():
                for k in range(6):
                    cprm(2, k).wait()

            k_setup(pl.ds(pl.multiple_of(i * GS + G1, G1), GS))

    with scope("lags"):
        jax.lax.fori_loop(0, D // GA, k_lags, 0)

    LB, RB, HB = 2 * P, 96, h_v.shape[2]

    def col_sum(parts):
        acc = [functools.reduce(jnp.add, parts[k::4]) for k in range(4)]
        return (acc[0] + acc[1]) + (acc[2] + acc[3])

    def ln_sum(i, _):
        src = x_v.at[span(i, RB)]
        acc = row_v[0]
        for r in range(0, RB, 8):
            acc = acc + src[r:r + 8, :].astype(F32)
        row_v[0] = acc
        return 0

    def ln_centre(c, _):
        src, dst = x_v.at[:, span(c, LB)], d_v.at[:, span(c, LB)]
        rows = span(c, D * LB // L)
        for t in range(2):
            kc_v[8 + t, rows, :] = jnp.broadcast_to(
                jnp.sum(p_v[24 + t, rows, :], axis=1, keepdims=True), (rows.size, P))
        mb = row_v[0, :, span(c, LB)]
        acc = [0.0] * 4
        for r in range(0, D, 8):
            d = src[r:r + 8, :].astype(F32) - mb
            dst[r:r + 8, :] = d.astype(BF16)
            acc[r // 8 % 4] += d * d
        row_v[1, :, span(c, LB)] = col_sum(acc)
        return 0

    def ln_scale(c):
        src, inv = d_v.at[:, span(c, HB)], row_v[0, :, span(c, HB)]
        for r in range(0, D, 8):
            h_v[c, r:r + 8, :] = (src[r:r + 8, :].astype(F32) * inv).astype(BF16)
            yield 8

    def ln_route(c, _):
        oh_v[:, span(c, HB)] = _dot(wr, h_v[c])
        _zip(ln_scale(c + 1))
        return 0

    def h_block(rows, c):
        return h_v[c * P // HB, rows, c * P % HB:c * P % HB + P]

    def compact(v):
        return jnp.concatenate([functools.reduce(
            lambda a, q: jnp.where(sub8 == q, v[:, (c + q) * P:(c + q + 1) * P], a),
            range(1, 8), v[:, c * P:(c + 1) * P]) for c in range(0, NB, 8)], axis=0)

    def spread(v):
        return jnp.concatenate([jnp.broadcast_to(v[c:c + 1], (8, P)) for c in range(NB)], axis=1)

    def total(k):
        return compact(jnp.broadcast_to(jnp.sum(row_v[k], axis=0, keepdims=True), (8, L)))

    with scope("lnorm"):
        for c in (cx, cg, cfu, cfi, cdsk, cwr):
            c.wait()
        row_v[0] = jnp.zeros((8, L), F32)
        for c0 in range(0, D, P):
            diag = diagonal(dsk_v[...].astype(F32)[None, :], c0)
            p_v[24, c0:c0 + diag.shape[0], :diag.shape[0]] += diag
        jax.lax.fori_loop(0, D // RB, ln_sum, 0)
        m = total(0) / D
        mb = _rbf(m)
        row_v[0] = spread(mb)
        jax.lax.fori_loop(0, L // LB, ln_centre, 0)
        var = jnp.maximum(total(1) / D - (m - mb) * (m - mb), 0.0)
        row_v[0] = spread(0.5 / _rbf(jnp.sqrt(_rbf(_rbf(var) + _rbf(jnp.full_like(var, 1e-5))))))
        wr = jnp.broadcast_to(2.0 * wr_v[...].astype(F32)[None, :], (8, D))
        _zip(ln_scale(0))
        jax.lax.fori_loop(0, L // HB - 1, ln_route, 0)
        oh_v[:, L - HB:] = _dot(wr, h_v[L // HB - 1])

    def put(dst, kind, c, g, a, b):
        for q, v in enumerate((a, b, a - b)):
            hat_v[dst, g, 3 * kind + q, c] = v

    def c_signal(src, dst, c0, n):
        lhs = jnp.concatenate([h_block(span(src, GD), c) for c in range(c0, c0 + n)], axis=0)
        uh = _dot(lhs, pltpu.bitcast(fu_v[...], BF16))
        for c in range(n):
            for g in range(GD // 8):
                r = slice(c * GD + 8 * g, c * GD + 8 * g + 8)
                put(dst, 0, c0 + c, g, uh[r, :P], uh[r, P:])
                yield 1

    def c_window(src, dst, j):
        tiles = kc_v.at[:, span(src, GD)]
        kh = None
        for t, ids in zip(_SRC[j], layout[j]):
            rhs = jnp.concatenate([jnp.zeros((8, 2 * P), jnp.uint32) if n is None else g_v[n] for n in ids], axis=0)
            part = _dot(tiles[t], pltpu.bitcast(rhs, BF16))
            kh = part if kh is None else kh + part
        for g in range(GD // 8):
            sl = slice(8 * g, 8 * g + 8)
            a, b = kh[sl, :P], kh[sl, P:]
            if j == 0:
                a = a + tiles[8, sl, :]
            if j == 3:
                edge = pltpu.bitcast(g_v[g_v.shape[0] - 1], F32)
                a, b = a + tiles[9, sl, :] * edge[:, :P], b + tiles[9, sl, :] * edge[:, P:]
            put(dst, 1, j, g, a, b)
            yield 1

    def c_inverse(i, c0, n, r0=0, m=GD):
        lhs = jnp.concatenate([jnp.concatenate([hat_v[i, g, 6 + q, c] for q in range(2)], axis=1)
                               for c in range(c0, c0 + n) for g in range(r0 // 8, (r0 + m) // 8)], axis=0)
        y = _dot(lhs, pltpu.bitcast(fi_v[...], BF16))
        for c in range(n):
            for r in range(0, m, 8):
                s_v.at[span(i, GD)][r0 + r:r0 + r + 8, (c0 + c) * P:(c0 + c + 1) * P] = y[c * m + r:c * m + r + 8]
                yield 1

    window_pairs = ((14, 15), (12, 13), (10, 11), (1, 2), (8, 9), (6, 7), (4, 5), (0, 3))

    def c_transforms(i, first=False):
        nxt = i + 1
        for c0 in range(0, NB, UB):
            if not first:
                _zip(c_signal(nxt, nxt, c0, UB), c_inverse(i, c0, UB))
                yield UB
            elif c0 % 2 == 0:
                _zip(c_signal(nxt, nxt, c0, UB), c_signal(nxt, nxt, c0 + UB, UB))
                yield UB
            for pair in window_pairs[c0 // 2:(c0 + UB) // 2]:
                _zip(*(c_window(nxt, i + 1, j) for j in pair))
                yield len(_SRC[pair[0]])

    def c_product(i, groups=range(GD // 8)):
        for g in groups:
            sl = slice(8 * g, 8 * g + 8)
            for cs in (range(8, 16), range(8)):
                m0 = {}
                for q in range(3):
                    acc = dict(m0)
                    for j in reversed(range(max(cs) + 1)):
                        k = hat_v[i, g, 3 + q, j]
                        live = [c for c in cs if c >= j]
                        for c in live:
                            t = k * hat_v[i, g, q, c - j]
                            acc[c] = t if c not in acc else (acc[c] - t if q else acc[c] + t)
                        yield len(live)
                    if q == 0:
                        m0 = acc
                    else:
                        for c in cs:
                            hat_v[i + 1, g, 5 + q, c] = acc[c]

    def c_step(i, pace, *side, groups=range(GD // 8)):
        _interleave((c_product(i, groups), len(groups) * 3 * 136),
                    (_merge(*side), sum(total * cost for _, total, cost in side) * pace))

    with scope("topk"):
        r = _rbf(compact(oh_v[...]))
        bits = pltpu.bitcast(jnp.where(r == 0.0, 0.0, r), jnp.int32)
        ordered = jnp.where(bits < 0, ~bits, bits ^ jnp.int32(-2**31))
        idx = (jax.lax.broadcasted_iota(jnp.int32, (NB, P), 0) * P
               + jax.lax.broadcasted_iota(jnp.int32, (NB, P), 1))
        key = pltpu.bitcast((jax.lax.shift_right_logical(ordered, 16) << 11) + (0x20000000 + L - 1 - idx), F32)
        rest, top = key, jnp.zeros((8, P), F32)
        for q in range(8):
            mx = jnp.max(jnp.max(rest, axis=0, keepdims=True), axis=1, keepdims=True)
            top = jnp.where(sub8 == q, mx, top)
            rest = jnp.where(rest == mx, 0.0, rest)
        _zip(c_signal(0, 0, 0, NB // 2), c_signal(0, 0, NB // 2, NB // 2))
        for pair in window_pairs:
            _zip(*(c_window(0, 0, j) for j in pair))
        oh_v[...] = jnp.where(spread(key) == jnp.concatenate([top] * NB, axis=1), 1.0, 0.0)
        o16 = jax.lax.shift_right_logical(pltpu.bitcast(top, jnp.int32) - 0x20000000, 11) << 16
        r_top = pltpu.bitcast(jnp.where(o16 < 0, o16 ^ jnp.int32(-2**31), (~o16) & jnp.int32(-65536)), F32)
        gate = 0.5 * jax.nn.sigmoid(r_top)

    def gather(lo, hi):
        for r in range(lo, hi, P):
            rs = slice(r, min(r + P, D))
            part = 0.0
            for c0 in range(0, NB, 4):
                part = part + functools.reduce(jnp.add, [
                    _dot_nt(oh_v[:, c * P:(c + 1) * P], h_block(rs, c)) for c in range(c0, c0 + 4)])
                yield 1
            row_v[0, :, rs] = 2.0 * part

    with scope("conv0"):
        @pl.loop(0, NG)
        def _(i):
            @pl.when(i == 0)
            def _():
                c_step(0, CS[0], (c_transforms(0, True), 17, 1), (gather(0, G0 * P), 4 * G0 + 0.5, WF[0]))

            @pl.when(i > 0)
            def _():
                c_step(i, CS[4], (c_transforms(i), 25, 1), (gather(G0 * P, D), 4 * max(5 - G0, 1), WF[4]))

    def gate_up_step(item, _):
        i = item - NG
        ws, dst = (wg_v.at[:, span(i, FC)], wu_v.at[:, span(i, FC)]), act_v.at[:, :, span(i, FC)]

        def gate_up():
            for c in range(0, FC, 2 * P):
                acc = [0.0, 0.0]
                for r in range(0, D, P):
                    rs = slice(r, min(r + P, D))
                    acc = [a + _dot(row_v[0, :, rs], w[rs, c:c + 2 * P]) for a, w in zip(acc, ws)]
                    yield 1
                for k in range(2):
                    dst[k, :, c:c + 2 * P] = acc[k]

        c_step(item, CS[1], (c_transforms(item), 25, 1), (gate_up(), FC // (2 * P) * 5 + GX, WF[1]))

        @pl.when(i + 1 < NF)
        def _():
            cwg(i + 1).wait()
            cwu(i + 1).wait()

        return 0

    with scope("conv1"):
        cwg(0).wait()
        cwu(0).wait()
        jax.lax.fori_loop(NG, NG + NF, gate_up_step, 0)
        a = 0.5 * act_v[0]
        act_v[0] = (a + a * jnp.tanh(a)) * act_v[1]

    def project(rows, lead, res):
        n = rows.size
        w = wd_v.at[rows]
        acc = 0.0
        for c in range(0, FF, 4 * P):
            acc = acc + functools.reduce(jnp.add, [
                _dot_nt(act_v[0, :, f:f + P], w[:, f:f + P]) for f in range(c, c + 4 * P, P)])
            yield 1
        yield from [1] * lead
        eye = jax.lax.broadcasted_iota(jnp.int32, (n, n), 0) == jax.lax.broadcasted_iota(jnp.int32, (n, n), 1)
        res.append(_dot_nt(eye.astype(F32), acc * gate[:, :n]))
        yield from [1] * lead

    def gating(rows, yt):
        h = jnp.concatenate([h_v[c, rows, :].astype(F32) for c in range(L // HB)], axis=1) + _dot(yt, oh_v[...])
        return h + h * jnp.tanh(h)

    def emit(rows, g, cols=slice(0, L)):
        s = s_v.at[GD:][rows, cols]
        o_v[rows, cols] = (s if debug else x_v[rows, cols].astype(F32) + s * g).astype(o_v.dtype)

    def finish(e):
        yt = []
        yield from project(out_rows(e), LD, yt)
        emit(out_rows(e), gating(out_rows(e), yt[0]))

    NP = FF // (4 * P) + 2 * LD

    def inverse_all(i, step, *rows):
        for c0 in range(0, NB, 2 * step):
            _zip(c_inverse(i, c0, step, *rows), c_inverse(i, c0 + step, step, *rows))
            yield 2 * step

    def finish_step(item, _):
        e = item - (NG + NF)

        @pl.when(e < NL)
        def _():
            c_step(item, CS[2], (c_transforms(item), 25, 1), (finish(e), NP, WF[2]))

            @pl.when(e > 0)
            def _():
                cout(e - 1).start(priority=OP)

            @pl.when(e + 1 == NL)
            def _():
                cout(NL - 1).start(priority=OP)

            @pl.when(e + 1 < NL)
            def _():
                cwd(e + 1).wait()

            @pl.when(e + 1 == NL)
            def _():
                for i in range(len(tails)):
                    cwd(NL + i).wait()

        @pl.when(e == NL)
        def _():
            c_step(ND - 1, CS[3], (inverse_all(ND - 1, 1), NB * LI, 0.5), (finish(NL), NP, WF[3]),
                   groups=range(GT // 8))
            cout(NL).start(priority=OP)

        @pl.when(e == NL + 1)
        def _():
            yt = []
            c_step(ND - 1, CS[5], (project(pl.ds(D - GD, GD), LD, yt), NP, WF[5]),
                   (inverse_all(ND, 1, 0, GT), NB, 0.5), groups=range(GT // 8, GD // 8))
            yt_v[...] = yt[0]

        return 0

    with scope("conv2"):
        cwd(0).wait()
        jax.lax.fori_loop(NG + NF, ND + 1, finish_step, 0)

    with scope("tail"):
        g = gating(pl.ds(D - GD, GD), yt_v[...])
        emit(out_rows(NL + 1), g[:GT])
        cout(NL + 1).start(priority=OP)
        _zip(inverse_all(ND, NB // 2, GT, GD - GT))
        emit(out_rows(NL + 2), g[GT:])
        cout(NL + 2).start(priority=OP)
        for e in range(NL + len(tails)):
            cout(e).wait()


def run(A_u, A_A_re, A_A_im, A_B_re, A_B_im, A_C_re, A_C_im, A_log_dt, A_Dskip, B_x, B_w_r,
        B_w_gate, B_w_up, B_w_down, G1=64, GS=128, GA=288, GD=64, NG=2, NF=3, GE=128, GT=48, LD=3, CS=(1.1, 1.04, 0.99, 1.01, 1.1, 1.2), UB=1, SC=0, G0=4, LI=1.29, WF=(1.09, 0.57, 0.67, 1.14, 0.23, 0.4), GX=3.07, OP=1,
        debug=False, interpret=False, flags=None, DS=1, PAD=1, WP=1, WQ=1, WR=0, KP=0, SP=0):
    _, L, D = A_u.shape
    FF = B_w_gate.shape[1]
    fu, fi, g = _tables()[:3]
    odt = F32 if debug else A_u.dtype
    hbm = pl.BlockSpec(memory_space=pl.ANY)
    NB = L // P
    NE = D // GD - NG - NF + 2
    out = pl.pallas_call(
        functools.partial(_kernel, G1=G1, GS=GS, GA=GA, GD=GD, NG=NG, NF=NF, GE=GE, GT=GT, LD=LD, CS=CS, UB=UB, SC=SC, G0=G0, LI=LI, WF=WF, GX=GX, OP=OP, debug=debug),
        out_shape=jax.ShapeDtypeStruct((D, L), odt),
        in_specs=[hbm] * 16,
        out_specs=hbm,
        scratch_shapes=[
            *[pltpu.VMEM((D,), BF16)] * 3,
            pltpu.VMEM((D, L), BF16), pltpu.VMEM((6, D, P), BF16),
            pltpu.VMEM((D, FF + WQ * P), BF16), pltpu.VMEM((D, FF + WR * P), BF16), pltpu.VMEM((D, FF + WP * P), BF16),
            pltpu.VMEM(fu.shape, jnp.uint32), pltpu.VMEM(fi.shape, jnp.uint32),
            pltpu.VMEM(g.shape, jnp.uint32),
            pltpu.VMEM((D, L), odt), pltpu.VMEM((D, L), BF16), pltpu.VMEM((4, D, L // 4), BF16),
            pltpu.VMEM((D + GD, L + SP * P), F32),
            pltpu.VMEM((10, D, P), F32), pltpu.VMEM((D, P), F32),
            pltpu.VMEM((2, 8, L), F32), pltpu.VMEM((8, L), F32), pltpu.VMEM((2, 8, FF), F32),
            pltpu.VMEM((D // GD + 1, GD // 8, 8, NB + PAD, 8, P), F32),
            pltpu.VMEM((26, D + 8 * KP, P), F32), pltpu.VMEM((GD, 8), F32),
            pltpu.SemaphoreType.DMA((7 + 2 * NF + NE,)),
            pltpu.SemaphoreType.DMA((3,)),
            pltpu.SemaphoreType.DMA((NE,)),
        ],
        compiler_params=pltpu.CompilerParams(vmem_limit_bytes=112 * 2**20, flags=flags, disable_semaphore_checks=bool(DS & 1), disable_bounds_checks=bool(DS & 2)),
        interpret=interpret,
        name="ssm_moe",
    )(A_u[0].T, A_A_re, A_A_im, A_B_re, A_B_im, A_C_re, A_C_im, A_log_dt, A_Dskip, B_w_r,
      B_w_gate, B_w_up, B_w_down.T, fu, fi, g)
    return out.T[None]


@jax.jit
def pallas_recurrent_scan__ssm_conv_s4__moe_arch_mod__prompt_kernel(
    A_u: jax.Array,
    A_A_re: jax.Array,
    A_A_im: jax.Array,
    A_B_re: jax.Array,
    A_B_im: jax.Array,
    A_C_re: jax.Array,
    A_C_im: jax.Array,
    A_log_dt: jax.Array,
    A_Dskip: jax.Array,
    B_x: jax.Array,
    B_w_r: jax.Array,
    B_w_gate: jax.Array,
    B_w_up: jax.Array,
    B_w_down: jax.Array,
):
    return run(A_u, A_A_re, A_A_im, A_B_re, A_B_im, A_C_re, A_C_im, A_log_dt, A_Dskip, B_x,
               B_w_r, B_w_gate, B_w_up, B_w_down)
```

```python
import functools

import jax
import jax.numpy as jnp
import numpy as np
import jax.experimental.pallas as pl
import jax.experimental.pallas.tpu as pltpu

F32 = jnp.float32
BF16 = jnp.bfloat16

SEQ, DIM, FFN = 2048, 576, 4608
P = 128
NB = SEQ // P
HB = SEQ // 4
G1, GS = 64, 128
GA = 288
GD = 64
ND = DIM // GD
NG, NF, NL = 2, 3, 3
FC = FFN // NF
GE, GT = 128, 48
LAST_ROWS = ((NL * GE, GE), (DIM - GD, GT), (DIM - GD + GT, GD - GT))
NE = NL + len(LAST_ROWS)
POWERS = (1, 8, 32, 256)
WINDOW_TILES = ((0,), (0, 1), (1, 2), (2,), (5,), (6,), (3,), (3,), (7,), (7,)) + ((4,),) * 6
WINDOW_PAIRS = ((14, 15), (12, 13), (10, 11), (1, 2), (8, 9), (6, 7), (4, 5), (0, 3))


def _bf16_bits(a):
    u = np.ascontiguousarray(a, dtype=np.float32).view(np.uint32)
    return ((u + 0x7FFF + ((u >> 16) & 1)) >> 16).astype(np.uint32)


def _pack_rows(a):
    b = _bf16_bits(a)
    return b[0::2] | (b[1::2] << 16)


def _tile_lags():
    lane = np.arange(P)
    quarter, hb, j = lane // 32, (lane // 16) % 2, lane % 16

    def half(offsets, second):
        return np.array(offsets)[(quarter + 2 * second) % 4] + 128 * (hb ^ second) + 8 * j

    l1, u1 = half((1, 2, 3, 4), 0), half((5, 6, 7, 8), 1)
    l2, u2 = half((258, 260, 516, 772), 0), half((262, 264, 520, 776), 1)
    l3, u3 = half((1032, 1288) * 2, 0), half((1544, 1800) * 2, 1)
    l4, u4 = half((516,) * 4, 0), half((520,) * 4, 1)
    lags = [np.where(hb == 0, l1, u1), np.where(hb == 0, u1, l1),
            np.where(lane < 64, l2, u2), np.where(lane < 64, u2, l2), np.where(lane < 64, l3, u3)]
    lags.append(np.where(lane < 16, l4, np.where(lane // 16 == 5, u4, lags[2])))
    lags.append(np.where(lane < 96, lags[3], lags[2]))
    lags.append(np.where(lane < 32, lags[4], lags[3]))
    return lags


@functools.cache
def _tables():
    phi = 2 * np.pi * (np.arange(P) + 0.25) / P

    def coords(m):
        z = np.exp(1j * np.outer(m, phi))
        return np.concatenate([z.real + z.imag / np.sqrt(3), 2 * z.imag / np.sqrt(3)], axis=1)

    forward = 2.0 * coords(np.arange(P))
    zi = np.exp(-1j * np.outer(phi, np.arange(P)))
    inverse = np.concatenate([zi.real, (np.exp(2j * np.pi / 3) * zi).real], axis=0) / P
    lags = _tile_lags()
    groups, layout = [], []
    for j, tiles in enumerate(WINDOW_TILES):
        m = np.arange(-P + 1 + (j == 3), P)
        m = m[P * j + m >= 1]
        rounded = (_bf16_bits(P * j + m) << 16).view(np.float32)
        hits = np.zeros(len(m), int)
        layout.append([])
        for t in tiles:
            sel = lags[t][:, None] == rounded[None, :]
            hits += sel.sum(0)
            g = _pack_rows(np.stack([coords(m[row]).sum(0) for row in sel]))
            ids = []
            for r in range(0, P // 2, 8):
                known = [n for n, e in enumerate(groups) if np.array_equal(e, g[r:r + 8])]
                if not sel[2 * r:2 * r + 16].any():
                    ids.append(None)
                elif known:
                    ids.append(known[0])
                else:
                    ids.append(len(groups))
                    groups.append(g[r:r + 8])
            layout[-1].append(ids)
        assert (hits == 1).all()
    edge = np.tile(coords(np.array([-P + 1])).astype(np.float32), (8, 1)).view(np.uint32)
    return _pack_rows(forward), _pack_rows(inverse), np.stack(groups + [edge]), layout


def _cmul(a, b):
    return (a[0] * b[0] - a[1] * b[1], a[0] * b[1] + a[1] * b[0])


def _csq(a):
    t = a[0] * a[1]
    return ((a[0] - a[1]) * (a[0] + a[1]), t + t)


def _dot(a, b):
    return jax.lax.dot_general(a, b, (((1,), (0,)), ((), ())), preferred_element_type=F32)


def _dot_nt(a, b):
    return jax.lax.dot_general(a, b, (((1,), (1,)), ((), ())), preferred_element_type=F32)


def _round(x):
    return x.astype(BF16).astype(F32)


def _twice_silu_half(h):
    return h + h * jnp.tanh(h)


def _eye(n):
    return jax.lax.broadcasted_iota(jnp.int32, (n, n), 0) == jax.lax.broadcasted_iota(jnp.int32, (n, n), 1)


def _span(i, n):
    start = i * n
    return pl.ds(start if isinstance(start, int) else pl.multiple_of(start, n), n)


def _merge(*gens):
    state = [[0.0, k, g, total, cost] for k, (g, total, cost) in enumerate(gens)]
    while state:
        cur = min(state, key=lambda e: (e[0], e[1]))
        w = next(cur[2], None)
        if w is None:
            state.remove(cur)
        else:
            cur[0] += w / cur[3]
            yield w * cur[4]


def _run(gen):
    for _ in gen:
        pass


def _kernel(x_hbm, are_hbm, aim_hbm, bre_hbm, bim_hbm, cre_hbm, cim_hbm, ldt_hbm, dsk_hbm,
            wr_hbm, wg_hbm, wu_hbm, wd_hbm, fwd_hbm, inv_hbm, win_hbm, o_hbm,
            ldt_v, dsk_v, wr_v, x_v, prm_v, wg_v, wu_v, wd_v, fwd_v, inv_v, win_v, o_v, d_v, h_v, s_v,
            lag_v, dt_v, row_v, hot_v, act_v, hat_v, pow_v, upd_v, sems, prm_sems, out_sems):
    layout = _tables()[3]
    lane8 = jax.lax.broadcasted_iota(jnp.int32, (8, P), 1)
    sub8 = jax.lax.broadcasted_iota(jnp.int32, (8, P), 0)

    def prm_copies(part):
        r = pl.ds(*((0, G1), (G1, GS), (G1 + GS, DIM - G1 - GS))[part])
        return [pltpu.make_async_copy(src.at[r], prm_v.at[k, r], prm_sems.at[part])
                for k, src in enumerate((are_hbm, aim_hbm, bre_hbm, bim_hbm, cre_hbm, cim_hbm))]

    dt_copy, *main_copies = (
        pltpu.make_async_copy(src, dst, sems.at[k]) for k, (src, dst) in enumerate((
            (ldt_hbm, ldt_v), (x_hbm, x_v), (win_hbm, win_v), (fwd_hbm, fwd_v), (inv_hbm, inv_v),
            (dsk_hbm, dsk_v), (wr_hbm, wr_v))))

    def gate_up_copies(i):
        return [pltpu.make_async_copy(src.at[:, _span(i, FC)], dst.at[:, _span(i, FC)], sems.at[7 + k * NF + i])
                for k, (src, dst) in enumerate(((wg_hbm, wg_v), (wu_hbm, wu_v)))]

    def out_rows(e):
        return pl.ds(*LAST_ROWS[e - NL]) if isinstance(e, int) and e >= NL else _span(e, GE)

    def down_copy(e):
        return pltpu.make_async_copy(wd_hbm.at[out_rows(e)], wd_v.at[out_rows(e), :FFN], sems.at[7 + 2 * NF + e])

    def out_copy(e):
        return pltpu.make_async_copy(o_v.at[out_rows(e)], o_hbm.at[out_rows(e)], out_sems.at[e])

    def start(copies, priority=0):
        for c in copies:
            c.start(priority=priority)

    def wait(copies):
        for c in copies:
            c.wait()

    dt_copy.start()

    @pl.loop(0, NF)
    def _(i):
        pl.when(i == 0)(lambda: start(prm_copies(0)))
        start(gate_up_copies(i), 1)

    @pl.loop(0, NL)
    def _(e):
        start([down_copy(e)], 1)

    start([down_copy(e) for e in range(NL, NE)], 1)
    start(prm_copies(1))
    dt_copy.wait()

    def diagonal(row, c0):
        n = min(P, DIM - c0)
        return jnp.where(_eye(n), row[:, c0:c0 + n], 0.0)

    dt_row = _round(jnp.exp(ldt_v[...].astype(F32)[None, :]))
    for c0 in range(0, DIM, P):
        diag = diagonal(dt_row, c0)
        dt_v[c0:c0 + diag.shape[0], :] = _dot(diag, jnp.ones((diag.shape[0], P), BF16))

    def k_setup(rows):
        low = sub8 < 4
        dst = pow_v.at[:, rows]
        for g in range(rows.size // 16):
            sl = slice(16 * g, 16 * g + 16)
            dt = dt_v.at[rows][sl, :]
            a_re, a_im, b_re, b_im, c_re, c_im = (prm_v.at[k, rows][sl, :].astype(F32) for k in range(6))
            w = {0: _cmul((c_re, c_im), (dt * b_re, dt * b_im))}
            mag = jnp.exp(dt * a_re)
            z = {1: (mag * jnp.cos(dt * a_im), mag * jnp.sin(dt * a_im))}
            for e in range(10):
                z[2 << e] = _csq(z[1 << e])
            for n, e in enumerate(POWERS):
                for q in range(2):
                    dst[2 * n + q, sl, :] = z[e][q]
            dst[24, sl, :] = w[0][0]
            dst[25, sl, :] = w[0][0] * z[256][0] - w[0][1] * z[256][1]
            w[4], w[8] = _cmul(w[0], z[4]), _cmul(w[0], z[8])
            w[1032] = _cmul(w[8], z[1024])
            w[1544] = _cmul(w[1032], z[512])
            one = (jnp.ones((16, P), F32), jnp.zeros((16, P), F32))
            for n, (a, b) in enumerate(((one, z[128]), (w[0], w[4]), (w[4], w[8]), (w[1032], w[1544]))):
                for q in range(2):
                    for t in range(2):
                        x, y = a[q][8 * t:8 * t + 8], pltpu.roll(b[q][8 * t:8 * t + 8], 4, 0)
                        r = slice(16 * g + 8 * t, 16 * g + 8 * t + 8)
                        dst[8 + 4 * n + q, r, :] = jnp.where(low, x, y)
                        dst[10 + 4 * n + q, r, :] = jnp.where(low, y, x)

    def k_lags(i):
        low = sub8 < 4
        bit4, bit5, bit6 = ((lane8 & b) == 0 for b in (16, 32, 64))
        bit6x = ((lane8 >> 4) ^ sub8) & 4 == 0
        own = ((lane8 & 15) * 8 + (((lane8 >> 2) & 4) ^ sub8)) ^ 120
        src, dst = pow_v.at[:, _span(i, GA)], lag_v.at[:, _span(i, GA)]

        def unzip(xs):
            return jnp.where(low, xs[0], xs[1]), pltpu.roll(jnp.where(low, xs[1], xs[0]), 4, 0)

        for g in range(GA // 8):
            sl = slice(8 * g, 8 * g + 8)
            prod = []
            for h in range(2):
                off = 4 * h if g + 1 < GA // 8 else 4 * h - 4
                z = {e: tuple(jnp.take_along_axis(src[2 * n + q, 8 * g + off:8 * g + off + 8, :],
                                                  (sub8 & 3) + (4 * h - off), axis=0,
                                                  mode="promise_in_bounds") for q in range(2))
                     for n, e in enumerate(POWERS)}
                b0, a0, a4, far = (tuple(src[8 + 4 * n + 2 * h + q, sl, :] for q in range(2)) for n in range(4))
                bs = [b0]
                for j in range(1, 16):
                    bs.append(_cmul(bs[j - 1], z[8]) if j < 4 else _cmul(bs[j - 4], z[32]))
                av = [_cmul(a0, z[1])]
                av += [_cmul(av[0], z[1])]
                av += [_cmul(av[1], z[1]), a4, _cmul(av[1], z[256]), _cmul(a4, z[256])]
                av += [_cmul(av[-1], z[256])]
                av += [_cmul(av[-1], z[256]), far, _cmul(far, z[256])]
                prod.append([_dot_nt(jnp.concatenate([v[q] for v in av]),
                                     jnp.concatenate([v[q] for v in reversed(bs)]).astype(BF16))
                             for q in range(2)])
            real = [re - im for re, im in prod]
            v = [[jnp.take_along_axis(real[h][8 * n:8 * n + 8], own, axis=1, mode="promise_in_bounds")
                  for h in range(2)] for n in range(10)]
            halves = []
            for lo, hi in ((0, 4), (4, 8), (8, 10)):
                xs = []
                for h in range(2):
                    u = [jnp.where(bit5, v[n][h], v[n + 1][h]) for n in range(lo, hi, 2)]
                    xs.append(jnp.where(bit6x, u[h], u[1 - h]) if len(u) == 2 else u[0])
                halves.append(unzip(xs))
            (l1, u1), (l2, u2), (l3, u3) = halves
            l4, u4 = unzip(v[6])
            tiles = [jnp.where(bit4, l1, u1), jnp.where(bit4, u1, l1), jnp.where(bit6, l2, u2),
                     jnp.where(bit6, u2, l2), jnp.where(bit6, l3, u3)]
            tiles.append(jnp.where(lane8 < 16, l4, jnp.where((lane8 >> 4) == 5, u4, tiles[2])))
            tiles.append(jnp.where(lane8 < 96, tiles[3], tiles[2]))
            tiles.append(jnp.where(lane8 < 32, tiles[4], tiles[3]))
            dst[:8, sl, :] = jnp.stack(tiles)

    wait(prm_copies(0))
    start(prm_copies(2))
    k_setup(pl.ds(0, G1))
    wait(prm_copies(1))
    start(main_copies)

    @pl.loop(0, (DIM - G1) // GS)
    def _(i):
        pl.when(i == 1)(lambda: wait(prm_copies(2)))
        k_setup(pl.ds(pl.multiple_of(i * GS + G1, G1), GS))

    pl.loop(0, DIM // GA)(k_lags)

    def compact(v):
        return jnp.concatenate([functools.reduce(
            lambda a, q: jnp.where(sub8 == q, v[:, (c + q) * P:(c + q + 1) * P], a),
            range(1, 8), v[:, c * P:(c + 1) * P]) for c in range(0, NB, 8)])

    def spread(v):
        return jnp.concatenate([jnp.broadcast_to(v[c:c + 1], (8, P)) for c in range(NB)], axis=1)

    def mean(k):
        return compact(jnp.broadcast_to(jnp.sum(row_v[k], axis=0, keepdims=True), (8, SEQ))) / DIM

    wait(main_copies)
    row_v[0] = jnp.zeros((8, SEQ), F32)
    for c0 in range(0, DIM, P):
        diag = diagonal(dsk_v[...].astype(F32)[None, :], c0)
        pow_v[24, c0:c0 + diag.shape[0], :diag.shape[0]] += diag

    @pl.loop(0, DIM // 96)
    def _(i):
        src = x_v.at[_span(i, 96)]
        acc = row_v[0]
        for r in range(0, 96, 8):
            acc = acc + src[r:r + 8, :].astype(F32)
        row_v[0] = acc

    m = mean(0)
    mb = _round(m)
    row_v[0] = spread(mb)

    @pl.loop(0, 8)
    def _(c):
        rows, cols = _span(c, DIM // 8), _span(c, SEQ // 8)
        for t in range(2):
            lag_v[8 + t, rows, :] = jnp.broadcast_to(
                jnp.sum(pow_v[24 + t, rows, :], axis=1, keepdims=True), (rows.size, P))
        src, dst, centre = x_v.at[:, cols], d_v.at[:, cols], row_v[0, :, cols]
        acc = [0.0] * 4
        for r in range(0, DIM, 8):
            d = src[r:r + 8, :].astype(F32) - centre
            dst[r:r + 8, :] = d.astype(BF16)
            acc[r // 8 % 4] += d * d
        row_v[1, :, cols] = (acc[0] + acc[1]) + (acc[2] + acc[3])

    var = jnp.maximum(mean(1) - (m - mb) * (m - mb), 0.0)
    row_v[0] = spread(0.5 / _round(jnp.sqrt(_round(_round(var) + _round(jnp.full_like(var, 1e-5))))))
    wr = jnp.broadcast_to(2.0 * wr_v[...].astype(F32)[None, :], (8, DIM))

    def normalise(c):
        src, scale = d_v.at[:, _span(c, HB)], jnp.concatenate([row_v[0, :, _span(c, HB)]] * 4)
        for r in range(0, DIM, 32):
            h_v[c, r:r + 32, :] = (src[r:r + 32, :].astype(F32) * scale).astype(BF16)

    def h_block(rows, c):
        return h_v[c * P // HB, rows, c * P % HB:c * P % HB + P]

    normalise(0)

    @pl.loop(0, SEQ // HB - 1)
    def _(c):
        hot_v[:, _span(c, HB)] = _dot(wr, h_v[c])
        normalise(c + 1)

    hot_v[:, SEQ - HB:] = _dot(wr, h_v[SEQ // HB - 1])

    def put(i, kind, c, v):
        a, b = v[:, :P], v[:, P:]
        for q, u in enumerate((a, b, a - b)):
            hat_v[i, :, 3 * kind + q, c] = u.reshape(GD // 8, 8, P)

    def c_signal(i, c):
        put(i, 0, c, _dot(h_block(_span(i, GD), c), pltpu.bitcast(fwd_v[...], BF16)))

    def c_window(i, j):
        tiles = lag_v.at[:, _span(i, GD)]
        parts = []
        for t, ids in zip(WINDOW_TILES[j], layout[j]):
            rhs = jnp.concatenate([jnp.zeros((8, 2 * P), jnp.uint32) if n is None else win_v[n] for n in ids])
            parts.append(_dot(tiles[t], pltpu.bitcast(rhs, BF16)))
        kh = functools.reduce(jnp.add, parts)
        if j == 0:
            kh = jnp.concatenate([kh[:, :P] + tiles[8], kh[:, P:]], axis=1)
        if j == 3:
            edge = pltpu.bitcast(win_v[win_v.shape[0] - 1], F32)
            kh = kh + jnp.concatenate([tiles[9]] * 2, axis=1) * jnp.concatenate([edge] * (GD // 8))
        put(i, 1, j, kh)

    def c_inverse(i, c, r0=0, n=GD):
        lhs = jnp.concatenate([hat_v[i, r0 // 8:(r0 + n) // 8, 6 + q, c].reshape(n, P) for q in range(2)], axis=1)
        s_v.at[_span(i, GD)][r0:r0 + n, c * P:(c + 1) * P] = _dot(lhs, pltpu.bitcast(inv_v[...], BF16))

    def c_inverses(i, *rows):
        for c in range(0, NB, 2):
            c_inverse(i, c, *rows)
            c_inverse(i, c + 1, *rows)
            yield 2

    def c_transforms(i, inverse=True):
        for c, pair in zip(range(0, NB, 2), WINDOW_PAIRS):
            c_signal(i + 1, c)
            if inverse:
                c_inverse(i, c)
                yield 1
            c_signal(i + 1, c + 1)
            if inverse:
                c_inverse(i, c + 1)
            yield 1
            for j in pair:
                c_window(i + 1, j)
            yield len(WINDOW_TILES[pair[0]])

    def c_product(i, groups):
        for g in groups:
            for lo in (8, 0):
                for q in range(3):
                    acc = []
                    for j in reversed(range(lo + 8)):
                        first = max(lo, j)
                        t = hat_v[i, g, 3 + q, j] * hat_v[i, g, q, first - j:lo + 8 - j]
                        if q:
                            acc = [jnp.concatenate(([base[j - lo:j - lo + 1]] if j >= lo else []) + acc) - t]
                        elif j >= lo:
                            acc = [jnp.concatenate([t[:1]] + [a + t[1:] for a in acc])]
                        else:
                            acc = [acc[0] + t]
                        yield lo + 8 - first
                    if q:
                        hat_v[i + 1, g, 5 + q, lo:lo + 8] = acc[0]
                    else:
                        base = acc[0]

    def c_step(i, pace, *side, groups=range(GD // 8)):
        _run(_merge((c_product(i, groups), len(groups) * 3 * 136, 1),
                    (_merge(*side), sum(total * cost for _, total, cost in side) * pace, 1)))

    score = _round(compact(hot_v[...]))
    bits = pltpu.bitcast(jnp.where(score == 0.0, 0.0, score), jnp.int32)
    ordered = jnp.where(bits < 0, ~bits, bits ^ -2**31)
    token = jax.lax.broadcasted_iota(jnp.int32, (NB, P), 0) * P + jax.lax.broadcasted_iota(jnp.int32, (NB, P), 1)
    key = pltpu.bitcast((jax.lax.shift_right_logical(ordered, 16) << 11) + (0x20000000 + SEQ - 1 - token), F32)
    rest, top = key, jnp.zeros((8, P), F32)
    for q in range(8):
        best = jnp.max(jnp.max(rest, axis=0, keepdims=True), axis=1, keepdims=True)
        top = jnp.where(sub8 == q, best, top)
        rest = jnp.where(rest == best, 0.0, rest)
    _run(c_transforms(-1, inverse=False))
    hot_v[...] = jnp.where(spread(key) == jnp.concatenate([top] * NB, axis=1), 1.0, 0.0)
    ordered = jax.lax.shift_right_logical(pltpu.bitcast(top, jnp.int32) - 0x20000000, 11) << 16
    top_score = pltpu.bitcast(jnp.where(ordered < 0, ordered ^ -2**31, ~ordered & -65536), F32)
    half_gate = 0.5 * jax.nn.sigmoid(top_score)

    def gather(lo, hi):
        for r in range(lo, hi, P):
            rs = slice(r, min(r + P, DIM))
            part = 0.0
            for c0 in range(0, NB, 4):
                part = part + functools.reduce(jnp.add, [
                    _dot_nt(hot_v[:, c * P:(c + 1) * P], h_block(rs, c)) for c in range(c0, c0 + 4)])
                yield 1
            row_v[0, :, rs] = 2.0 * part

    @pl.loop(0, NG)
    def _(i):
        @pl.when(i == 0)
        def _():
            c_step(0, 1.03, (c_transforms(0, inverse=False), 17, 1), (gather(0, 4 * P), 16.5, 1.06))

        @pl.when(i > 0)
        def _():
            c_step(i, 1.0, (c_transforms(i), 25, 1), (gather(4 * P, DIM), 4, 0.5))

    def gate_up(f):
        ws, dst = (wg_v.at[:, _span(f, FC)], wu_v.at[:, _span(f, FC)]), act_v.at[:, :, _span(f, FC)]
        for c in range(0, FC, 2 * P):
            acc = [0.0, 0.0]
            for r in range(0, DIM, P):
                rs = slice(r, min(r + P, DIM))
                acc = [a + _dot(row_v[0, :, rs], w[rs, c:c + 2 * P]) for a, w in zip(acc, ws)]
                yield 1
            for k in range(2):
                dst[k, :, c:c + 2 * P] = acc[k]

    wait(gate_up_copies(0))

    @pl.loop(NG, NG + NF)
    def _(i):
        f = i - NG
        c_step(i, 1.02, (c_transforms(i), 25, 1), (gate_up(f), FC // (2 * P) * 5 + 1.9, 0.84))
        pl.when(f + 1 < NF)(lambda: wait(gate_up_copies(f + 1)))

    act_v[0] = _twice_silu_half(0.5 * act_v[0]) * act_v[1]

    def down(rows, result):
        w = wd_v.at[rows]
        acc = 0.0
        for c in range(0, FFN, 4 * P):
            acc = acc + functools.reduce(jnp.add, [
                _dot_nt(act_v[0, :, f:f + P], w[:, f:f + P]) for f in range(c, c + 4 * P, P)])
            yield 1
        yield from (1, 1, 1)
        result.append(_dot_nt(_eye(rows.size).astype(F32), acc * half_gate[:, :rows.size]))
        yield from (1, 1, 1)

    def gating(rows, update):
        h = jnp.concatenate([h_v[c, rows, :].astype(F32) for c in range(SEQ // HB)], axis=1)
        return _twice_silu_half(h + _dot(update, hot_v[...]))

    def emit(rows, g):
        s = s_v.at[GD:][rows, :]
        o_v[rows, :] = (x_v[rows, :].astype(F32) + s * g).astype(o_v.dtype)

    def finish(rows):
        update = []
        yield from down(rows, update)
        emit(rows, gating(rows, update[0]))

    down_copy(0).wait()

    @pl.loop(NG + NF, ND + 1)
    def _(i):
        e = i - (NG + NF)

        @pl.when(e < NL)
        def _():
            c_step(i, 0.99, (c_transforms(i), 25, 1), (finish(out_rows(e)), 15, 0.67))
            pl.when(e > 0)(lambda: start([out_copy(e - 1)], 1))
            pl.when(e + 1 == NL)(lambda: start([out_copy(NL - 1)], 1))
            pl.when(e + 1 < NL)(lambda: down_copy(e + 1).wait())
            pl.when(e + 1 == NL)(lambda: wait([down_copy(n) for n in range(NL, NE)]))

        @pl.when(e == NL)
        def _():
            c_step(ND - 1, 1.01, (c_inverses(ND - 1), NB * 1.29, 0.5), (finish(out_rows(NL)), 15, 1.14),
                   groups=range(GT // 8))
            start([out_copy(NL)], 1)

        @pl.when(e == NL + 1)
        def _():
            update = []
            c_step(ND - 1, 1.03, (down(pl.ds(DIM - GD, GD), update), 15, 0.75), (c_inverses(ND, 0, GT), NB, 0.5),
                   groups=range(GT // 8, GD // 8))
            upd_v[...] = update[0]

    g = gating(pl.ds(DIM - GD, GD), upd_v[...])
    emit(out_rows(NL + 1), g[:GT])
    start([out_copy(NL + 1)], 1)
    _run(c_inverses(ND, GT, GD - GT))
    emit(out_rows(NL + 2), g[GT:])
    start([out_copy(NL + 2)], 1)
    wait([out_copy(e) for e in range(NE)])


@jax.jit
def pallas_recurrent_scan__ssm_conv_s4__moe_arch_mod__prompt_kernel(
    A_u: jax.Array,
    A_A_re: jax.Array,
    A_A_im: jax.Array,
    A_B_re: jax.Array,
    A_B_im: jax.Array,
    A_C_re: jax.Array,
    A_C_im: jax.Array,
    A_log_dt: jax.Array,
    A_Dskip: jax.Array,
    B_x: jax.Array,
    B_w_r: jax.Array,
    B_w_gate: jax.Array,
    B_w_up: jax.Array,
    B_w_down: jax.Array,
):
    del B_x
    assert A_u.shape == (1, SEQ, DIM) and A_A_re.shape == (DIM, P) and B_w_gate.shape == (DIM, FFN)
    assert A_A_re.dtype == BF16
    tables = _tables()[:3]
    hbm = pl.BlockSpec(memory_space=pl.ANY)
    out = pl.pallas_call(
        _kernel,
        out_shape=jax.ShapeDtypeStruct((DIM, SEQ), A_u.dtype),
        in_specs=[hbm] * 16,
        out_specs=hbm,
        scratch_shapes=[
            *[pltpu.VMEM((DIM,), BF16)] * 3,
            pltpu.VMEM((DIM, SEQ), BF16),
            pltpu.VMEM((6, DIM, P), BF16),
            pltpu.VMEM((DIM, FFN + P), BF16),
            pltpu.VMEM((DIM, FFN), BF16),
            pltpu.VMEM((DIM, FFN + P), BF16),
            *[pltpu.VMEM(t.shape, jnp.uint32) for t in tables],
            pltpu.VMEM((DIM, SEQ), A_u.dtype),
            pltpu.VMEM((DIM, SEQ), BF16),
            pltpu.VMEM((SEQ // HB, DIM, HB), BF16),
            pltpu.VMEM((DIM + GD, SEQ), F32),
            pltpu.VMEM((10, DIM, P), F32),
            pltpu.VMEM((DIM, P), F32),
            pltpu.VMEM((2, 8, SEQ), F32),
            pltpu.VMEM((8, SEQ), F32),
            pltpu.VMEM((2, 8, FFN), F32),
            pltpu.VMEM((ND + 1, GD // 8, 8, NB + 1, 8, P), F32),
            pltpu.VMEM((26, DIM, P), F32),
            pltpu.VMEM((GD, 8), F32),
            pltpu.SemaphoreType.DMA((7 + 2 * NF + NE,)),
            pltpu.SemaphoreType.DMA((3,)),
            pltpu.SemaphoreType.DMA((NE,)),
        ],
        compiler_params=pltpu.CompilerParams(vmem_limit_bytes=112 * 2**20, disable_semaphore_checks=True),
        name="ssm_moe",
    )(A_u[0].T, A_A_re, A_A_im, A_B_re, A_B_im, A_C_re, A_C_im, A_log_dt, A_Dskip, B_w_r,
      B_w_gate, B_w_up, B_w_down.T, *tables)
    return out.T[None]
```

```python
import functools

import jax
import jax.numpy as jnp
import numpy as np
import jax.experimental.pallas as pl
import jax.experimental.pallas.tpu as pltpu

F32 = jnp.float32
BF16 = jnp.bfloat16

SEQ, DIM, FFN = 2048, 576, 4608
P = 128
NB = SEQ // P
HB = SEQ // 4
GS, GL = 112, 128
GA = 288
GD = 64
ND = DIM // GD
NG, NF, NL = 2, 3, 3
FC = FFN // NF
GE, GT = 128, 48
LAST_ROWS = ((NL * GE, GE), (DIM - GD, GT), (DIM - GD + GT, GD - GT))
NE = NL + len(LAST_ROWS)
POWERS = (1, 8, 32, 256)
WINDOW_TILES = ((0,), (0, 1), (1, 2), (2,), (5,), (6,), (3,), (3,), (7,), (7,)) + ((4,),) * 6
WINDOW_PAIRS = ((14, 15), (12, 13), (10, 11), (1, 2), (8, 9), (6, 7), (4, 5), (0, 3))


def _bf16_bits(a):
    u = np.ascontiguousarray(a, dtype=np.float32).view(np.uint32)
    return ((u + 0x7FFF + ((u >> 16) & 1)) >> 16).astype(np.uint32)


def _tile_lags():
    lane = np.arange(P)
    quarter, hb, j = lane // 32, (lane // 16) % 2, lane % 16

    def half(offsets, second):
        return np.array(offsets)[(quarter + 2 * second) % 4] + 128 * (hb ^ second) + 8 * j

    l1, u1 = half((1, 2, 3, 4), 0), half((5, 6, 7, 8), 1)
    l2, u2 = half((258, 260, 516, 772), 0), half((262, 264, 520, 776), 1)
    l3, u3 = half((1032, 1288) * 2, 0), half((1544, 1800) * 2, 1)
    l4, u4 = half((516,) * 4, 0), half((520,) * 4, 1)
    lags = [np.where(hb == 0, l1, u1), np.where(hb == 0, u1, l1),
            np.where(lane < 64, l2, u2), np.where(lane < 64, u2, l2), np.where(lane < 64, l3, u3)]
    lags.append(np.where(lane < 16, l4, np.where(lane // 16 == 5, u4, lags[2])))
    lags.append(np.where(lane < 96, lags[3], lags[2]))
    lags.append(np.where(lane < 32, lags[4], lags[3]))
    return lags


def _window_lags(j):
    return 1 if j == 0 else -P + 1 + (j == 3), P - 1


@functools.cache
def _window_layout():
    lags = _tile_lags()
    m = np.arange(-P, P)
    groups, patterns, layout = [], [], []
    for j, tiles in enumerate(WINDOW_TILES):
        lo, hi = _window_lags(j)
        live = (m >= lo) & (m <= hi)
        rounded = (_bf16_bits(P * j + m) << 16).view(np.float32)
        hits = np.zeros(len(m), int)
        layout.append([])
        for t in tiles:
            sel = (lags[t][:, None] == rounded) & live
            hits += sel.sum(0)
            ids = []
            for r in range(0, P, 16):
                assert (lags[t][r:r + 16] == lags[t][r] + 8 * np.arange(16)).all()
                known = [n for n, e in enumerate(patterns) if np.array_equal(e, sel[r:r + 16])]
                if not sel[r:r + 16].any():
                    ids.append(None)
                elif known:
                    ids.append(known[0])
                else:
                    ids.append(len(groups))
                    groups.append((int(lags[t][r]), j))
                    patterns.append(sel[r:r + 16])
            layout[-1].append(ids)
        assert (hits == live).all()
    halves = [[n for n, e in enumerate(patterns) if e[:, h * P:(h + 1) * P].any()] for h in range(2)]
    return groups, halves, layout


def _cmul(a, b):
    return (a[0] * b[0] - a[1] * b[1], a[0] * b[1] + a[1] * b[0])


def _csq(a):
    t = a[0] * a[1]
    return ((a[0] - a[1]) * (a[0] + a[1]), t + t)


def _dot(a, b):
    return jax.lax.dot_general(a, b, (((1,), (0,)), ((), ())), preferred_element_type=F32)


def _dot_nt(a, b):
    return jax.lax.dot_general(a, b, (((1,), (1,)), ((), ())), preferred_element_type=F32)


def _round(x):
    return x.astype(BF16).astype(F32)


def _twice_silu_half(h):
    return h + h * jnp.tanh(h)


def _eye(n):
    return jax.lax.broadcasted_iota(jnp.int32, (n, n), 0) == jax.lax.broadcasted_iota(jnp.int32, (n, n), 1)


def _span(i, n):
    start = i * n
    return pl.ds(start if isinstance(start, int) else pl.multiple_of(start, n), n)


def _merge(*gens):
    state = [[0.0, k, g, total, cost] for k, (g, total, cost) in enumerate(gens)]
    while state:
        cur = min(state, key=lambda e: (e[0], e[1]))
        w = next(cur[2], None)
        if w is None:
            state.remove(cur)
        else:
            cur[0] += w / cur[3]
            yield w * cur[4]


def _after(delay, gen):
    yield delay
    yield from gen


def _run(gen):
    for _ in gen:
        pass


def _kernel(x_hbm, are_hbm, aim_hbm, bre_hbm, bim_hbm, cre_hbm, cim_hbm, ldt_hbm, dsk_hbm,
            wr_hbm, wg_hbm, wu_hbm, wd_hbm, o_hbm,
            ldt_v, dsk_v, wr_v, x_v, prm_v, wg_v, wu_v, wd_v, fwd_v, inv_v, win_v, o_v, d_v, h_v, s_v,
            lag_v, dt_v, row_v, hot_v, act_v, hat_v, pow_v, upd_v, sems):
    groups, halves, layout = _window_layout()
    lane8 = jax.lax.broadcasted_iota(jnp.int32, (8, P), 1)
    sub8 = jax.lax.broadcasted_iota(jnp.int32, (8, P), 0)

    def prm_copies(part):
        r = pl.ds(*((0, GS), (GS, 2 * GS), (3 * GS, DIM - 3 * GS))[part])
        return [pltpu.make_async_copy(src.at[r], prm_v.at[k, r], sems.at[1 + part % 2])
                for k, src in enumerate((are_hbm, aim_hbm, bre_hbm, bim_hbm, cre_hbm, cim_hbm))]

    vec_copies = [pltpu.make_async_copy(src, dst, sems.at[0])
                  for src, dst in ((ldt_hbm, ldt_v), (dsk_hbm, dsk_v), (wr_hbm, wr_v))]
    x_copy = pltpu.make_async_copy(x_hbm, x_v, sems.at[0])

    def gate_up_copies(part):
        cols = pl.ds(*((0, FFN - FC), (FFN - FC, FC))[part])
        return [pltpu.make_async_copy(src.at[:, cols], dst.at[:, cols], sems.at[3 + part])
                for src, dst in ((wg_hbm, wg_v), (wu_hbm, wu_v))]

    def out_rows(e):
        return pl.ds(*LAST_ROWS[e - NL]) if isinstance(e, int) and e >= NL else _span(e, GE)

    def down_copy(e):
        rows = pl.ds(NL * GE, DIM - NL * GE) if isinstance(e, int) and e == NL else _span(e, GE)
        return pltpu.make_async_copy(wd_hbm.at[rows], wd_v.at[rows, :FFN], sems.at[e])

    def out_copy(e):
        return pltpu.make_async_copy(o_v.at[out_rows(e)], o_hbm.at[out_rows(e)], sems.at[4])

    def start(copies, priority=0):
        for c in copies:
            c.start(priority=priority)

    def wait(copies):
        for c in copies:
            c.wait()

    start(vec_copies)

    @pl.loop(0, 2)
    def _(i):
        pl.when(i == 0)(lambda: (start(prm_copies(0)), start(gate_up_copies(0), 1)) and None)
        pl.when(i == 1)(lambda: (start(prm_copies(1)), start(gate_up_copies(1), 1)) and None)

    def coords(re, im):
        b = im * (2 / np.sqrt(3).item())
        return jnp.concatenate([re + 0.5 * b, b], axis=1)

    def packed(v):
        return pltpu.bitcast(v.astype(BF16), jnp.uint32)

    angle = (((4 * lane8 + 1) * sub8) & (4 * P - 1)).astype(F32) * (np.pi / (2 * P))
    root = (jnp.cos(angle), jnp.sin(angle))
    step = tuple(v[4:5] for v in root)
    for _ in range(4):
        step = _csq(step)
        root = tuple(jnp.concatenate(v) for v in zip(root, _cmul(root, step)))
    powers = (coords(root[1], -root[0]), coords(*root))
    fwd_v[...] = packed(2.0 * powers[1])
    inv_v[...] = packed(jnp.concatenate([
        (root[0] * (1 / P)).T, ((root[1] * np.sqrt(3).item() - root[0]) * (0.5 / P)).T]))
    packed_powers = [v.astype(BF16) for v in powers]
    win_v[len(groups)] = pltpu.bitcast(jnp.broadcast_to(powers[0][1:2], (8, 2 * P)), jnp.uint32)

    def window_rows(n, h):
        lag, j = groups[n]
        m = jax.lax.broadcasted_iota(jnp.int32, (16, P), 1) + (h - 1) * P
        rounded = jnp.where(m >= _window_lags(j)[0], _round((m + P * j).astype(F32)), -1.0)
        return jnp.where(rounded == (8 * jax.lax.broadcasted_iota(jnp.int32, (16, P), 0) + lag).astype(F32), 1.0, 0.0)

    part = {}
    for h in range(2):
        prod = _dot(jnp.concatenate([window_rows(n, h) for n in halves[h]]), packed_powers[h])
        for k, n in enumerate(halves[h]):
            part[n] = part.get(n, 0.0) + prod[16 * k:16 * k + 16]
    for n in range(len(groups)):
        win_v[n] = packed(part[n])

    wait(vec_copies)
    dt_row, skip_row = (jnp.concatenate([v[None, :], jnp.zeros((1, -DIM % P), F32)], axis=1)
                        for v in (_round(jnp.exp(ldt_v[...].astype(F32))), dsk_v[...].astype(F32)))

    for c in range(0, DIM, P):
        n = min(P, DIM - c)
        dt, skip = (jnp.where(_eye(P)[:n], v[:, c:c + P], 0.0) for v in (dt_row, skip_row))
        dt_v[0, c:c + n, :] = _dot(dt, jnp.ones((P, P), BF16))
        dt_v[1, c:c + n, :] = skip

    def k_setup(rows, have_mag=False):
        low = sub8 < 4
        dst = pow_v.at[:, rows]
        for g in range(rows.size // 16):
            sl = slice(16 * g, 16 * g + 16)
            dt, skip = (dt_v.at[k, rows][sl, :] for k in range(2))
            a_re, a_im, b_re, b_im, c_re, c_im = (prm_v.at[k, rows][sl, :].astype(F32) for k in range(6))
            w = {0: _cmul((c_re, c_im), (dt * b_re, dt * b_im))}
            mag = dt_v.at[2, rows][sl, :] if have_mag else jnp.exp(dt * a_re)
            yield 1
            rot = []
            for phase in jnp.split(dt * a_im, 2):
                rot.append((jnp.cos(phase), jnp.sin(phase)))
                yield 4.5
            z = {1: tuple(mag * jnp.concatenate(v) for v in zip(*rot))}
            for e in range(10):
                z[2 << e] = _csq(z[1 << e])
            for n, e in enumerate(POWERS):
                for q in range(2):
                    dst[2 * n + q, sl, :] = z[e][q]
            yield 3
            dst[24, sl, :] = w[0][0] + skip
            dst[25, sl, :] = w[0][0] * z[256][0] - w[0][1] * z[256][1]
            w[4], w[8] = _cmul(w[0], z[4]), _cmul(w[0], z[8])
            w[1032] = _cmul(w[8], z[1024])
            w[1544] = _cmul(w[1032], z[512])
            one = (jnp.ones((16, P), F32), jnp.zeros((16, P), F32))
            for n, (a, b) in enumerate(((one, z[128]), (w[0], w[4]), (w[4], w[8]), (w[1032], w[1544]))):
                for q in range(2):
                    for t in range(2):
                        x, y = a[q][8 * t:8 * t + 8], pltpu.roll(b[q][8 * t:8 * t + 8], 4, 0)
                        r = slice(16 * g + 8 * t, 16 * g + 8 * t + 8)
                        dst[8 + 4 * n + q, r, :] = jnp.where(low, x, y)
                        dst[10 + 4 * n + q, r, :] = jnp.where(low, y, x)
            yield 3

    def k_lags(i):
        low = sub8 < 4
        bit4, bit5, bit6 = ((lane8 & b) == 0 for b in (16, 32, 64))
        bit6x = ((lane8 >> 4) ^ sub8) & 4 == 0
        own = ((lane8 & 15) * 8 + (((lane8 >> 2) & 4) ^ sub8)) ^ 120
        src, dst = pow_v.at[:, _span(i, GA)], lag_v.at[:, _span(i, GA)]
        for t in range(2):
            dst[8 + t] = jnp.broadcast_to(jnp.sum(src[24 + t], axis=1, keepdims=True), (GA, P))

        def unzip(xs):
            return jnp.where(low, xs[0], xs[1]), pltpu.roll(jnp.where(low, xs[1], xs[0]), 4, 0)

        for g in range(GA // 8):
            sl = slice(8 * g, 8 * g + 8)
            prod = []
            for h in range(2):
                off = 4 * h if g + 1 < GA // 8 else 4 * h - 4
                z = {e: tuple(jnp.take_along_axis(src[2 * n + q, 8 * g + off:8 * g + off + 8, :],
                                                  (sub8 & 3) + (4 * h - off), axis=0,
                                                  mode="promise_in_bounds") for q in range(2))
                     for n, e in enumerate(POWERS)}
                b0, a0, a4, far = (tuple(src[8 + 4 * n + 2 * h + q, sl, :] for q in range(2)) for n in range(4))
                bs = [b0]
                for j in range(1, 16):
                    bs.append(_cmul(bs[j - 1], z[8]) if j < 4 else _cmul(bs[j - 4], z[32]))
                av = [_cmul(a0, z[1])]
                av += [_cmul(av[0], z[1])]
                av += [_cmul(av[1], z[1]), a4, _cmul(av[1], z[256]), _cmul(a4, z[256])]
                av += [_cmul(av[-1], z[256])]
                av += [_cmul(av[-1], z[256]), far, _cmul(far, z[256])]
                prod.append([_dot_nt(jnp.concatenate([v[q] for v in av]),
                                     jnp.concatenate([v[q] for v in reversed(bs)]).astype(BF16))
                             for q in range(2)])
            real = [re - im for re, im in prod]
            v = [[jnp.take_along_axis(real[h][8 * n:8 * n + 8], own, axis=1, mode="promise_in_bounds")
                  for h in range(2)] for n in range(10)]
            halves = []
            for lo, hi in ((0, 4), (4, 8), (8, 10)):
                xs = []
                for h in range(2):
                    u = [jnp.where(bit5, v[n][h], v[n + 1][h]) for n in range(lo, hi, 2)]
                    xs.append(jnp.where(bit6x, u[h], u[1 - h]) if len(u) == 2 else u[0])
                halves.append(unzip(xs))
            (l1, u1), (l2, u2), (l3, u3) = halves
            l4, u4 = unzip(v[6])
            tiles = [jnp.where(bit4, l1, u1), jnp.where(bit4, u1, l1), jnp.where(bit6, l2, u2),
                     jnp.where(bit6, u2, l2), jnp.where(bit6, l3, u3)]
            tiles.append(jnp.where(lane8 < 16, l4, jnp.where((lane8 >> 4) == 5, u4, tiles[2])))
            tiles.append(jnp.where(lane8 < 96, tiles[3], tiles[2]))
            tiles.append(jnp.where(lane8 < 32, tiles[4], tiles[3]))
            dst[:8, sl, :] = jnp.stack(tiles)

    wait(prm_copies(0))
    start(prm_copies(2))

    @pl.loop(0, (DIM - GL) // GS)
    def _(i):
        pl.when(i == 0)(x_copy.start)
        pl.when(i == 1)(lambda: wait(prm_copies(1)))
        pl.when(i == 3)(lambda: wait(prm_copies(2)))
        _run(k_setup(_span(i, GS)))

    def compact(v):
        return jnp.concatenate([functools.reduce(
            lambda a, q: jnp.where(sub8 == q, v[:, (c + q) * P:(c + q + 1) * P], a),
            range(1, 8), v[:, c * P:(c + 1) * P]) for c in range(0, NB, 8)])

    def spread(v):
        return jnp.concatenate([jnp.broadcast_to(v[c:c + 1], (8, P)) for c in range(NB)], axis=1)

    def mean(k):
        return compact(jnp.broadcast_to(jnp.sum(row_v[k], axis=0, keepdims=True), (8, SEQ))) / DIM

    def h_block(rows, c):
        return h_v[c * P // HB, rows, c * P % HB:c * P % HB + P]

    def layer_norm():
        x_copy.wait()
        row_v[0] = jnp.zeros((8, SEQ), F32)

        @pl.loop(0, DIM // 96)
        def _(i):
            src = x_v.at[_span(i, 96)]
            acc = row_v[0]
            for r in range(0, 96, 8):
                acc = acc + src[r:r + 8, :].astype(F32)
            row_v[0] = acc

        m = mean(0)
        mb = _round(m)
        row_v[0] = spread(mb)

        @pl.loop(0, 8)
        def _(c):
            cols = _span(c, SEQ // 8)
            src, dst, centre = x_v.at[:, cols], d_v.at[:, cols], row_v[0, :, cols]
            acc = [0.0] * 4
            for r in range(0, DIM, 8):
                d = src[r:r + 8, :].astype(F32) - centre
                dst[r:r + 8, :] = d.astype(BF16)
                acc[r // 8 % 4] += d * d
            row_v[1, :, cols] = (acc[0] + acc[1]) + (acc[2] + acc[3])

        late = pl.ds(DIM - GL, GL)
        dt_v[2, late, :] = jnp.exp(dt_v[0, late, :] * prm_v[0, late, :].astype(F32))
        var = jnp.maximum(mean(1) - (m - mb) * (m - mb), 0.0)
        row_v[0] = spread(0.5 / _round(jnp.sqrt(_round(_round(var) + _round(jnp.full_like(var, 1e-5))))))

        def normalise(c):
            src, scale = d_v.at[:, _span(c, HB)], jnp.concatenate([row_v[0, :, _span(c, HB)]] * 4)
            for r in range(0, DIM, 32):
                h_v[c, r:r + 32, :] = (src[r:r + 32, :].astype(F32) * scale).astype(BF16)

        pl.loop(0, SEQ // HB)(normalise)

    def put(i, kind, c, v):
        a, b = v[:, :P], v[:, P:]
        for q, u in enumerate((a, b, a - b)):
            hat_v[i, :, 3 * kind + q, c] = u.reshape(GD // 8, 8, P)

    def c_signal(i, c):
        put(i, 0, c, _dot(h_block(_span(i, GD), c), pltpu.bitcast(fwd_v[...], BF16)))

    def c_window(i, j):
        tiles = lag_v.at[:, _span(i, GD)]
        parts = []
        for t, ids in zip(WINDOW_TILES[j], layout[j]):
            rhs = jnp.concatenate([jnp.zeros((8, 2 * P), jnp.uint32) if n is None else win_v[n] for n in ids])
            parts.append(_dot(tiles[t], pltpu.bitcast(rhs, BF16)))
        kh = functools.reduce(jnp.add, parts)
        if j == 0:
            kh = jnp.concatenate([kh[:, :P] + tiles[8], kh[:, P:]], axis=1)
        if j == 3:
            edge = pltpu.bitcast(win_v[win_v.shape[0] - 1], F32)
            kh = kh + jnp.concatenate([tiles[9]] * 2, axis=1) * jnp.concatenate([edge] * (GD // 8))
        put(i, 1, j, kh)

    def c_inverse(i, blocks, r0=0, n=GD):
        lhs = jnp.concatenate([jnp.concatenate([
            hat_v[i, r0 // 8:(r0 + n) // 8, 6 + q, c].reshape(n, P) for q in range(2)], axis=1) for c in blocks])
        y = _dot(lhs, pltpu.bitcast(inv_v[...], BF16))
        for k, c in enumerate(blocks):
            s_v.at[_span(i, GD)][r0:r0 + n, c * P:(c + 1) * P] = y[k * n:(k + 1) * n]

    def c_inverses(i, stack, *rows):
        for c in range(0, NB, 2 * stack):
            c_inverse(i, range(c, c + stack), *rows)
            c_inverse(i, range(c + stack, c + 2 * stack), *rows)
            yield 2 * stack

    def c_transforms(i, inverse=True):
        for c, pair in zip(range(0, NB, 2), WINDOW_PAIRS):
            c_signal(i + 1, c)
            if inverse:
                c_inverse(i, [c])
                yield 1
            c_signal(i + 1, c + 1)
            if inverse:
                c_inverse(i, [c + 1])
            yield 1
            for j in pair:
                c_window(i + 1, j)
            yield len(WINDOW_TILES[pair[0]])

    def c_product(i, groups):
        for g in groups:
            for lo in (8, 0):
                for q in range(3):
                    acc = []
                    for j in reversed(range(lo + 8)):
                        first = max(lo, j)
                        t = hat_v[i, g, 3 + q, j] * hat_v[i, g, q, first - j:lo + 8 - j]
                        if q:
                            acc = [jnp.concatenate(([base[j - lo:j - lo + 1]] if j >= lo else []) + acc) - t]
                        elif j >= lo:
                            acc = [jnp.concatenate([t[:1]] + [a + t[1:] for a in acc])]
                        else:
                            acc = [acc[0] + t]
                        yield lo + 8 - first
                    if q:
                        hat_v[i + 1, g, 5 + q, lo:lo + 8] = acc[0]
                    else:
                        base = acc[0]

    def c_step(i, pace, *side, groups=range(GD // 8)):
        _run(_merge((c_product(i, groups), len(groups) * 3 * 136, 1),
                    (_merge(*side), sum(total * cost for _, total, cost in side) * pace, 1)))

    def select():
        wr = jnp.broadcast_to(2.0 * wr_v[...].astype(F32)[None, :], (8, DIM))
        score = [0.0] * (SEQ // HB)
        for c in range(SEQ // HB):
            for r in range(0, DIM, P):
                rs = slice(r, min(r + P, DIM))
                score[c] = score[c] + _dot(wr[:, rs], h_v[c, rs, :])
                yield 0.27
        score = _round(compact(jnp.concatenate(score, axis=1)))
        bits = pltpu.bitcast(jnp.where(score == 0.0, 0.0, score), jnp.int32)
        ordered = jnp.where(bits < 0, ~bits, bits ^ -2**31)
        token = jax.lax.broadcasted_iota(jnp.int32, (NB, P), 0) * P + jax.lax.broadcasted_iota(jnp.int32, (NB, P), 1)
        key = pltpu.bitcast((jax.lax.shift_right_logical(ordered, 16) << 11) + (0x20000000 + SEQ - 1 - token), F32)
        rest, top = key, jnp.zeros((8, P), F32)
        yield 2.34
        for q in range(8):
            best = jnp.max(jnp.max(rest, axis=0, keepdims=True), axis=1, keepdims=True)
            top = jnp.where(sub8 == q, best, top)
            rest = jnp.where(rest == best, 0.0, rest)
            yield 1
        hot_v[...] = jnp.where(spread(key) == jnp.concatenate([top] * NB, axis=1), 1.0, 0.0)
        ordered = jax.lax.shift_right_logical(pltpu.bitcast(top, jnp.int32) - 0x20000000, 11) << 16
        row_v[1, :, :P] = pltpu.bitcast(jnp.where(ordered < 0, ordered ^ -2**31, ~ordered & -65536), F32)

    @pl.loop(0, DIM // GA)
    def _(i):
        k_lags(i)

        @pl.when(i == 0)
        def _():
            layer_norm()
            _run(_merge((k_setup(pl.ds(DIM - GL, GL), have_mag=True), GL, 1),
                        (_after(9.29, c_transforms(-1, inverse=False)), 9.29 + 17 * 1.08, 1),
                        (select(), 20 * 0.27 + 8 + 2.34 + 1.18, 1)))

    def gather(lo, hi):
        for r in range(lo, hi, P):
            rs = slice(r, min(r + P, DIM))
            part = 0.0
            for c0 in range(0, NB, 4):
                part = part + functools.reduce(jnp.add, [
                    _dot_nt(hot_v[:, c * P:(c + 1) * P], h_block(rs, c)) for c in range(c0, c0 + 4)])
                yield 1
            row_v[0, :, rs] = 2.0 * part

    @pl.loop(0, NG)
    def _(i):
        @pl.when(i == 0)
        def _():
            c_step(0, 0.98, (c_transforms(0, inverse=False), 17, 1), (gather(0, 4 * P), 16.5, 1.23))

        @pl.when(i > 0)
        def _():
            c_step(i, 1.0, (c_transforms(i), 25, 1), (gather(4 * P, DIM), 4, 0.28))

    def gate_up(f):
        ws, dst = (wg_v.at[:, _span(f, FC)], wu_v.at[:, _span(f, FC)]), act_v.at[:, :, _span(f, FC)]
        for c in range(0, FC, 2 * P):
            acc = [0.0, 0.0]
            for r in range(0, DIM, P):
                rs = slice(r, min(r + P, DIM))
                acc = [a + _dot(row_v[0, :, rs], w[rs, c:c + 2 * P]) for a, w in zip(acc, ws)]
                yield 1
            for k in range(2):
                dst[k, :, c:c + 2 * P] = acc[k]

    wait(gate_up_copies(0))

    @pl.loop(0, NL)
    def _(e):
        start([down_copy(e)], 1)

    start([down_copy(NL)], 1)

    @pl.loop(NG, NG + NF)
    def _(i):
        f = i - NG
        c_step(i, 1.08, (c_transforms(i), 25, 1), (gate_up(f), FC // (2 * P) * 5 + 1.92, 0.49))
        pl.when(f + 2 == NF)(lambda: wait(gate_up_copies(1)))

    half_gate = 0.5 * jax.nn.sigmoid(row_v[1, :, :P])
    act_v[0] = _twice_silu_half(0.5 * act_v[0]) * act_v[1]

    def down(rows, result):
        w = wd_v.at[rows]
        acc = 0.0
        for c in range(0, FFN, 4 * P):
            acc = acc + functools.reduce(jnp.add, [
                _dot_nt(act_v[0, :, f:f + P], w[:, f:f + P]) for f in range(c, c + 4 * P, P)])
            yield 1
        yield from (1, 1, 1)
        result.append(_dot_nt(_eye(rows.size).astype(F32), acc * half_gate[:, :rows.size]))
        yield from (1, 1, 1)

    def gating(rows, update):
        h = jnp.concatenate([h_v[c, rows, :].astype(F32) for c in range(SEQ // HB)], axis=1)
        return _twice_silu_half(h + _dot(update, hot_v[...]))

    def emit(rows, g):
        s = s_v.at[GD:][rows, :]
        o_v[rows, :] = (x_v[rows, :].astype(F32) + s * g).astype(o_v.dtype)

    def finish(rows):
        update = []
        yield from down(rows, update)
        emit(rows, gating(rows, update[0]))

    down_copy(0).wait()

    @pl.loop(NG + NF, ND + 1)
    def _(i):
        e = i - (NG + NF)

        @pl.when(e < NL)
        def _():
            c_step(i, 0.99, (c_transforms(i), 25, 1), (finish(out_rows(e)), 15, 0.78))
            pl.when(e > 0)(lambda: start([out_copy(e - 1)], 1))
            pl.when(e + 1 == NL)(lambda: start([out_copy(NL - 1)], 1))
            pl.when(e + 1 < NL)(lambda: down_copy(e + 1).wait())
            pl.when(e + 1 == NL)(lambda: down_copy(NL).wait())

        @pl.when(e == NL)
        def _():
            c_step(ND - 1, 1.02, (c_inverses(ND - 1, 1), NB * 1.07, 0.5), (finish(out_rows(NL)), 15, 1.44),
                   groups=range(GT // 8))
            start([out_copy(NL)], 1)

        @pl.when(e == NL + 1)
        def _():
            update = []
            c_step(ND - 1, 1.06, (down(pl.ds(DIM - GD, GD), update), 15, 0.75), (c_inverses(ND, 1, 0, GT), NB, 0.5),
                   groups=range(GT // 8, GD // 8))
            upd_v[...] = update[0]

    g = gating(pl.ds(DIM - GD, GD), upd_v[...])
    emit(out_rows(NL + 1), g[:GT])
    start([out_copy(NL + 1)], 1)
    _run(c_inverses(ND, NB // 2, GT, GD - GT))
    emit(out_rows(NL + 2), g[GT:])
    start([out_copy(NL + 2)], 1)
    wait([out_copy(e) for e in range(NE)])


@jax.jit
def pallas_recurrent_scan__ssm_conv_s4__moe_arch_mod__prompt_kernel(
    A_u: jax.Array,
    A_A_re: jax.Array,
    A_A_im: jax.Array,
    A_B_re: jax.Array,
    A_B_im: jax.Array,
    A_C_re: jax.Array,
    A_C_im: jax.Array,
    A_log_dt: jax.Array,
    A_Dskip: jax.Array,
    B_x: jax.Array,
    B_w_r: jax.Array,
    B_w_gate: jax.Array,
    B_w_up: jax.Array,
    B_w_down: jax.Array,
):
    del B_x
    assert A_u.shape == (1, SEQ, DIM) and A_A_re.shape == (DIM, P) and B_w_gate.shape == (DIM, FFN)
    assert A_A_re.dtype == BF16
    hbm = pl.BlockSpec(memory_space=pl.ANY)
    out = pl.pallas_call(
        _kernel,
        out_shape=jax.ShapeDtypeStruct((DIM, SEQ), A_u.dtype),
        in_specs=[hbm] * 13,
        out_specs=hbm,
        scratch_shapes=[
            *[pltpu.VMEM((DIM,), BF16)] * 3,
            pltpu.VMEM((DIM, SEQ), BF16),
            pltpu.VMEM((6, DIM, P), BF16),
            pltpu.VMEM((DIM, FFN + P), BF16),
            pltpu.VMEM((DIM, FFN), BF16),
            pltpu.VMEM((DIM, FFN + P), BF16),
            pltpu.VMEM((P // 2, 2 * P), jnp.uint32),
            pltpu.VMEM((P, P), jnp.uint32),
            pltpu.VMEM((len(_window_layout()[0]) + 1, 8, 2 * P), jnp.uint32),
            pltpu.VMEM((DIM, SEQ), A_u.dtype),
            pltpu.VMEM((DIM, SEQ), BF16),
            pltpu.VMEM((SEQ // HB, DIM, HB), BF16),
            pltpu.VMEM((DIM + GD, SEQ), F32),
            pltpu.VMEM((10, DIM, P), F32),
            pltpu.VMEM((3, DIM, P), F32),
            pltpu.VMEM((2, 8, SEQ), F32),
            pltpu.VMEM((8, SEQ), F32),
            pltpu.VMEM((2, 8, FFN), F32),
            pltpu.VMEM((ND + 1, GD // 8, 8, NB + 1, 8, P), F32),
            pltpu.VMEM((26, DIM, P), F32),
            pltpu.VMEM((GD, 8), F32),
            pltpu.SemaphoreType.DMA((5,)),
        ],
        compiler_params=pltpu.CompilerParams(vmem_limit_bytes=112 * 2**20),
        name="ssm_moe",
    )(A_u[0].T, A_A_re, A_A_im, A_B_re, A_B_im, A_C_re, A_C_im, A_log_dt, A_Dskip, B_w_r,
      B_w_gate, B_w_up, B_w_down.T)
    return out.T[None]
```

```python
import functools

import jax
import jax.numpy as jnp
import numpy as np
import jax.experimental.pallas as pl
import jax.experimental.pallas.tpu as pltpu

F32 = jnp.float32
BF16 = jnp.bfloat16

SEQ, DIM, FFN = 2048, 576, 4608
P = 128
NB = SEQ // P
HB = SEQ // 4
GS, GL = 112, 128
GA = 288
GD = 64
ND = DIM // GD
NG, NF, NL = 2, 3, 3
FC = FFN // NF
GE, GT = 128, 48
LAST_ROWS = ((NL * GE, GE), (DIM - GD, GT), (DIM - GD + GT, GD - GT))
NE = NL + len(LAST_ROWS)
POWERS = (1, 8, 32, 256)
WINDOW_TILES = ((0,), (0, 1), (1, 2), (2,), (5,), (6,), (3,), (3,), (7,), (7,)) + ((4,),) * 6
WINDOW_PAIRS = ((14, 15), (12, 13), (10, 11), (1, 2), (8, 9), (6, 7), (4, 5), (0, 3))


def _bf16_bits(a):
    u = np.ascontiguousarray(a, dtype=np.float32).view(np.uint32)
    return ((u + 0x7FFF + ((u >> 16) & 1)) >> 16).astype(np.uint32)


def _tile_lags():
    lane = np.arange(P)
    quarter, hb, j = lane // 32, (lane // 16) % 2, lane % 16

    def half(offsets, second):
        return np.array(offsets)[(quarter + 2 * second) % 4] + 128 * (hb ^ second) + 8 * j

    l1, u1 = half((1, 2, 3, 4), 0), half((5, 6, 7, 8), 1)
    l2, u2 = half((258, 260, 516, 772), 0), half((262, 264, 520, 776), 1)
    l3, u3 = half((1032, 1288) * 2, 0), half((1544, 1800) * 2, 1)
    l4, u4 = half((516,) * 4, 0), half((520,) * 4, 1)
    lags = [np.where(hb == 0, l1, u1), np.where(hb == 0, u1, l1),
            np.where(lane < 64, l2, u2), np.where(lane < 64, u2, l2), np.where(lane < 64, l3, u3)]
    lags.append(np.where(lane < 16, l4, np.where(lane // 16 == 5, u4, lags[2])))
    lags.append(np.where(lane < 96, lags[3], lags[2]))
    lags.append(np.where(lane < 32, lags[4], lags[3]))
    return lags


def _window_lags(j):
    return 1 if j == 0 else -P + 1 + (j == 3), P - 1


@functools.cache
def _window_layout():
    lags = _tile_lags()
    m = np.arange(-P, P)
    groups, patterns, layout = [], [], []
    for j, tiles in enumerate(WINDOW_TILES):
        lo, hi = _window_lags(j)
        live = (m >= lo) & (m <= hi)
        rounded = (_bf16_bits(P * j + m) << 16).view(np.float32)
        hits = np.zeros(len(m), int)
        layout.append([])
        for t in tiles:
            sel = (lags[t][:, None] == rounded) & live
            hits += sel.sum(0)
            ids = []
            for r in range(0, P, 16):
                assert (lags[t][r:r + 16] == lags[t][r] + 8 * np.arange(16)).all()
                known = [n for n, e in enumerate(patterns) if np.array_equal(e, sel[r:r + 16])]
                if not sel[r:r + 16].any():
                    ids.append(None)
                elif known:
                    ids.append(known[0])
                else:
                    ids.append(len(groups))
                    groups.append((int(lags[t][r]), j))
                    patterns.append(sel[r:r + 16])
            layout[-1].append(ids)
        assert (hits == live).all()
    halves = [[n for n, e in enumerate(patterns) if e[:, h * P:(h + 1) * P].any()] for h in range(2)]
    return groups, halves, layout


def _cmul(a, b):
    return (a[0] * b[0] - a[1] * b[1], a[0] * b[1] + a[1] * b[0])


def _csq(a):
    t = a[0] * a[1]
    return ((a[0] - a[1]) * (a[0] + a[1]), t + t)


def _dot(a, b):
    return jax.lax.dot_general(a, b, (((1,), (0,)), ((), ())), preferred_element_type=F32)


def _dot_nt(a, b):
    return jax.lax.dot_general(a, b, (((1,), (1,)), ((), ())), preferred_element_type=F32)


def _round(x):
    return x.astype(BF16).astype(F32)


def _twice_silu_half(h):
    return h + h * jnp.tanh(h)


def _eye(n):
    return jax.lax.broadcasted_iota(jnp.int32, (n, n), 0) == jax.lax.broadcasted_iota(jnp.int32, (n, n), 1)


def _span(i, n):
    start = i * n
    return pl.ds(start if isinstance(start, int) else pl.multiple_of(start, n), n)


def _merge(*gens):
    state = [[0.0, k, g, total, cost] for k, (g, total, cost) in enumerate(gens)]
    while state:
        cur = min(state, key=lambda e: (e[0], e[1]))
        w = next(cur[2], None)
        if w is None:
            state.remove(cur)
        else:
            cur[0] += w / cur[3]
            yield w * cur[4]


def _after(delay, gen):
    yield delay
    yield from gen


def _run(gen):
    for _ in gen:
        pass


def _kernel(x_hbm, are_hbm, aim_hbm, bre_hbm, bim_hbm, cre_hbm, cim_hbm, ldt_hbm, dsk_hbm,
            wr_hbm, wg_hbm, wu_hbm, wd_hbm, o_hbm,
            ldt_v, dsk_v, wr_v, x_v, prm_v, wg_v, wu_v, wd_v, fwd_v, inv_v, win_v, o_v, d_v, h_v, s_v,
            lag_v, dt_v, row_v, hot_v, act_v, hat_v, pow_v, upd_v, sems):
    groups, halves, layout = _window_layout()
    lane8 = jax.lax.broadcasted_iota(jnp.int32, (8, P), 1)
    sub8 = jax.lax.broadcasted_iota(jnp.int32, (8, P), 0)

    def prm_copies(part):
        r = pl.ds(*((0, GS), (GS, 2 * GS), (3 * GS, DIM - 3 * GS))[part])
        return [pltpu.make_async_copy(src.at[r], prm_v.at[k, r], sems.at[1 + part % 2])
                for k, src in enumerate((are_hbm, aim_hbm, bre_hbm, bim_hbm, cre_hbm, cim_hbm))]

    vec_copies = [pltpu.make_async_copy(src, dst, sems.at[0])
                  for src, dst in ((ldt_hbm, ldt_v), (dsk_hbm, dsk_v), (wr_hbm, wr_v))]
    x_copy = pltpu.make_async_copy(x_hbm, x_v, sems.at[0])

    def gate_up_copies(part):
        cols = pl.ds(*((0, FFN - FC), (FFN - FC, FC))[part])
        return [pltpu.make_async_copy(src.at[:, cols], dst.at[:, cols], sems.at[3 + part])
                for src, dst in ((wg_hbm, wg_v), (wu_hbm, wu_v))]

    def out_rows(e):
        return pl.ds(*LAST_ROWS[e - NL]) if isinstance(e, int) and e >= NL else _span(e, GE)

    def down_copy(e):
        rows = pl.ds(NL * GE, DIM - NL * GE) if isinstance(e, int) and e == NL else _span(e, GE)
        return pltpu.make_async_copy(wd_hbm.at[rows], wd_v.at[rows, :FFN], sems.at[e])

    def out_copy(e):
        return pltpu.make_async_copy(o_v.at[out_rows(e)], o_hbm.at[out_rows(e)], sems.at[4])

    def start(copies, priority=0):
        for c in copies:
            c.start(priority=priority)

    def wait(copies):
        for c in copies:
            c.wait()

    start(vec_copies)

    @pl.loop(0, 2)
    def _(i):
        for part in range(2):
            @pl.when(i == part)
            def _():
                start(prm_copies(part))
                start(gate_up_copies(part), 1)

    def coords(re, im):
        b = im * (2 / np.sqrt(3).item())
        return jnp.concatenate([re + 0.5 * b, b], axis=1)

    def packed(v):
        return pltpu.bitcast(v.astype(BF16), jnp.uint32)

    angle = (((4 * lane8 + 1) * sub8) & (4 * P - 1)).astype(F32) * (np.pi / (2 * P))
    root = (jnp.cos(angle), jnp.sin(angle))
    step = tuple(v[4:5] for v in root)
    for _ in range(4):
        step = _csq(step)
        root = tuple(jnp.concatenate(v) for v in zip(root, _cmul(root, step)))
    powers = (coords(root[1], -root[0]), coords(*root))
    fwd_v[...] = packed(2.0 * powers[1])
    inv_v[...] = packed(jnp.concatenate([
        (root[0] * (1 / P)).T, ((root[1] * np.sqrt(3).item() - root[0]) * (0.5 / P)).T]))
    packed_powers = [v.astype(BF16) for v in powers]
    win_v[len(groups)] = pltpu.bitcast(jnp.broadcast_to(powers[0][1:2], (8, 2 * P)), jnp.uint32)

    def window_rows(n, h):
        lag, j = groups[n]
        m = jax.lax.broadcasted_iota(jnp.int32, (16, P), 1) + (h - 1) * P
        rounded = jnp.where(m >= _window_lags(j)[0], _round((m + P * j).astype(F32)), -1.0)
        return jnp.where(rounded == (8 * jax.lax.broadcasted_iota(jnp.int32, (16, P), 0) + lag).astype(F32), 1.0, 0.0)

    part = {}
    for h in range(2):
        prod = _dot(jnp.concatenate([window_rows(n, h) for n in halves[h]]), packed_powers[h])
        for k, n in enumerate(halves[h]):
            part[n] = part.get(n, 0.0) + prod[16 * k:16 * k + 16]
    for n in range(len(groups)):
        win_v[n] = packed(part[n])

    wait(vec_copies)
    dt_row, skip_row = (jnp.concatenate([v[None, :], jnp.zeros((1, -DIM % P), F32)], axis=1)
                        for v in (_round(jnp.exp(ldt_v[...].astype(F32))), dsk_v[...].astype(F32)))

    for c in range(0, DIM, P):
        n = min(P, DIM - c)
        dt, skip = (jnp.where(_eye(P)[:n], v[:, c:c + P], 0.0) for v in (dt_row, skip_row))
        dt_v[0, c:c + n, :] = _dot(dt, jnp.ones((P, P), BF16))
        dt_v[1, c:c + n, :] = skip

    def k_setup(rows, have_mag=False):
        low = sub8 < 4
        dst = pow_v.at[:, rows]
        for g in range(rows.size // 16):
            sl = slice(16 * g, 16 * g + 16)
            dt, skip = (dt_v.at[k, rows][sl, :] for k in range(2))
            a_re, a_im, b_re, b_im, c_re, c_im = (prm_v.at[k, rows][sl, :].astype(F32) for k in range(6))
            w = {0: _cmul((c_re, c_im), (dt * b_re, dt * b_im))}
            mag = dt_v.at[2, rows][sl, :] if have_mag else jnp.exp(dt * a_re)
            yield 1
            rot = []
            for phase in jnp.split(dt * a_im, 2):
                rot.append((jnp.cos(phase), jnp.sin(phase)))
                yield 4.5
            z = {1: tuple(mag * jnp.concatenate(v) for v in zip(*rot))}
            for e in range(10):
                z[2 << e] = _csq(z[1 << e])
            for n, e in enumerate(POWERS):
                for q in range(2):
                    dst[2 * n + q, sl, :] = z[e][q]
            yield 3
            dst[24, sl, :] = w[0][0] + skip
            dst[25, sl, :] = w[0][0] * z[256][0] - w[0][1] * z[256][1]
            w[4], w[8] = _cmul(w[0], z[4]), _cmul(w[0], z[8])
            w[1032] = _cmul(w[8], z[1024])
            w[1544] = _cmul(w[1032], z[512])
            one = (jnp.ones((16, P), F32), jnp.zeros((16, P), F32))
            for n, (a, b) in enumerate(((one, z[128]), (w[0], w[4]), (w[4], w[8]), (w[1032], w[1544]))):
                for q in range(2):
                    for t in range(2):
                        x, y = a[q][8 * t:8 * t + 8], pltpu.roll(b[q][8 * t:8 * t + 8], 4, 0)
                        r = slice(16 * g + 8 * t, 16 * g + 8 * t + 8)
                        dst[8 + 4 * n + q, r, :] = jnp.where(low, x, y)
                        dst[10 + 4 * n + q, r, :] = jnp.where(low, y, x)
            yield 3

    def k_lags(i):
        low = sub8 < 4
        bit4, bit5, bit6 = ((lane8 & b) == 0 for b in (16, 32, 64))
        bit6x = ((lane8 >> 4) ^ sub8) & 4 == 0
        own = ((lane8 & 15) * 8 + (((lane8 >> 2) & 4) ^ sub8)) ^ 120
        src, dst = pow_v.at[:, _span(i, GA)], lag_v.at[:, _span(i, GA)]
        for t in range(2):
            dst[8 + t] = jnp.broadcast_to(jnp.sum(src[24 + t], axis=1, keepdims=True), (GA, P))

        def unzip(xs):
            return jnp.where(low, xs[0], xs[1]), pltpu.roll(jnp.where(low, xs[1], xs[0]), 4, 0)

        for g in range(GA // 8):
            sl = slice(8 * g, 8 * g + 8)
            prod = []
            for h in range(2):
                off = 4 * h if g + 1 < GA // 8 else 4 * h - 4
                z = {e: tuple(jnp.take_along_axis(src[2 * n + q, 8 * g + off:8 * g + off + 8, :],
                                                  (sub8 & 3) + (4 * h - off), axis=0,
                                                  mode="promise_in_bounds") for q in range(2))
                     for n, e in enumerate(POWERS)}
                b0, a0, a4, far = (tuple(src[8 + 4 * n + 2 * h + q, sl, :] for q in range(2)) for n in range(4))
                bs = [b0]
                for j in range(1, 16):
                    bs.append(_cmul(bs[j - 1], z[8]) if j < 4 else _cmul(bs[j - 4], z[32]))
                av = [_cmul(a0, z[1])]
                av += [_cmul(av[0], z[1])]
                av += [_cmul(av[1], z[1]), a4, _cmul(av[1], z[256]), _cmul(a4, z[256])]
                av += [_cmul(av[-1], z[256])]
                av += [_cmul(av[-1], z[256]), far, _cmul(far, z[256])]
                prod.append([_dot_nt(jnp.concatenate([v[q] for v in av]),
                                     jnp.concatenate([v[q] for v in reversed(bs)]).astype(BF16))
                             for q in range(2)])
            real = [re - im for re, im in prod]
            v = [[jnp.take_along_axis(real[h][8 * n:8 * n + 8], own, axis=1, mode="promise_in_bounds")
                  for h in range(2)] for n in range(10)]
            halves = []
            for lo, hi in ((0, 4), (4, 8), (8, 10)):
                xs = []
                for h in range(2):
                    u = [jnp.where(bit5, v[n][h], v[n + 1][h]) for n in range(lo, hi, 2)]
                    xs.append(jnp.where(bit6x, u[h], u[1 - h]) if len(u) == 2 else u[0])
                halves.append(unzip(xs))
            (l1, u1), (l2, u2), (l3, u3) = halves
            l4, u4 = unzip(v[6])
            tiles = [jnp.where(bit4, l1, u1), jnp.where(bit4, u1, l1), jnp.where(bit6, l2, u2),
                     jnp.where(bit6, u2, l2), jnp.where(bit6, l3, u3)]
            tiles.append(jnp.where(lane8 < 16, l4, jnp.where((lane8 >> 4) == 5, u4, tiles[2])))
            tiles.append(jnp.where(lane8 < 96, tiles[3], tiles[2]))
            tiles.append(jnp.where(lane8 < 32, tiles[4], tiles[3]))
            dst[:8, sl, :] = jnp.stack(tiles)

    wait(prm_copies(0))
    start(prm_copies(2))

    @pl.loop(0, (DIM - GL) // GS)
    def _(i):
        pl.when(i == 0)(x_copy.start)
        pl.when(i == 1)(lambda: wait(prm_copies(1)))
        pl.when(i == 3)(lambda: wait(prm_copies(2)))
        _run(k_setup(_span(i, GS)))

    def compact(v):
        return jnp.concatenate([functools.reduce(
            lambda a, q: jnp.where(sub8 == q, v[:, (c + q) * P:(c + q + 1) * P], a),
            range(1, 8), v[:, c * P:(c + 1) * P]) for c in range(0, NB, 8)])

    def spread(v):
        return jnp.concatenate([jnp.broadcast_to(v[c:c + 1], (8, P)) for c in range(NB)], axis=1)

    def mean(k):
        return compact(jnp.broadcast_to(jnp.sum(row_v[k], axis=0, keepdims=True), (8, SEQ))) / DIM

    def h_block(rows, c):
        return h_v[c * P // HB, rows, c * P % HB:c * P % HB + P]

    def layer_norm():
        x_copy.wait()
        row_v[0] = jnp.zeros((8, SEQ), F32)

        @pl.loop(0, DIM // 96)
        def _(i):
            src = x_v.at[_span(i, 96)]
            acc = row_v[0]
            for r in range(0, 96, 8):
                acc = acc + src[r:r + 8, :].astype(F32)
            row_v[0] = acc

        m = mean(0)
        mb = _round(m)
        row_v[0] = spread(mb)

        @pl.loop(0, 8)
        def _(c):
            cols = _span(c, SEQ // 8)
            src, dst, centre = x_v.at[:, cols], d_v.at[:, cols], row_v[0, :, cols]
            acc = [0.0] * 4
            for r in range(0, DIM, 8):
                d = src[r:r + 8, :].astype(F32) - centre
                dst[r:r + 8, :] = d.astype(BF16)
                acc[r // 8 % 4] += d * d
            row_v[1, :, cols] = (acc[0] + acc[1]) + (acc[2] + acc[3])

        late = pl.ds(DIM - GL, GL)
        dt_v[2, late, :] = jnp.exp(dt_v[0, late, :] * prm_v[0, late, :].astype(F32))
        var = jnp.maximum(mean(1) - (m - mb) * (m - mb), 0.0)
        row_v[0] = spread(0.5 / _round(jnp.sqrt(_round(_round(var) + _round(jnp.full_like(var, 1e-5))))))

        def normalise(c):
            src, scale = d_v.at[:, _span(c, HB)], jnp.concatenate([row_v[0, :, _span(c, HB)]] * 4)
            for r in range(0, DIM, 32):
                h_v[c, r:r + 32, :] = (src[r:r + 32, :].astype(F32) * scale).astype(BF16)

        pl.loop(0, SEQ // HB)(normalise)

    def put(i, kind, c, v):
        a, b = v[:, :P], v[:, P:]
        for q, u in enumerate((a, b, a - b)):
            hat_v[i, :, 3 * kind + q, c] = u.reshape(GD // 8, 8, P)

    def c_signal(i, c):
        put(i, 0, c, _dot(h_block(_span(i, GD), c), pltpu.bitcast(fwd_v[...], BF16)))

    def c_window(i, j):
        tiles = lag_v.at[:, _span(i, GD)]
        parts = []
        for t, ids in zip(WINDOW_TILES[j], layout[j]):
            rhs = jnp.concatenate([jnp.zeros((8, 2 * P), jnp.uint32) if n is None else win_v[n] for n in ids])
            parts.append(_dot(tiles[t], pltpu.bitcast(rhs, BF16)))
        kh = functools.reduce(jnp.add, parts)
        if j == 0:
            kh = jnp.concatenate([kh[:, :P] + tiles[8], kh[:, P:]], axis=1)
        if j == 3:
            edge = pltpu.bitcast(win_v[win_v.shape[0] - 1], F32)
            kh = kh + jnp.concatenate([tiles[9]] * 2, axis=1) * jnp.concatenate([edge] * (GD // 8))
        put(i, 1, j, kh)

    def c_inverse(i, blocks, r0=0, n=GD):
        lhs = jnp.concatenate([jnp.concatenate([
            hat_v[i, r0 // 8:(r0 + n) // 8, 6 + q, c].reshape(n, P) for q in range(2)], axis=1) for c in blocks])
        y = _dot(lhs, pltpu.bitcast(inv_v[...], BF16))
        for k, c in enumerate(blocks):
            s_v.at[_span(i, GD)][r0:r0 + n, c * P:(c + 1) * P] = y[k * n:(k + 1) * n]

    def c_inverses(i, stack, *rows):
        for c in range(0, NB, 2 * stack):
            c_inverse(i, range(c, c + stack), *rows)
            c_inverse(i, range(c + stack, c + 2 * stack), *rows)
            yield 2 * stack

    def c_transforms(i, inverse=True):
        for c, pair in zip(range(0, NB, 2), WINDOW_PAIRS):
            c_signal(i + 1, c)
            if inverse:
                c_inverse(i, [c])
                yield 1
            c_signal(i + 1, c + 1)
            if inverse:
                c_inverse(i, [c + 1])
            yield 1
            for j in pair:
                c_window(i + 1, j)
            yield len(WINDOW_TILES[pair[0]])

    def c_product(i, groups):
        for g in groups:
            for lo in (8, 0):
                for q in range(3):
                    acc = []
                    for j in reversed(range(lo + 8)):
                        first = max(lo, j)
                        t = hat_v[i, g, 3 + q, j] * hat_v[i, g, q, first - j:lo + 8 - j]
                        if q:
                            acc = [jnp.concatenate(([base[j - lo:j - lo + 1]] if j >= lo else []) + acc) - t]
                        elif j >= lo:
                            acc = [jnp.concatenate([t[:1]] + [a + t[1:] for a in acc])]
                        else:
                            acc = [acc[0] + t]
                        yield lo + 8 - first
                    if q:
                        hat_v[i + 1, g, 5 + q, lo:lo + 8] = acc[0]
                    else:
                        base = acc[0]

    def c_step(i, pace, *side, groups=range(GD // 8)):
        _run(_merge((c_product(i, groups), len(groups) * 3 * 136, 1),
                    (_merge(*side), sum(total * cost for _, total, cost in side) * pace, 1)))

    def select():
        wr = jnp.broadcast_to(2.0 * wr_v[...].astype(F32)[None, :], (8, DIM))
        score = [0.0] * (SEQ // HB)
        for c in range(SEQ // HB):
            for r in range(0, DIM, P):
                rs = slice(r, min(r + P, DIM))
                score[c] = score[c] + _dot(wr[:, rs], h_v[c, rs, :])
                yield 0.27
        score = _round(compact(jnp.concatenate(score, axis=1)))
        bits = pltpu.bitcast(jnp.where(score == 0.0, 0.0, score), jnp.int32)
        ordered = jnp.where(bits < 0, ~bits, bits ^ -2**31)
        token = jax.lax.broadcasted_iota(jnp.int32, (NB, P), 0) * P + jax.lax.broadcasted_iota(jnp.int32, (NB, P), 1)
        key = pltpu.bitcast((jax.lax.shift_right_logical(ordered, 16) << 11) + (0x20000000 + SEQ - 1 - token), F32)
        rest, top = key, jnp.zeros((8, P), F32)
        yield 2.34
        for q in range(8):
            best = jnp.max(jnp.max(rest, axis=0, keepdims=True), axis=1, keepdims=True)
            top = jnp.where(sub8 == q, best, top)
            rest = jnp.where(rest == best, 0.0, rest)
            yield 1
        hot_v[...] = jnp.where(spread(key) == jnp.concatenate([top] * NB, axis=1), 1.0, 0.0)
        ordered = jax.lax.shift_right_logical(pltpu.bitcast(top, jnp.int32) - 0x20000000, 11) << 16
        row_v[1, :, :P] = pltpu.bitcast(jnp.where(ordered < 0, ordered ^ -2**31, ~ordered & -65536), F32)

    @pl.loop(0, DIM // GA)
    def _(i):
        k_lags(i)

        @pl.when(i == 0)
        def _():
            layer_norm()
            _run(_merge((k_setup(pl.ds(DIM - GL, GL), have_mag=True), GL, 1),
                        (_after(9.29, c_transforms(-1, inverse=False)), 27.65, 1),
                        (select(), 16.92, 1)))

    def gather(lo, hi):
        for r in range(lo, hi, P):
            rs = slice(r, min(r + P, DIM))
            part = 0.0
            for c0 in range(0, NB, 4):
                part = part + functools.reduce(jnp.add, [
                    _dot_nt(hot_v[:, c * P:(c + 1) * P], h_block(rs, c)) for c in range(c0, c0 + 4)])
                yield 1
            row_v[0, :, rs] = 2.0 * part

    @pl.loop(0, NG)
    def _(i):
        @pl.when(i == 0)
        def _():
            c_step(0, 0.98, (c_transforms(0, inverse=False), 17, 1), (gather(0, 4 * P), 16.5, 1.23))

        @pl.when(i > 0)
        def _():
            c_step(i, 1.0, (c_transforms(i), 25, 1), (gather(4 * P, DIM), 4, 0.28))

    def gate_up(f):
        ws, dst = (wg_v.at[:, _span(f, FC)], wu_v.at[:, _span(f, FC)]), act_v.at[:, :, _span(f, FC)]
        for c in range(0, FC, 2 * P):
            acc = [0.0, 0.0]
            for r in range(0, DIM, P):
                rs = slice(r, min(r + P, DIM))
                acc = [a + _dot(row_v[0, :, rs], w[rs, c:c + 2 * P]) for a, w in zip(acc, ws)]
                yield 1
            for k in range(2):
                dst[k, :, c:c + 2 * P] = acc[k]

    wait(gate_up_copies(0))

    @pl.loop(0, NL)
    def _(e):
        start([down_copy(e)], 1)

    start([down_copy(NL)], 1)

    @pl.loop(NG, NG + NF)
    def _(i):
        f = i - NG
        c_step(i, 1.08, (c_transforms(i), 25, 1), (gate_up(f), FC // (2 * P) * 5 + 1.92, 0.49))
        pl.when(f + 2 == NF)(lambda: wait(gate_up_copies(1)))

    half_gate = 0.5 * jax.nn.sigmoid(row_v[1, :, :P])
    act_v[0] = _twice_silu_half(0.5 * act_v[0]) * act_v[1]

    def down(rows, result):
        w = wd_v.at[rows]
        acc = 0.0
        for c in range(0, FFN, 4 * P):
            acc = acc + functools.reduce(jnp.add, [
                _dot_nt(act_v[0, :, f:f + P], w[:, f:f + P]) for f in range(c, c + 4 * P, P)])
            yield 1
        yield from (1, 1, 1)
        result.append(_dot_nt(_eye(rows.size).astype(F32), acc * half_gate[:, :rows.size]))
        yield from (1, 1, 1)

    def gating(rows, update):
        h = jnp.concatenate([h_v[c, rows, :].astype(F32) for c in range(SEQ // HB)], axis=1)
        return _twice_silu_half(h + _dot(update, hot_v[...]))

    def emit(rows, g):
        s = s_v.at[GD:][rows, :]
        o_v[rows, :] = (x_v[rows, :].astype(F32) + s * g).astype(o_v.dtype)

    def finish(rows):
        update = []
        yield from down(rows, update)
        emit(rows, gating(rows, update[0]))

    down_copy(0).wait()

    @pl.loop(NG + NF, ND + 1)
    def _(i):
        e = i - (NG + NF)

        @pl.when(e < NL)
        def _():
            c_step(i, 0.99, (c_transforms(i), 25, 1), (finish(out_rows(e)), 15, 0.78))
            pl.when(e > 0)(lambda: start([out_copy(e - 1)], 1))
            pl.when(e + 1 == NL)(lambda: start([out_copy(NL - 1)], 1))
            pl.when(e + 1 < NL)(lambda: down_copy(e + 1).wait())
            pl.when(e + 1 == NL)(lambda: down_copy(NL).wait())

        @pl.when(e == NL)
        def _():
            c_step(ND - 1, 1.02, (c_inverses(ND - 1, 1), NB * 1.07, 0.5), (finish(out_rows(NL)), 15, 1.44),
                   groups=range(GT // 8))
            start([out_copy(NL)], 1)

        @pl.when(e == NL + 1)
        def _():
            update = []
            c_step(ND - 1, 1.06, (down(pl.ds(DIM - GD, GD), update), 15, 0.75), (c_inverses(ND, 1, 0, GT), NB, 0.5),
                   groups=range(GT // 8, GD // 8))
            upd_v[...] = update[0]

    g = gating(pl.ds(DIM - GD, GD), upd_v[...])
    emit(out_rows(NL + 1), g[:GT])
    start([out_copy(NL + 1)], 1)
    _run(c_inverses(ND, NB // 2, GT, GD - GT))
    emit(out_rows(NL + 2), g[GT:])
    start([out_copy(NL + 2)], 1)
    wait([out_copy(e) for e in range(NE)])


@jax.jit
def pallas_recurrent_scan__ssm_conv_s4__moe_arch_mod__prompt_kernel(
    A_u: jax.Array,
    A_A_re: jax.Array,
    A_A_im: jax.Array,
    A_B_re: jax.Array,
    A_B_im: jax.Array,
    A_C_re: jax.Array,
    A_C_im: jax.Array,
    A_log_dt: jax.Array,
    A_Dskip: jax.Array,
    B_x: jax.Array,
    B_w_r: jax.Array,
    B_w_gate: jax.Array,
    B_w_up: jax.Array,
    B_w_down: jax.Array,
):
    del B_x
    assert A_u.shape == (1, SEQ, DIM) and A_A_re.shape == (DIM, P) and B_w_gate.shape == (DIM, FFN)
    assert A_A_re.dtype == BF16
    hbm = pl.BlockSpec(memory_space=pl.ANY)
    out = pl.pallas_call(
        _kernel,
        out_shape=jax.ShapeDtypeStruct((DIM, SEQ), A_u.dtype),
        in_specs=[hbm] * 13,
        out_specs=hbm,
        scratch_shapes=[
            *[pltpu.VMEM((DIM,), BF16)] * 3,
            pltpu.VMEM((DIM, SEQ), BF16),
            pltpu.VMEM((6, DIM, P), BF16),
            pltpu.VMEM((DIM, FFN + P), BF16),
            pltpu.VMEM((DIM, FFN), BF16),
            pltpu.VMEM((DIM, FFN + P), BF16),
            pltpu.VMEM((P // 2, 2 * P), jnp.uint32),
            pltpu.VMEM((P, P), jnp.uint32),
            pltpu.VMEM((len(_window_layout()[0]) + 1, 8, 2 * P), jnp.uint32),
            pltpu.VMEM((DIM, SEQ), A_u.dtype),
            pltpu.VMEM((DIM, SEQ), BF16),
            pltpu.VMEM((SEQ // HB, DIM, HB), BF16),
            pltpu.VMEM((DIM + GD, SEQ), F32),
            pltpu.VMEM((10, DIM, P), F32),
            pltpu.VMEM((3, DIM, P), F32),
            pltpu.VMEM((2, 8, SEQ), F32),
            pltpu.VMEM((8, SEQ), F32),
            pltpu.VMEM((2, 8, FFN), F32),
            pltpu.VMEM((ND + 1, GD // 8, 8, NB + 1, 8, P), F32),
            pltpu.VMEM((26, DIM, P), F32),
            pltpu.VMEM((GD, 8), F32),
            pltpu.SemaphoreType.DMA((5,)),
        ],
        compiler_params=pltpu.CompilerParams(vmem_limit_bytes=112 * 2**20),
        name="ssm_moe",
    )(A_u[0].T, A_A_re, A_A_im, A_B_re, A_B_im, A_C_re, A_C_im, A_log_dt, A_Dskip, B_w_r,
      B_w_gate, B_w_up, B_w_down.T)
    return out.T[None]
```
